```python
import os as _os
_os.environ.setdefault("JAX_PLATFORMS", "cpu")
import jax
import jax.numpy as jnp

def _softmax(x, axis=-1):
    return jax.nn.softmax(x, axis=axis)
def _gelu(x):
    return jax.nn.gelu(x, approximate=True)
def _silu(x):
    return jax.nn.silu(x)
def _sigmoid(x):
    return jax.nn.sigmoid(x)
def _layernorm(x, axis=-1, eps=1e-5):
    m = jnp.mean(x, axis=axis, keepdims=True)
    v = jnp.var(x, axis=axis, keepdims=True)
    return (x - m) / jnp.sqrt(v + eps)
def _scatter_add(tgt, idx, src, axis=0):
    return tgt.at[idx].add(src)
def _segment_sum(src, seg, n):
    return jax.ops.segment_sum(src, seg, n)
class _Rng:
    def __init__(self, key):
        self._k = key
    def _next(self):
        self._k, sub = jax.random.split(self._k)
        return sub
    def normal(self, shape):
        return jax.random.normal(self._next(), shape, dtype=jnp.bfloat16)
    def randint(self, lo, hi, shape):
        return jax.random.randint(self._next(), shape, lo, hi, dtype=jnp.int32)
    def uniform(self, shape, lo=0.0, hi=1.0):
        return jax.random.uniform(self._next(), shape, jnp.bfloat16, lo, hi)
    def permutation(self, n):
        return jax.random.permutation(self._next(), n)


kernel_name = 'sequential_preLN__spectral_gfnet__glu_gated_bilinear__prompt'

def setup_inputs():
    _rng = _Rng(jax.random.key(int.from_bytes(__import__("os").urandom(4), "little")))
    _w = (lambda a: (lambda t: t.astype(jnp.bfloat16) if jnp.issubdtype(t.dtype, jnp.floating) else t)(jnp.asarray(a)))
    def _A_setup():
        B, S, D = 1, 2048, 448
        Df = D // 2 + 1
        return {
            "x": _w((lambda *s: _rng.normal(s) * 0.05)(B, S, D)),
            "w_r": _w((lambda *s: _rng.normal(s) * 0.2)(S, Df) * 0.02),
            "w_i": _w((lambda *s: _rng.normal(s) * 0.2)(S, Df) * 0.02),
        }
    _A_in = _A_setup()

    def _B_setup():
        B, S, D, F = 1, 2048, 448, 1792
        return {
            "x": _w((lambda *s: _rng.normal(s) * 0.05)(B, S, D)),
            "w_gate": _w((lambda *s: _rng.normal(s) * 0.05)(D, F) * (D ** -0.5)),
            "w_up": _w((lambda *s: _rng.normal(s) * 0.05)(D, F) * (D ** -0.5)),
            "w_down": _w((lambda *s: _rng.normal(s) * 0.05)(F, D) * (F ** -0.5)),
        }
    _B_in = _B_setup()

    return {
        "A_x": _A_in["x"],
        "A_w_r": _A_in["w_r"],
        "A_w_i": _A_in["w_i"],
        "B_x": _B_in["x"],
        "B_w_gate": _B_in["w_gate"],
        "B_w_up": _B_in["w_up"],
        "B_w_down": _B_in["w_down"],
    }

def reference(A_x, A_w_r, A_w_i, B_x, B_w_gate, B_w_up, B_w_down):
    def _A_ref(x, w_r, w_i):
        B, S, D = x.shape
        X = (lambda x, axes=(-2,-1): jnp.fft.rfft2(x.astype(jnp.float32), axes=axes))(x, axes=(-2, -1))
        W = w_r + 1j * w_i
        X = X * W
        y = (lambda x, s, axes=(-2,-1): jnp.fft.irfft2(x, s=s, axes=axes).astype(jnp.bfloat16))(X, (S, D), axes=(-2, -1))
        return y

    def _B_ref(x, w_gate, w_up, w_down):
        g = jnp.einsum("bsd,df->bsf", x, w_gate)
        u = jnp.einsum("bsd,df->bsf", x, w_up)
        h = g * u
        return jnp.einsum("bsf,fd->bsd", h, w_down)

    x = A_x
    h = x + _A_ref(_layernorm(x, axis=-1), A_w_r, A_w_i)
    h2 = h + _B_ref(_layernorm(h, axis=-1), B_w_gate, B_w_up, B_w_down)
    return h2
```

```python
import functools
import numpy as np
import jax
import jax.numpy as jnp
from jax import lax
from jax.experimental import pallas as pl
from jax.experimental.pallas import tpu as pltpu

S, D, F = 2048, 448, 1792
DH = D // 2
NT = S // 128
EPS = 1e-5
bf16 = jnp.bfloat16
f32 = jnp.float32
u32 = jnp.uint32
NT_DIMS = (((1,), (1,)), ((), ()))


def _make_consts():
    d = np.arange(DH)[None, :].astype(np.float64)
    m = np.arange(128)[:, None].astype(np.float64)
    angE = 2 * np.pi * (2 * m) * d / D
    angO = 2 * np.pi * (2 * m + 1) * d / D
    vE = (m <= 112)
    vO = (m <= 111)
    FeT = np.concatenate([np.where(vE, np.cos(angE), 0), np.where(vE, -np.sin(angE), 0)], 0)
    FoT = np.concatenate([np.where(vO, np.cos(angO), 0), np.where(vO, -np.sin(angO), 0)], 0)
    fd = np.stack([np.pad(FeT, ((0, 0), (0, 32))), np.pad(FoT, ((0, 0), (0, 32)))])
    k2 = np.arange(128)[:, None]
    s2 = np.arange(128)[None, :]
    G = np.zeros((16, 256, 128))
    GH = np.zeros((16, 256, 128))
    for k1 in range(16):
        ang = 2 * np.pi * ((s2 * (k1 + 16 * k2)) % S) / S
        Gr, Gi = np.cos(ang), -np.sin(ang)
        G[k1, :128], G[k1, 128:] = Gr, Gi
        GH[k1, :128], GH[k1, 128:] = Gr.T, Gi.T
    dd = np.arange(DH)[:, None].astype(np.float64)
    mm = np.arange(128)[None, :].astype(np.float64)
    cE = np.where((mm == 0) | (mm == 112), 1.0, 2.0) * (mm <= 112)
    cO = 2.0 * (mm <= 111)
    sc = 1.0 / (D * S)
    aE = 2 * np.pi * (2 * mm) * dd / D
    aO = 2 * np.pi * (2 * mm + 1) * dd / D
    BeT = np.concatenate([cE * np.cos(aE), -cE * np.sin(aE)], 1) * sc
    BoT = np.concatenate([cO * np.cos(aO), -cO * np.sin(aO)], 1) * sc
    bd = np.stack([BeT, BoT])
    cast = lambda a: np.asarray(a, np.float32).astype(bf16)
    return cast(fd), cast(G), cast(GH), cast(bd)


class V:
    __slots__ = ("a", "n")

    def __init__(self, a, n=False):
        self.a, self.n = a, n

    def __neg__(self):
        return V(self.a, not self.n)

    def __add__(self, o):
        if not self.n and not o.n:
            return V(self.a + o.a)
        if not self.n and o.n:
            return V(self.a - o.a)
        if self.n and not o.n:
            return V(o.a - self.a)
        return V(self.a + o.a, True)

    def __sub__(self, o):
        return self + (-o)

    def mul(self, c):
        return V(self.a * np.float32(-c if self.n else c))

    def val(self):
        return -self.a if self.n else self.a


def _r4(x, sg):
    (x0r, x0i), (x1r, x1i), (x2r, x2i), (x3r, x3i) = x
    t0r, t0i = x0r + x2r, x0i + x2i
    t1r, t1i = x0r - x2r, x0i - x2i
    t2r, t2i = x1r + x3r, x1i + x3i
    t3r, t3i = x1r - x3r, x1i - x3i
    if sg > 0:
        ur, ui = -t3i, t3r
    else:
        ur, ui = t3i, -t3r
    return [(t0r + t2r, t0i + t2i), (t1r + ur, t1i + ui), (t0r - t2r, t0i - t2i), (t1r - ur, t1i - ui)]


def _tw(x, e, sg):
    xr, xi = x
    e = e % 16
    if e % 4 == 0:
        q = (e // 4) if sg > 0 else (-(e // 4)) % 4
        q %= 4
        if q == 0:
            return xr, xi
        if q == 1:
            return -xi, xr
        if q == 2:
            return -xr, -xi
        return xi, -xr
    c, s = np.cos(2 * np.pi * e / 16), sg * np.sin(2 * np.pi * e / 16)
    if e % 2 == 0:
        h = abs(c)
        sc_, ss_ = (1 if c > 0 else -1), (1 if s > 0 else -1)
        a = xr if sc_ > 0 else -xr
        b = xi if ss_ > 0 else -xi
        re = (a - b).mul(h)
        a = xi if sc_ > 0 else -xi
        b = xr if ss_ > 0 else -xr
        im = (a + b).mul(h)
        return re, im
    return xr.mul(c) - xi.mul(s), xi.mul(c) + xr.mul(s)


def _fft16(re, im, sg):
    x = [(V(re[a]), V(im[a])) for a in range(16)]
    T = [_r4([x[4 * a1 + a0] for a1 in range(4)], sg) for a0 in range(4)]
    out_re, out_im = [None] * 16, [None] * 16
    for k0 in range(4):
        col = [_tw(T[a0][k0], a0 * k0, sg) for a0 in range(4)]
        y = _r4(col, sg)
        for k1 in range(4):
            out_re[k0 + 4 * k1] = y[k1][0].val()
            out_im[k0 + 4 * k1] = y[k1][1].val()
    return out_re, out_im


def _ln_T(x):
    m = jnp.sum(x, axis=0, keepdims=True) * (1.0 / D)
    xc = x - m
    v = jnp.sum(xc * xc, axis=0, keepdims=True) * (1.0 / D)
    return xc * lax.rsqrt(v + EPS)


WP = 136


def _kernel(x_hbm, wr_hbm, wi_hbm, wg_hbm, wu_hbm, wd_hbm, fd_hbm, g_hbm, gh_hbm, bd_hbm,
            out_hbm,
            x_v, wr_v, wi_v, wg_v, wu_v, wd_v, fd_v, g_v, gh_v, bd_v,
            X1, Y, Wtr, Wti, Vb, Z, out_v, sems, osems):
    XC = 4
    cw = S // XC
    x_cp = [pltpu.make_async_copy(x_hbm.at[:, pl.ds(c * cw, cw)], x_v.at[:, pl.ds(c * cw, cw)], sems.at[c])
            for c in range(XC)]
    cp_fd = pltpu.make_async_copy(fd_hbm, fd_v, sems.at[4])
    cp_wr = pltpu.make_async_copy(wr_hbm, wr_v, sems.at[5])
    cp_wi = pltpu.make_async_copy(wi_hbm, wi_v, sems.at[6])
    cp_g = pltpu.make_async_copy(g_hbm, g_v, sems.at[7])
    cp_gh = pltpu.make_async_copy(gh_hbm, gh_v, sems.at[8])
    cp_bd = pltpu.make_async_copy(bd_hbm, bd_v, sems.at[9])
    cp_wg = pltpu.make_async_copy(wg_hbm, wg_v, sems.at[10])
    cp_wu = pltpu.make_async_copy(wu_hbm, wu_v, sems.at[11])
    cp_wd = pltpu.make_async_copy(wd_hbm, wd_v, sems.at[12])
    x_cp[0].start()
    cp_fd.start()
    for c in range(1, XC):
        x_cp[c].start()
    for cp in (cp_wr, cp_wi, cp_g, cp_gh, cp_bd, cp_wg, cp_wu, cp_wd):
        cp.start()

    cp_fd.wait()
    zpad = jnp.zeros((32, 128), bf16)
    for a in range(NT):
        if a % (NT // XC) == 0:
            x_cp[a // (NT // XC)].wait()
        xn = _ln_T(x_v[:, a * 128:(a + 1) * 128].astype(f32))
        xa, xb = xn[:DH], xn[DH:]
        e = jnp.concatenate([(xa + xb).astype(bf16), zpad], axis=0)
        o = jnp.concatenate([(xa - xb).astype(bf16), zpad], axis=0)
        X1[a, 0:256, :] = jnp.dot(fd_v[0], e, preferred_element_type=f32)
        X1[a, 256:512, :] = jnp.dot(fd_v[1], o, preferred_element_type=f32)

    cp_wr.wait()
    cp_wi.wait()
    rows = lax.broadcasted_iota(jnp.int32, (8, 128), 0)
    for w_v, Wt in ((wr_v, Wtr), (wi_v, Wti)):
        for a in range(NT):
            w32 = pltpu.bitcast(w_v[0:DH, a * 128:(a + 1) * 128], u32)
            ny = w_v[DH:DH + 1, a * 128:(a + 1) * 128].astype(f32)
            ny = jnp.broadcast_to(ny, (8, 128))
            nyu = lax.shift_right_logical(lax.bitcast_convert_type(ny, u32), np.uint32(16))
            nyu = jnp.where(rows == 0, nyu, np.uint32(0))
            t = jnp.concatenate([w32, nyu, jnp.zeros((8, 128), u32)], axis=0).T
            for j in range(8):
                Wt[pl.ds(a * WP + 17 * j, 16), :] = t[16 * j:16 * j + 16, :]

    for p in range(2):
        for r in range(0, 128, 16):
            re = [X1[a, p * 256 + r:p * 256 + r + 16, :] for a in range(16)]
            im = [X1[a, p * 256 + 128 + r:p * 256 + 128 + r + 16, :] for a in range(16)]
            ore, oim = _fft16(re, im, -1)
            for k1 in range(16):
                Y[k1, p * 256 + r:p * 256 + r + 16, :] = ore[k1].astype(bf16)
                Y[k1, p * 256 + 128 + r:p * 256 + 128 + r + 16, :] = oim[k1].astype(bf16)

    cp_g.wait()
    cp_gh.wait()
    for k1 in range(16):
        P = lax.dot_general(g_v[k1], Y[k1], NT_DIMS, preferred_element_type=f32)
        wr32 = jnp.concatenate([Wtr[pl.ds(A * WP + k1, 8, stride=17), :] for A in range(16)], axis=0)
        wi32 = jnp.concatenate([Wti[pl.ds(A * WP + k1, 8, stride=17), :] for A in range(16)], axis=0)
        parts = []
        for p in range(2):
            c0 = p * 256
            xr = P[0:128, c0:c0 + 128] - P[128:256, c0 + 128:c0 + 256]
            xi = P[128:256, c0:c0 + 128] + P[0:128, c0 + 128:c0 + 256]
            if p == 0:
                wr = lax.bitcast_convert_type(lax.shift_left(wr32, np.uint32(16)), f32)
                wi = lax.bitcast_convert_type(lax.shift_left(wi32, np.uint32(16)), f32)
            else:
                wr = lax.bitcast_convert_type(wr32 & np.uint32(0xFFFF0000), f32)
                wi = lax.bitcast_convert_type(wi32 & np.uint32(0xFFFF0000), f32)
            parts.append((xr * wr - xi * wi).astype(bf16))
            parts.append((xr * wi + xi * wr).astype(bf16))
        X3 = jnp.concatenate(parts, axis=1)
        Q = jnp.dot(gh_v[k1], X3, preferred_element_type=f32)
        for p in range(2):
            c0 = p * 256
            Vb[k1, 2 * p] = Q[0:128, c0:c0 + 128] + Q[128:256, c0 + 128:c0 + 256]
            Vb[k1, 2 * p + 1] = Q[0:128, c0 + 128:c0 + 256] - Q[128:256, c0:c0 + 128]

    for p in range(2):
        for r in range(0, 128, 16):
            re = [Vb[k1, 2 * p, r:r + 16, :] for k1 in range(16)]
            im = [Vb[k1, 2 * p + 1, r:r + 16, :] for k1 in range(16)]
            ore, oim = _fft16(re, im, +1)
            for s1 in range(16):
                Z[s1, p, r:r + 16, 0:128] = ore[s1].astype(bf16)
                Z[s1, p, r:r + 16, 128:256] = oim[s1].astype(bf16)

    cp_bd.wait()
    cp_wg.wait()
    cp_wu.wait()
    cp_wd.wait()
    TPC = 2
    ocp = []
    for c in range(NT // TPC):
        hs, hns = [], []
        for t in range(TPC):
            a = c * TPC + t
            E = lax.dot_general(bd_v[0], Z[a, 0], NT_DIMS, preferred_element_type=f32)
            O = lax.dot_general(bd_v[1], Z[a, 1], NT_DIMS, preferred_element_type=f32)
            y = jnp.concatenate([E + O, E - O], axis=0).astype(bf16)
            h = (x_v[:, a * 128:(a + 1) * 128].astype(f32) + y.astype(f32)).astype(bf16)
            hs.append(h)
            hns.append(_ln_T(h.astype(f32)).astype(bf16).T)
        hn = jnp.concatenate(hns, axis=0)
        h = jnp.concatenate(hs, axis=1)
        g = jnp.dot(hn, wg_v[...], preferred_element_type=f32)
        u = jnp.dot(hn, wu_v[...], preferred_element_type=f32)
        hh = (g * u).astype(bf16)
        mlp = lax.dot_general(wd_v[...], hh, NT_DIMS, preferred_element_type=f32)
        w0 = c * TPC * 128
        out_v[:, w0:w0 + TPC * 128] = (h.astype(f32) + mlp.astype(bf16).astype(f32)).astype(bf16)
        cp = pltpu.make_async_copy(out_v.at[:, pl.ds(w0, TPC * 128)], out_hbm.at[:, pl.ds(w0, TPC * 128)],
                                   osems.at[c])
        cp.start()
        ocp.append(cp)
    for cp in ocp:
        cp.wait()


@jax.jit
def pallas_sequential_preLN__spectral_gfnet__glu_gated_bilinear__prompt_kernel(
    A_x: jax.Array,
    A_w_r: jax.Array,
    A_w_i: jax.Array,
    B_x: jax.Array,
    B_w_gate: jax.Array,
    B_w_up: jax.Array,
    B_w_down: jax.Array,
):
    del B_x
    fd, G, GH, bd = _make_consts()
    xT = A_x.reshape(S, D).T
    any_spec = pl.BlockSpec(memory_space=pl.ANY)
    outT = pl.pallas_call(
        _kernel,
        out_shape=jax.ShapeDtypeStruct((D, S), bf16),
        in_specs=[any_spec] * 10,
        out_specs=any_spec,
        scratch_shapes=[
            pltpu.VMEM((D, S), bf16),
            pltpu.VMEM((DH + 1, S), bf16),
            pltpu.VMEM((DH + 1, S), bf16),
            pltpu.VMEM((D, F), bf16),
            pltpu.VMEM((D, F), bf16),
            pltpu.VMEM((D, F), bf16),
            pltpu.VMEM((2, 256, 256), bf16),
            pltpu.VMEM((16, 256, 128), bf16),
            pltpu.VMEM((16, 256, 128), bf16),
            pltpu.VMEM((2, DH, 256), bf16),
            pltpu.VMEM((16, 512, 128), f32),
            pltpu.VMEM((16, 512, 128), bf16),
            pltpu.VMEM((16 * WP, 128), u32),
            pltpu.VMEM((16 * WP, 128), u32),
            pltpu.VMEM((16, 4, 128, 128), f32),
            pltpu.VMEM((16, 2, 128, 256), bf16),
            pltpu.VMEM((D, S), bf16),
            pltpu.SemaphoreType.DMA((13,)),
            pltpu.SemaphoreType.DMA((8,)),
        ],
        compiler_params=pltpu.CompilerParams(vmem_limit_bytes=100 * 2**20),
        name="gfnet_glu",
    )(xT, A_w_r.T, A_w_i.T, B_w_gate, B_w_up, B_w_down.T, fd, G, GH, bd)
    return outT.T.reshape(1, S, D)
```

```python
import numpy as np
import jax
import jax.numpy as jnp
from jax import lax
from jax.experimental import pallas as pl
from jax.experimental.pallas import tpu as pltpu

S, D, F = 2048, 448, 1792
DH = D // 2
NT = S // 128
EPS = 1e-5
bf16 = jnp.bfloat16
f32 = jnp.float32
u32 = jnp.uint32
NT_DIMS = (((1,), (1,)), ((), ()))
TN_DIMS = (((0,), (0,)), ((), ()))
WP = 136

CFG = dict(xchunks=(4, 4, 4, 4), ndefer=8, re_per=2, ro_per=1, ge_per=2, go_per=2, pro_at=10, tpc=2, nmlp=8,
           groups=[["EOE", "EOO", "EOD", "YE", "YO"], ["X2O", "ZE", "ZO"]], static=[], ln_first=0,
           re_at=0, ro_at=0, ge_at=0, go_at=0)
CFG.update(OPQ)
BUFS = dict(EOE=NT * 128, EOO=NT * 128, EOD=NT * 128, X1E=4096, X1O=4096, YE=4096, YO=4096, X2E=4096, X2O=4096,
            VE=4096, VO=4096, ZE=4096, ZO=4096, HE=NT * DH)


def _layout():
    groups = [list(g) for g in CFG["groups"]]
    used = {b for g in groups for b in g}
    groups += [[b] for b in BUFS if b not in used]
    loc, sizes = {}, []
    for gi, g in enumerate(groups):
        off = 0
        for b in g:
            loc[b] = (gi, off)
            off += BUFS[b]
        sizes.append(off)
    return groups, loc, sizes


def _pack_u32(a):
    b = np.asarray(a, np.float32).astype(bf16).view(np.uint16).astype(np.uint32)
    return b[..., 0::2, :] | (b[..., 1::2, :] << np.uint32(16))


_PI = np.array([16 * (q // 16) + 2 * (q % 8) + ((q % 16) // 8) for q in range(256)])


def _make_consts():
    d = np.arange(DH)[None, :].astype(np.float64)
    m = np.arange(128)[:, None].astype(np.float64)
    angE = 2 * np.pi * (2 * m) * d / D
    angO = 2 * np.pi * (2 * m + 1) * d / D
    vE = (m <= 112)
    vO = (m <= 111)
    FeT = np.concatenate([np.where(vE, np.cos(angE), 0), np.where(vE, -np.sin(angE), 0)], 0)
    FoT = np.concatenate([np.where(vO, np.cos(angO), 0), np.where(vO, -np.sin(angO), 0)], 0)
    fd = np.stack([np.pad(FeT, ((0, 0), (0, 32))), np.pad(FoT, ((0, 0), (0, 32)))])
    fdp = np.zeros_like(fd)
    fdp[:, :, _PI] = fd
    fd = fdp.reshape(2, 256, 2, 128).transpose(0, 2, 1, 3)
    k2 = np.arange(128)[:, None]
    s2 = np.arange(128)[None, :]
    G = np.zeros((9, 256, 128))
    GT = np.zeros((9, 256, 128))
    ilv = lambda a, b: np.stack([a.reshape(8, 16, 128), b.reshape(8, 16, 128)], 1).reshape(256, 128)
    for k1 in range(9):
        ang = 2 * np.pi * ((s2 * (k1 + 16 * k2)) % S) / S
        Gr, Gi = np.cos(ang), -np.sin(ang)
        G[k1] = ilv(Gr, Gi)
        GT[k1] = ilv(Gr.T, Gi.T)
    dd = np.arange(DH)[:, None].astype(np.float64)
    mm = np.arange(128)[None, :].astype(np.float64)
    cE = np.where((mm == 0) | (mm == 112), 1.0, 2.0) * (mm <= 112)
    cO = 2.0 * (mm <= 111)
    sc = 1.0 / (D * S)
    aE = 2 * np.pi * (2 * mm) * dd / D
    aO = 2 * np.pi * (2 * mm + 1) * dd / D
    bd = np.stack([np.stack([cE * np.cos(aE), -cE * np.sin(aE)]), np.stack([cO * np.cos(aO), -cO * np.sin(aO)])]) * sc
    return _pack_u32(fd), _pack_u32(G), _pack_u32(GT), _pack_u32(bd)


class V:
    __slots__ = ("a", "n")

    def __init__(self, a, n=False):
        self.a, self.n = a, n

    def __neg__(self):
        return V(self.a, not self.n)

    def __add__(self, o):
        if not self.n and not o.n:
            return V(self.a + o.a)
        if not self.n and o.n:
            return V(self.a - o.a)
        if self.n and not o.n:
            return V(o.a - self.a)
        return V(self.a + o.a, True)

    def __sub__(self, o):
        return self + (-o)

    def mul(self, c):
        return V(self.a * np.float32(-c if self.n else c))

    def val(self):
        return -self.a if self.n else self.a


def _r4(x, sg):
    (x0r, x0i), (x1r, x1i), (x2r, x2i), (x3r, x3i) = x
    t0r, t0i = x0r + x2r, x0i + x2i
    t1r, t1i = x0r - x2r, x0i - x2i
    t2r, t2i = x1r + x3r, x1i + x3i
    t3r, t3i = x1r - x3r, x1i - x3i
    if sg > 0:
        ur, ui = -t3i, t3r
    else:
        ur, ui = t3i, -t3r
    return [(t0r + t2r, t0i + t2i), (t1r + ur, t1i + ui), (t0r - t2r, t0i - t2i), (t1r - ur, t1i - ui)]


def _tw(x, e, sg):
    xr, xi = x
    e = e % 16
    if e % 4 == 0:
        q = ((e // 4) if sg > 0 else (-(e // 4))) % 4
        if q == 0:
            return xr, xi
        if q == 1:
            return -xi, xr
        if q == 2:
            return -xr, -xi
        return xi, -xr
    c, s = np.cos(2 * np.pi * e / 16), sg * np.sin(2 * np.pi * e / 16)
    if e % 2 == 0:
        h = abs(c)
        a = xr if c > 0 else -xr
        b = xi if s > 0 else -xi
        re = (a - b).mul(h)
        a = xi if c > 0 else -xi
        b = xr if s > 0 else -xr
        im = (a + b).mul(h)
        return re, im
    return xr.mul(c) - xi.mul(s), xi.mul(c) + xr.mul(s)


def _fft16(re, im, sg):
    x = [(V(re[a]), V(im[a])) for a in range(16)]
    T = [_r4([x[4 * a1 + a0] for a1 in range(4)], sg) for a0 in range(4)]
    out_re, out_im = [None] * 16, [None] * 16
    for k0 in range(4):
        col = [_tw(T[a0][k0], a0 * k0, sg) for a0 in range(4)]
        y = _r4(col, sg)
        for k1 in range(4):
            out_re[k0 + 4 * k1] = y[k1][0].val()
            out_im[k0 + 4 * k1] = y[k1][1].val()
    return out_re, out_im


def _colsum(x):
    parts = [x[i:i + 8] for i in range(0, x.shape[0], 8)]
    while len(parts) > 1:
        nxt = [parts[i] + parts[i + 1] for i in range(0, len(parts) - 1, 2)]
        if len(parts) % 2:
            nxt.append(parts[-1])
        parts = nxt
    return jnp.sum(parts[0], axis=0, keepdims=True)


def _deilv16(x):
    a = jnp.concatenate([x[32 * j:32 * j + 16] for j in range(8)], axis=0)
    b = jnp.concatenate([x[32 * j + 16:32 * j + 32] for j in range(8)], axis=0)
    return a, b


def _pack16(x):
    return pltpu.pack_elementwise([x[0:8], x[8:16]], packed_dtype=bf16)


def _bf(x):
    return pltpu.bitcast(x, bf16)


class Arena:
    def __init__(self, ref, zs, zl, static=False):
        n = ref.shape[0]
        self.sv = ref if static else ref.at[pl.ds(zs, n)]
        self.lv = ref if static else ref.at[pl.ds(zl, n)]


class Buf:
    def __init__(self, arena, off):
        self.a, self.off = arena, off

    def st(self, row, val):
        if val.dtype != u32:
            val = lax.bitcast_convert_type(val, u32)
        row += self.off
        self.a.sv[row:row + val.shape[0], :] = val

    def ld(self, row, n, dtype=f32):
        row += self.off
        v = self.a.lv[row:row + n, :]
        return v if dtype == u32 else lax.bitcast_convert_type(v, dtype)


def _kernel(x_hbm, wr_hbm, wi_hbm, wg_hbm, wu_hbm, wd_hbm, fd_hbm, g_hbm, gt_hbm, bd_hbm, z_hbm,
            out_hbm,
            x_v, wr_v, wi_v, wg_v, wu_v, wd_v, fd_v, g_v, gt_v, bd_v, z_v,
            Wtr, Wti, out_v, sems, osems, *arenas):
    cfg = CFG
    xch = cfg["xchunks"]
    xst = [sum(xch[:c]) for c in range(len(xch) + 1)]
    x_cp = [pltpu.make_async_copy(x_hbm.at[:, pl.ds(128 * xst[c], 128 * xch[c])],
                                  x_v.at[:, pl.ds(128 * xst[c], 128 * xch[c])], sems.at[c])
            for c in range(len(xch))]
    cp_fd = pltpu.make_async_copy(fd_hbm, fd_v, sems.at[4])
    cp_wr = pltpu.make_async_copy(wr_hbm, wr_v, sems.at[5])
    cp_wi = pltpu.make_async_copy(wi_hbm, wi_v, sems.at[6])
    cp_g = pltpu.make_async_copy(g_hbm, g_v, sems.at[7])
    cp_bd = pltpu.make_async_copy(bd_hbm, bd_v, sems.at[8])
    cp_wg = pltpu.make_async_copy(wg_hbm, wg_v, sems.at[9])
    cp_wu = pltpu.make_async_copy(wu_hbm, wu_v, sems.at[10])
    cp_wd = pltpu.make_async_copy(wd_hbm, wd_v, sems.at[11])
    cp_gt = pltpu.make_async_copy(gt_hbm, gt_v, sems.at[12])
    cp_z = pltpu.make_async_copy(z_hbm, z_v, sems.at[13])
    cp_z.start()
    x_cp[0].start()
    cp_fd.start()
    for c in range(1, len(xch)):
        x_cp[c].start()
    for cp in (cp_g, cp_wr, cp_wi, cp_gt, cp_bd, cp_wg, cp_wu, cp_wd):
        cp.start()

    cp_z.wait()
    x_cp[0].wait()
    cp_fd.wait()
    z1 = pl.multiple_of(jnp.max(z_v[0]), 8)
    z2 = pl.multiple_of(jnp.max(z_v[1]), 8)
    groups, loc, _ = _layout()
    ars = [Arena(r, z1, z2, static=all(b in cfg["static"] for b in g)) for r, g in zip(arenas, groups)]
    bufs = {b: Buf(ars[gi], off) for b, (gi, off) in loc.items()}
    nd = cfg["ndefer"]
    EO = lambda p, a: bufs["EOE"] if p == 0 else (bufs["EOD"] if a >= NT - nd else bufs["EOO"])
    X1 = [bufs["X1E"], bufs["X1O"]]
    Yb = [bufs["YE"], bufs["YO"]]
    X2 = [bufs["X2E"], bufs["X2O"]]
    Vb = [bufs["VE"], bufs["VO"]]
    Zb = [bufs["ZE"], bufs["ZO"]]
    HE = bufs["HE"]
    rstd = [None] * NT

    def ln1(a):
        x = x_v[:, a * 128:(a + 1) * 128].astype(f32)
        s, op, acc = [], [], [None, None]
        for j in range(DH // 16):
            xa, xb = x[16 * j:16 * j + 16], x[DH + 16 * j:DH + 16 * j + 16]
            d = xa - xb
            s.append(xa + xb)
            op.append(_pack16(d))
            acc[j % 2] = d * d if acc[j % 2] is None else acc[j % 2] + d * d
        m2 = _colsum(jnp.concatenate(s, axis=0)) * (2.0 / D)
        ep = []
        for j in range(DH // 16):
            t = s[j] - m2
            ep.append(_pack16(t))
            acc[j % 2] = acc[j % 2] + t * t
        v = _colsum(acc[0] + acc[1]) * (0.5 / D)
        rstd[a] = lax.rsqrt(v + EPS)
        EO(1, a).st(a * 128, jnp.concatenate(op, axis=0))
        EO(0, a).st(a * 128, jnp.concatenate(ep, axis=0))

    def dftd(p, a):
        lhs = jnp.concatenate([_bf(fd_v[p, 0]), _bf(fd_v[p, 1])], axis=1)
        rhs = jnp.concatenate([EO(p, a).ld(a * 128, 112, u32), jnp.zeros((16, 128), u32)], axis=0)
        X1[p].st(a * 256, jnp.dot(lhs, _bf(rhs), preferred_element_type=f32) * rstd[a])

    def rad_fwd(p, j):
        r = 8 * j
        re = [X1[p].ld(a * 256 + r, 8) for a in range(16)]
        im = [X1[p].ld(a * 256 + 128 + r, 8) for a in range(16)]
        ore, oim = _fft16(re, im, -1)
        for k1 in range(16):
            Yb[p].st(k1 * 256 + r, ore[k1])
            Yb[p].st(k1 * 256 + 128 + r, oim[k1])

    def y_get(p, k1):
        if p == 1:
            z = jnp.zeros((16, 128), f32)
            y = jnp.concatenate([Yb[1].ld(k1 * 256, 112), z, Yb[1].ld(k1 * 256 + 128, 112), z], axis=0)
        else:
            y = Yb[0].ld(k1 * 256, 256)
        return y.astype(bf16)

    def gmat(k1):
        return (k1, 1) if k1 < 8 else (16 - k1, -1)

    def x2row(p, k1):
        return k1 * 256

    def dft128(p, k1):
        km, sg = gmat(k1)
        P = lax.dot_general(_bf(g_v[km]), y_get(p, k1), NT_DIMS, preferred_element_type=f32)
        Pr, Pi = _deilv16(P)
        if sg > 0:
            xr, xi = Pr[:, :128] - Pi[:, 128:], Pi[:, :128] + Pr[:, 128:]
        else:
            xr, xi = Pr[:, :128] + Pi[:, 128:], Pr[:, 128:] - Pi[:, :128]
        X2[p].st(x2row(p, k1), xr)
        X2[p].st(x2row(p, k1) + 128, xi)

    rows8 = lax.broadcasted_iota(jnp.int32, (8, 128), 0)

    def wprep(w_v, Wt, a):
        w32 = pltpu.bitcast(w_v[0:DH, a * 128:(a + 1) * 128], u32)
        ny = w_v[DH:DH + 1, a * 128:(a + 1) * 128].astype(f32)
        ny = jnp.broadcast_to(ny, (8, 128))
        nyu = lax.shift_right_logical(lax.bitcast_convert_type(ny, u32), np.uint32(16))
        nyu = jnp.where(rows8 == 0, nyu, np.uint32(0))
        t = jnp.concatenate([w32, nyu, jnp.zeros((8, 128), u32)], axis=0).T
        for j in range(8):
            Wt[pl.ds(a * WP + 17 * j, 8), :] = t[16 * j:16 * j + 8, :]
            Wt[pl.ds((15 - a) * WP + 17 * (7 - j) + 8, 8), :] = t[16 * j + 8:16 * j + 16, :]

    def idft128(p, k1):
        km, sg = gmat(k1)
        wr32 = jnp.concatenate([Wtr[pl.ds(A_ * WP + k1, 8, stride=17), :] for A_ in range(16)], axis=0)
        wi32 = jnp.concatenate([Wti[pl.ds(A_ * WP + k1, 8, stride=17), :] for A_ in range(16)], axis=0)
        if p == 0:
            wr = lax.bitcast_convert_type(lax.shift_left(wr32, np.uint32(16)), f32)
            wi = lax.bitcast_convert_type(lax.shift_left(wi32, np.uint32(16)), f32)
        else:
            wr = lax.bitcast_convert_type(wr32 & np.uint32(0xFFFF0000), f32)
            wi = lax.bitcast_convert_type(wi32 & np.uint32(0xFFFF0000), f32)
        xr, xi = X2[p].ld(x2row(p, k1), 128), X2[p].ld(x2row(p, k1) + 128, 128)
        x3 = jnp.concatenate([xr * wr - xi * wi, xr * wi + xi * wr], axis=1).astype(bf16)
        Q = jnp.dot(_bf(gt_v[km]), x3, preferred_element_type=f32)
        Qr, Qi = _deilv16(Q)
        if sg > 0:
            vr, vi = Qr[:, :128] + Qi[:, 128:], Qr[:, 128:] - Qi[:, :128]
        else:
            vr, vi = Qr[:, :128] - Qi[:, 128:], Qr[:, 128:] + Qi[:, :128]
        Vb[p].st(k1 * 256, vr)
        Vb[p].st(k1 * 256 + 128, vi)

    def rad_inv(p, j):
        r = 8 * j
        re = [Vb[p].ld(k1 * 256 + r, 8) for k1 in range(16)]
        im = [Vb[p].ld(k1 * 256 + 128 + r, 8) for k1 in range(16)]
        ore, oim = _fft16(re, im, +1)
        for s1 in range(16):
            Zb[p].st(s1 * 256 + r, ore[s1])
            Zb[p].st(s1 * 256 + 128 + r, oim[s1])

    def idftd(p, a):
        z = jnp.concatenate([Zb[p].ld(a * 256, 128), Zb[p].ld(a * 256 + 128, 128)], axis=1).astype(bf16)
        lhs = jnp.concatenate([_bf(bd_v[p, 0]), _bf(bd_v[p, 1])], axis=1)
        return lax.dot_general(lhs, z, NT_DIMS, preferred_element_type=f32)

    TPC = cfg["tpc"]
    ocp = []

    def prologue(c):
        hs, hns = [], []
        for t in range(TPC):
            a = c * TPC + t
            O = idftd(1, a)
            E = HE.ld(a * DH, DH)
            y = jnp.concatenate([E + O, E - O], axis=0)
            hf = (x_v[:, a * 128:(a + 1) * 128].astype(f32) + y).astype(bf16).astype(f32)
            m = _colsum(hf) * (1.0 / D)
            hc = hf - m
            v = _colsum(hc * hc) * (1.0 / D)
            hs.append(hf)
            hns.append(hc * lax.rsqrt(v + EPS))
        return jnp.concatenate(hs, axis=1), jnp.concatenate(hns, axis=1).astype(bf16)

    def mlp(c, h, hnT):
        g = lax.dot_general(hnT, wg_v[...], TN_DIMS, preferred_element_type=f32)
        u = lax.dot_general(hnT, wu_v[...], TN_DIMS, preferred_element_type=f32)
        hh = (g * u).astype(bf16)
        if c == 0:
            cp_wd.wait()
        mlp = lax.dot_general(wd_v[...], hh, NT_DIMS, preferred_element_type=f32)
        w0 = c * TPC * 128
        out_v[:, w0:w0 + TPC * 128] = (h + mlp.astype(bf16).astype(f32)).astype(bf16)
        cp = pltpu.make_async_copy(out_v.at[:, pl.ds(w0, TPC * 128)], out_hbm.at[:, pl.ds(w0, TPC * 128)],
                                   osems.at[c])
        cp.start()
        ocp.append(cp)

    def fwd_tile(a):
        dftd(0, a)
        if a < NT - nd:
            dftd(1, a)

    ln1(0)
    for a in range(1, NT):
        if a in xst:
            x_cp[xst.index(a)].wait()
        if cfg["ln_first"]:
            ln1(a)
            fwd_tile(a - 1)
        else:
            fwd_tile(a - 1)
            ln1(a)
    fwd_tile(NT - 1)
    j = 0
    for a in range(NT - nd, NT):
        dftd(1, a)
        for _ in range(cfg["re_per"] if a - (NT - nd) >= cfg["re_at"] else 0):
            if j < 16:
                rad_fwd(0, j)
                j += 1
    while j < 16:
        rad_fwd(0, j)
        j += 1
    cp_g.wait()
    j = 0
    for k1 in range(16):
        dft128(0, k1)
        for _ in range(cfg["ro_per"] if k1 >= cfg["ro_at"] else 0):
            if j < 14:
                rad_fwd(1, j)
                j += 1
    while j < 14:
        rad_fwd(1, j)
        j += 1
    cp_wr.wait()
    for k1 in range(8):
        dft128(1, k1)
        wprep(wr_v, Wtr, 2 * k1)
        wprep(wr_v, Wtr, 2 * k1 + 1)
    cp_wi.wait()
    for k1 in range(8, 16):
        dft128(1, k1)
        wprep(wi_v, Wti, 2 * (k1 - 8))
        wprep(wi_v, Wti, 2 * (k1 - 8) + 1)
    cp_gt.wait()
    for k1 in range(16):
        idft128(0, k1)
    j = 0
    for k1 in range(16):
        idft128(1, k1)
        for _ in range(cfg["ge_per"] if k1 >= cfg["ge_at"] else 0):
            if j < 16:
                rad_inv(0, j)
                j += 1
    while j < 16:
        rad_inv(0, j)
        j += 1
    cp_bd.wait()
    j = 0
    nxt = None
    for a in range(16):
        if a == cfg["pro_at"]:
            while j < 16:
                rad_inv(1, j)
                j += 1
            nxt = prologue(0)
        HE.st(a * DH, idftd(0, a))
        for _ in range(cfg["go_per"] if a >= cfg["go_at"] else 0):
            if j < 16:
                rad_inv(1, j)
                j += 1
    if nxt is None:
        while j < 16:
            rad_inv(1, j)
            j += 1
        nxt = prologue(0)
    NC = cfg["nmlp"]
    cp_wg.wait()
    cp_wu.wait()
    for c in range(NC):
        cur = nxt
        if c + 1 < NC:
            nxt = prologue(c + 1)
        mlp(c, *cur)
    for cp in ocp:
        cp.wait()


@jax.jit
def pallas_sequential_preLN__spectral_gfnet__glu_gated_bilinear__prompt_kernel(
    A_x: jax.Array,
    A_w_r: jax.Array,
    A_w_i: jax.Array,
    B_x: jax.Array,
    B_w_gate: jax.Array,
    B_w_up: jax.Array,
    B_w_down: jax.Array,
):
    del B_x
    fd, G, GT, bd = _make_consts()
    xT = A_x.reshape(S, D).T
    any_spec = pl.BlockSpec(memory_space=pl.ANY)
    outT = pl.pallas_call(
        _kernel,
        out_shape=jax.ShapeDtypeStruct((D, S), bf16),
        in_specs=[any_spec] * 11,
        out_specs=any_spec,
        scratch_shapes=[
            pltpu.VMEM((D, S), bf16),
            pltpu.VMEM((DH + 1, S), bf16),
            pltpu.VMEM((DH + 1, S), bf16),
            pltpu.VMEM((D, F), bf16),
            pltpu.VMEM((D, F), bf16),
            pltpu.VMEM((D, F), bf16),
            pltpu.VMEM((2, 2, 128, 128), u32),
            pltpu.VMEM((9, 128, 128), u32),
            pltpu.VMEM((9, 128, 128), u32),
            pltpu.VMEM((2, 2, DH // 2, 128), u32),
            pltpu.VMEM((2, 8, 128), jnp.int32),
            pltpu.VMEM((16 * WP, 128), u32),
            pltpu.VMEM((16 * WP, 128), u32),
            pltpu.VMEM((D, S), bf16),
            pltpu.SemaphoreType.DMA((14,)),
            pltpu.SemaphoreType.DMA((8,)),
        ] + [pltpu.VMEM((n, 128), u32) for n in _layout()[2]],
        compiler_params=pltpu.CompilerParams(vmem_limit_bytes=100 * 2**20),
        name="gfnet_glu",
    )(xT, A_w_r.T, A_w_i.T, B_w_gate, B_w_up, B_w_down.T, fd, G, GT, bd, np.zeros((2, 8, 128), np.int32))
    return outT.T.reshape(1, S, D)
```

```python
import numpy as np
import jax
import jax.numpy as jnp
from jax import lax
from jax.experimental import pallas as pl
from jax.experimental.pallas import tpu as pltpu

S, D, F = 2048, 448, 1792
DH = D // 2
NT = S // 128
EPS = 1e-5
bf16 = jnp.bfloat16
f32 = jnp.float32
u32 = jnp.uint32
NT_DIMS = (((1,), (1,)), ((), ()))
TN_DIMS = (((0,), (0,)), ((), ()))
WP = 136

CFG = dict(xchunks=(4, 4, 4, 4), ro_per=1, ge_per=2, go_per=1, pro_at=16, tpc=2, nmlp=8,
           groups=[["YE", "YO"], ["ZE", "ZO"]], static=["EOE", "EOO"], ln_first=0,
           order=["g", "wr", "wi", "bd", "wg", "wu", "wd"], re_at=0, ro_at=0, ge_at=0, go_at=0, fd_late=0, m_c=16, gec_per=2, gec_max=16, mlp_loop=0, pre_t=0, down_split=0, loop_ssa=1, mlp_unroll=1, mlp_peel=2, mlp_mem=0, wd_early=0, wr_at=16, wi_at=8, bd_early=0, wgwu_at=16)
CFG.update(OPQ)
BUFS = dict(EOE=NT * 128, EOO=NT * 128, X1E=4096, X1O=4096, YE=4096, YO=4096, X2E=4096, X2O=4096,
            VE=4096, VO=4096, ZE=4096, ZO=4096, HE=NT * DH)


TRACE = []


def _layout():
    groups = [list(g) for g in CFG["groups"]]
    used = {b for g in groups for b in g}
    groups += [[b] for b in BUFS if b not in used]
    loc, sizes = {}, []
    for gi, g in enumerate(groups):
        off = 0
        for b in g:
            loc[b] = (gi, off)
            off += BUFS[b]
        sizes.append(off)
    return groups, loc, sizes


def _pack_u32(a):
    b = np.asarray(a, np.float32).astype(bf16).view(np.uint16).astype(np.uint32)
    return b[..., 0::2, :] | (b[..., 1::2, :] << np.uint32(16))


_PI = np.array([16 * (q // 16) + 2 * (q % 8) + ((q % 16) // 8) for q in range(256)])


DQ = D // 4
FD_ROWS = 56 + 56 + 2 * 112 + 16


def _make_consts():
    dq = np.arange(DQ)[None, :].astype(np.float64)
    j = np.arange(56)[:, None].astype(np.float64)
    a0 = 2 * np.pi * (4 * j) * dq / D
    f0 = np.concatenate([np.cos(a0), -np.sin(a0)], 0)
    f0[56] = np.cos(np.pi * dq[0])
    a2 = 2 * np.pi * (4 * j + 2) * dq / D
    f2 = np.concatenate([np.cos(a2), -np.sin(a2)], 0)
    d = np.arange(DH)[None, :].astype(np.float64)
    m = np.arange(DQ)[:, None].astype(np.float64)
    ao = 2 * np.pi * (2 * m + 1) * d / D
    fo = np.concatenate([np.cos(ao), -np.sin(ao)], 0)

    def kperm(a, k):
        out = np.zeros((a.shape[0], k))
        out[:, _PI[:a.shape[1]]] = a
        return out

    f0, f2, fo = kperm(f0, 128), kperm(f2, 128), kperm(fo, 256)
    fd = np.concatenate([_pack_u32(f0), _pack_u32(f2), _pack_u32(fo[:, :128]), _pack_u32(fo[:, 128:]),
                         np.zeros((16, 128), np.uint32)], 0)
    k2 = np.arange(128)[:, None]
    s2 = np.arange(128)[None, :]
    G = np.zeros((9, 256, 128))
    for k1 in range(9):
        ang = 2 * np.pi * ((s2 * (k1 + 16 * k2)) % S) / S
        Gr, Gi = np.cos(ang), -np.sin(ang)
        G[k1, :128], G[k1, 128:] = Gr, Gi
    dd = np.arange(DH)[:, None].astype(np.float64)
    mm = np.arange(128)[None, :].astype(np.float64)
    cE = np.where((mm == 0) | (mm == 112), 1.0, 2.0) * (mm <= 112)
    cO = 2.0 * (mm <= 111)
    sc = 1.0 / (D * S)
    aE = 2 * np.pi * (2 * mm) * dd / D
    aO = 2 * np.pi * (2 * mm + 1) * dd / D
    bd = np.stack([np.stack([cE * np.cos(aE), -cE * np.sin(aE)]), np.stack([cO * np.cos(aO), -cO * np.sin(aO)])]) * sc
    return fd, _pack_u32(G), _pack_u32(bd)


class V:
    __slots__ = ("a", "n")

    def __init__(self, a, n=False):
        self.a, self.n = a, n

    def __neg__(self):
        return V(self.a, not self.n)

    def __add__(self, o):
        if o.a is None:
            return self
        if self.a is None:
            return o
        if not self.n and not o.n:
            return V(self.a + o.a)
        if not self.n and o.n:
            return V(self.a - o.a)
        if self.n and not o.n:
            return V(o.a - self.a)
        return V(self.a + o.a, True)

    def __sub__(self, o):
        return self + (-o)

    def mul(self, c):
        if self.a is None:
            return self
        return V(self.a * np.float32(-c if self.n else c))

    def val(self, like):
        if self.a is None:
            return jnp.zeros_like(like)
        return -self.a if self.n else self.a


def _r4(x, sg):
    (x0r, x0i), (x1r, x1i), (x2r, x2i), (x3r, x3i) = x
    t0r, t0i = x0r + x2r, x0i + x2i
    t1r, t1i = x0r - x2r, x0i - x2i
    t2r, t2i = x1r + x3r, x1i + x3i
    t3r, t3i = x1r - x3r, x1i - x3i
    if sg > 0:
        ur, ui = -t3i, t3r
    else:
        ur, ui = t3i, -t3r
    return [(t0r + t2r, t0i + t2i), (t1r + ur, t1i + ui), (t0r - t2r, t0i - t2i), (t1r - ur, t1i - ui)]


def _tw(x, e, sg):
    xr, xi = x
    e = e % 16
    if e % 4 == 0:
        q = ((e // 4) if sg > 0 else (-(e // 4))) % 4
        if q == 0:
            return xr, xi
        if q == 1:
            return -xi, xr
        if q == 2:
            return -xr, -xi
        return xi, -xr
    c, s = np.cos(2 * np.pi * e / 16), sg * np.sin(2 * np.pi * e / 16)
    if e % 2 == 0:
        h = abs(c)
        a = xr if c > 0 else -xr
        b = xi if s > 0 else -xi
        re = (a - b).mul(h)
        a = xi if c > 0 else -xi
        b = xr if s > 0 else -xr
        im = (a + b).mul(h)
        return re, im
    return xr.mul(c) - xi.mul(s), xi.mul(c) + xr.mul(s)


def _fft16(re, im, sg):
    x = [(V(re[a]), V(im[a])) for a in range(16)]
    T = [_r4([x[4 * a1 + a0] for a1 in range(4)], sg) for a0 in range(4)]
    out_re, out_im = [None] * 16, [None] * 16
    for k0 in range(4):
        col = [_tw(T[a0][k0], a0 * k0, sg) for a0 in range(4)]
        y = _r4(col, sg)
        for k1 in range(4):
            out_re[k0 + 4 * k1] = y[k1][0].val(re[0])
            out_im[k0 + 4 * k1] = y[k1][1].val(re[0])
    return out_re, out_im


def _colsum(x):
    parts = [x[i:i + 8] for i in range(0, x.shape[0], 8)]
    while len(parts) > 1:
        nxt = [parts[i] + parts[i + 1] for i in range(0, len(parts) - 1, 2)]
        if len(parts) % 2:
            nxt.append(parts[-1])
        parts = nxt
    return jnp.sum(parts[0], axis=0, keepdims=True)


def _deilv16(x):
    a = jnp.concatenate([x[32 * j:32 * j + 16] for j in range(8)], axis=0)
    b = jnp.concatenate([x[32 * j + 16:32 * j + 32] for j in range(8)], axis=0)
    return a, b


def _pack16(x):
    return pltpu.pack_elementwise([x[0:8], x[8:16]], packed_dtype=bf16)


def _lo(w):
    return lax.bitcast_convert_type(lax.shift_left(w, np.uint32(16)), f32)


def _hi(w):
    return lax.bitcast_convert_type(w & np.uint32(0xFFFF0000), f32)


def _bf(x):
    return pltpu.bitcast(x, bf16)


class Arena:
    def __init__(self, ref, static=False):
        self.ref, self.static = ref, static
        self.sv = self.lv = ref if static else None

    def bind(self, zs, zl):
        self.zs, self.zl = zs, zl
        if not self.static:
            n = self.ref.shape[0]
            self.sv = self.ref.at[pl.ds(zs, n)]
            self.lv = self.ref.at[pl.ds(zl, n)]


class Buf:
    def __init__(self, arena, off):
        self.a, self.off = arena, off

    def sub(self, c, n):
        if isinstance(c, int):
            return Buf(self.a, self.off + c * n)
        ar = Arena(self.a.ref)
        base = pl.multiple_of(self.off + c * n, 8)
        ar.sv = self.a.ref.at[pl.ds(self.a.zs + base, n)]
        ar.lv = self.a.ref.at[pl.ds(self.a.zl + base, n)]
        return Buf(ar, 0)

    def st(self, row, val):
        if val.dtype != u32:
            val = lax.bitcast_convert_type(val, u32)
        row += self.off
        self.a.sv[row:row + val.shape[0], :] = val

    def st_strided(self, row, val, stride):
        if val.dtype != u32:
            val = lax.bitcast_convert_type(val, u32)
        row += self.off
        self.a.sv[pl.ds(row, val.shape[0], stride=stride), :] = val

    def ld(self, row, n, dtype=f32):
        row += self.off
        v = self.a.lv[row:row + n, :]
        return v if dtype == u32 else lax.bitcast_convert_type(v, dtype)


def _kernel(x_hbm, wr_hbm, wi_hbm, wg_hbm, wu_hbm, wd_hbm, fd_hbm, g_hbm, bd_hbm,
            out_hbm,
            x_v, wr_v, wi_v, wg_v, wu_v, wd_v, fd_v, g_v, gs_v, bd_v,
            Wtr, Wti, out_v, hn_v, hn2_v, sems, osems, *arenas):
    cfg = CFG
    xch = cfg["xchunks"]
    xst = [sum(xch[:c]) for c in range(len(xch) + 1)]
    x_cp = [pltpu.make_async_copy(x_hbm.at[:, pl.ds(128 * xst[c], 128 * xch[c])],
                                  x_v.at[:, pl.ds(128 * xst[c], 128 * xch[c])], sems.at[c])
            for c in range(len(xch))]
    cp_fd = pltpu.make_async_copy(fd_hbm, fd_v, sems.at[4])
    cp_wr = pltpu.make_async_copy(wr_hbm, wr_v, sems.at[5])
    cp_wi = pltpu.make_async_copy(wi_hbm, wi_v, sems.at[6])
    cp_g = pltpu.make_async_copy(g_hbm, g_v, sems.at[7])
    cp_bd = pltpu.make_async_copy(bd_hbm, bd_v, sems.at[8])
    cp_wg = pltpu.make_async_copy(wg_hbm, wg_v, sems.at[9])
    cp_wu = pltpu.make_async_copy(wu_hbm, wu_v, sems.at[10])
    cp_wd = pltpu.make_async_copy(wd_hbm, wd_v, sems.at[11])
    cps = dict(fd=cp_fd, wr=cp_wr, wi=cp_wi, g=cp_g, bd=cp_bd, wg=cp_wg, wu=cp_wu, wd=cp_wd)
    for c in range(len(xch)):
        cps["x%d" % c] = x_cp[c]
    order = ["x0", "fd"] + ["x%d" % c for c in range(1, len(xch))] + cfg["order"]

    del TRACE[:]
    TRACE.append(("order", order, list(xch)))
    for n in order:
        cps[n].start()

    def wait(*names):
        TRACE.append(("wait", names))
        if cfg.get("scopes"):
            with jax.named_scope("wait_" + names[0]):
                for n in names:
                    cps[n].wait()
            return
        for n in names:
            cps[n].wait()

    if cfg["fd_late"]:
        wait("x0")
    else:
        wait("x0", "fd")
    groups, loc, _ = _layout()
    ars = [Arena(r, static=all(b in cfg["static"] for b in g)) for r, g in zip(arenas, groups)]
    bufs = {b: Buf(ars[gi], off) for b, (gi, off) in loc.items()}
    X1 = [bufs["X1E"], bufs["X1O"]]
    Yb = [bufs["YE"], bufs["YO"]]
    X2 = [bufs["X2E"], bufs["X2O"]]
    Vb = [bufs["VE"], bufs["VO"]]
    Zb = [bufs["ZE"], bufs["ZO"]]
    HE = bufs["HE"]

    def make_views():
        zz = lax.bitcast_convert_type(fd_v[FD_ROWS - 16:FD_ROWS, :], jnp.int32)
        z1 = pl.multiple_of(jnp.max(zz[0:8]), 8)
        z2 = pl.multiple_of(jnp.max(zz[8:16]), 8)
        for ar in ars:
            ar.bind(z1, z2)
    rstd = [None] * NT

    def ln1(a):
        if cfg.get("dbg_noln") and a < 15:
            return
        x = x_v[:, a * 128:(a + 1) * 128].astype(f32)
        a0, o_lo, o_hi, a2p = [], [], [], []
        accd, acca = [None, None], [None, None]

        def acc(l, i, v):
            l[i] = v if l[i] is None else l[i] + v

        for j in range(DQ // 16):
            x0, x1, x2, x3 = (x[q * DQ + 16 * j:q * DQ + 16 * j + 16] for q in range(4))
            s02, s13 = x0 + x2, x1 + x3
            d02, d13 = x0 - x2, x1 - x3
            a0.append(s02 + s13)
            a2 = s02 - s13
            o_lo.append(_pack16(d02))
            o_hi.append(_pack16(d13))
            a2p.append(_pack16(a2))
            acc(accd, 0, d02 * d02)
            acc(accd, 1, d13 * d13)
            acc(acca, 0, a2 * a2)
        m4 = _colsum(jnp.concatenate(a0, axis=0)) * (4.0 / D)
        a0p = []
        for j in range(DQ // 16):
            t = a0[j] - m4
            a0p.append(_pack16(t))
            acc(acca, 1, t * t)
        v = _colsum((accd[0] + accd[1]) * 2.0 + (acca[0] + acca[1])) * (0.25 / D)
        rstd[a] = lax.rsqrt(v + EPS)
        bufs["EOO"].st(a * 128, jnp.concatenate(o_lo + o_hi, axis=0))
        bufs["EOE"].st(a * 128, jnp.concatenate(a0p + a2p, axis=0))

    row0 = lax.broadcasted_iota(jnp.int32, (8, 128), 0) == 0

    def dftd_e(a, q):
        rhs = jnp.concatenate([bufs["EOE"].ld(a * 128 + 56 * q, 56, u32), jnp.zeros((8, 128), u32)], axis=0)
        r = jnp.dot(_bf(fd_v[56 * q:56 * q + 56, :]), _bf(rhs), preferred_element_type=f32) * rstd[a]
        for c in range(2):
            for v in range(7):
                t = r[56 * c + 8 * v:56 * c + 8 * v + 8]
                if q == 0 and c == 1 and v == 0:
                    X1[0].st(a * 256 + 112, jnp.where(row0, t, 0.0))
                    t = jnp.where(row0, 0.0, t)
                X1[0].st_strided(a * 256 + 128 * c + 16 * v + q, t, 2)

    def dftd_o(a):
        lhs = jnp.concatenate([_bf(fd_v[112:224, :]), _bf(fd_v[224:336, :])], axis=1)
        rhs = jnp.concatenate([bufs["EOO"].ld(a * 128, 112, u32), jnp.zeros((16, 128), u32)], axis=0)
        r = jnp.dot(lhs, _bf(rhs), preferred_element_type=f32) * rstd[a]
        X1[1].st(a * 256, r[:DQ])
        X1[1].st(a * 256 + 128, r[DQ:])

    def rad_fwd(p, j):
        r = 8 * j
        re = [X1[p].ld(a * 256 + r, 8) for a in range(16)]
        nyq = (p == 0 and j == 14)
        im = [None if nyq else X1[p].ld(a * 256 + 128 + r, 8) for a in range(16)]
        ore, oim = _fft16(re, im, -1)
        for k1 in range(16):
            Yb[p].st(k1 * 256 + r, ore[k1])
            Yb[p].st(k1 * 256 + 128 + r, oim[k1])

    def y_get(p, k1):
        n = 112 if p else 120
        z = jnp.zeros((128 - n, 128), f32)
        return (jnp.concatenate([Yb[p].ld(k1 * 256, n), z], axis=0),
                jnp.concatenate([Yb[p].ld(k1 * 256 + 128, n), z], axis=0))

    def gmat(k1):
        return (k1, 1) if k1 < 8 else (16 - k1, -1)

    def gsum(km):
        wr_, wi_ = g_v[km, 0:64, :], g_v[km, 64:128, :]
        lo = _lo(wr_) + _lo(wi_)
        hi = _hi(wr_) + _hi(wi_)
        gs_v[km] = pltpu.pack_elementwise([lo, hi], packed_dtype=bf16)

    def gparts(km):
        return _bf(g_v[km, 0:64, :]), _bf(g_v[km, 64:128, :]), _bf(gs_v[km])

    def cmul3(km, conj, a, b, dims):
        gr, gi, gs = gparts(km)
        t1 = lax.dot_general(gr, a.astype(bf16), dims, preferred_element_type=f32)
        t2 = lax.dot_general(gi, b.astype(bf16), dims, preferred_element_type=f32)
        if conj:
            t3 = lax.dot_general(gs, (b - a).astype(bf16), dims, preferred_element_type=f32)
            return t1 + t2, t3 + (t1 - t2)
        t3 = lax.dot_general(gs, (a + b).astype(bf16), dims, preferred_element_type=f32)
        return t1 - t2, t3 - (t1 + t2)

    def x2row(p, k1):
        return k1 * 256

    def dft128(p, k1):
        km, sg = gmat(k1)
        yr, yi = y_get(p, k1)
        xr, xi = cmul3(km, sg < 0, yr, yi, NT_DIMS)
        X2[p].st(x2row(p, k1), xr)
        X2[p].st(x2row(p, k1) + 128, xi)

    rows8 = lax.broadcasted_iota(jnp.int32, (8, 128), 0)

    def wprep(w_v, Wt, a):
        w32 = pltpu.bitcast(w_v[0:DH, a * 128:(a + 1) * 128], u32)
        ny = w_v[DH:DH + 1, a * 128:(a + 1) * 128].astype(f32)
        ny = jnp.broadcast_to(ny, (8, 128))
        nyu = lax.shift_right_logical(lax.bitcast_convert_type(ny, u32), np.uint32(16))
        nyu = jnp.where(rows8 == 0, nyu, np.uint32(0))
        t = jnp.concatenate([w32, nyu, jnp.zeros((8, 128), u32)], axis=0).T
        for j in range(8):
            Wt[pl.ds(a * WP + 17 * j, 8), :] = t[16 * j:16 * j + 8, :]
            Wt[pl.ds((15 - a) * WP + 17 * (7 - j) + 8, 8), :] = t[16 * j + 8:16 * j + 16, :]

    def idft128(p, k1):
        km, sg = gmat(k1)
        wr32 = jnp.concatenate([Wtr[pl.ds(A_ * WP + k1, 8, stride=17), :] for A_ in range(16)], axis=0)
        wi32 = jnp.concatenate([Wti[pl.ds(A_ * WP + k1, 8, stride=17), :] for A_ in range(16)], axis=0)
        if p == 0:
            wr, wi = _lo(wr32), _lo(wi32)
        else:
            wr, wi = _hi(wr32), _hi(wi32)
        xr, xi = X2[p].ld(x2row(p, k1), 128), X2[p].ld(x2row(p, k1) + 128, 128)
        vr, vi = cmul3(km, sg > 0, xr * wr - xi * wi, xr * wi + xi * wr, TN_DIMS)
        Vb[p].st(k1 * 256, vr)
        Vb[p].st(k1 * 256 + 128, vi)

    def rad_inv(p, j):
        r = 8 * j
        re = [Vb[p].ld(k1 * 256 + r, 8) for k1 in range(16)]
        im = [Vb[p].ld(k1 * 256 + 128 + r, 8) for k1 in range(16)]
        ore, oim = _fft16(re, im, +1)
        for s1 in range(16):
            Zb[p].st(s1 * 256 + r, ore[s1])
            Zb[p].st(s1 * 256 + 128 + r, oim[s1])

    def idftd2(p, zb, t):
        z = jnp.concatenate([zb.ld(t * 256, 128), zb.ld(t * 256 + 128, 128)], axis=1).astype(bf16)
        lhs = jnp.concatenate([_bf(bd_v[p, 0]), _bf(bd_v[p, 1])], axis=1)
        return lax.dot_general(lhs, z, NT_DIMS, preferred_element_type=f32)

    def idftd(p, a):
        return idftd2(p, Zb[p], a)

    TPC = 2
    CW = TPC * 128

    def cols(c, t=0, n=CW):
        if isinstance(c, int):
            return pl.ds(c * CW + t * 128, n)
        return pl.ds(pl.multiple_of(c * CW, CW) + t * 128, n)

    def prologue(c, mem):
        zo, he = Zb[1].sub(c, TPC * 256), HE.sub(c, TPC * DH)
        hs, hns = [], []
        for t in range(TPC):
            O = idftd2(1, zo, t)
            E = he.ld(t * DH, DH)
            y = jnp.concatenate([E + O, E - O], axis=0)
            hb = (x_v[:, cols(c, t, 128)].astype(f32) + y).astype(bf16)
            hf = hb.astype(f32)
            m = _colsum(hf) * (1.0 / D)
            hc = hf - m
            v = _colsum(hc * hc) * (1.0 / D)
            hs.append(hf)
            hns.append(hc * lax.rsqrt(v + EPS))
            if mem:
                out_v[:, cols(c, t, 128)] = hb
        hn = jnp.concatenate(hns, axis=1).astype(bf16)
        if cfg["pre_t"]:
            hn = hn.T
            if mem:
                hn2_v[rows(c), :] = hn
                return None
        if mem:
            hn_v[:, cols(c)] = hn
            return None
        return jnp.concatenate(hs, axis=1), hn

    def rows(c):
        if isinstance(c, int):
            return pl.ds(c * CW, CW)
        return pl.ds(pl.multiple_of(c * CW, CW), CW)

    def out_copy(c, t=None):
        if t is None:
            return pltpu.make_async_copy(out_v.at[:, cols(c)], out_hbm.at[:, cols(c)], osems.at[2 * c])
        return pltpu.make_async_copy(out_v.at[:, cols(c, t, 128)], out_hbm.at[:, cols(c, t, 128)], osems.at[2 * c + t])

    def mlp(c, cur, nxt_fn=None, wd_wait=False):
        if cfg["pre_t"]:
            hn = hn2_v[rows(c), :] if cur is None else cur[1]
            nxt = nxt_fn() if nxt_fn is not None else None
            g = jnp.dot(hn, wg_v[...], preferred_element_type=f32)
            u = jnp.dot(hn, wu_v[...], preferred_element_type=f32)
        else:
            hnT = hn_v[:, cols(c)] if cur is None else cur[1]
            nxt = nxt_fn() if nxt_fn is not None else None
            g = lax.dot_general(hnT, wg_v[...], TN_DIMS, preferred_element_type=f32)
            u = lax.dot_general(hnT, wu_v[...], TN_DIMS, preferred_element_type=f32)
        hh = (g * u).astype(bf16)
        if wd_wait is True:
            wait("wd")
        elif wd_wait is not False:
            @pl.when(wd_wait)
            def _():
                wait("wd")
        if cfg["down_split"]:
            for t in range(TPC):
                mlp = lax.dot_general(wd_v[...], hh[t * 128:(t + 1) * 128], NT_DIMS, preferred_element_type=f32)
                h = out_v[:, cols(c, t, 128)].astype(f32) if cur is None else cur[0][:, t * 128:(t + 1) * 128]
                out_v[:, cols(c, t, 128)] = (h + mlp.astype(bf16).astype(f32)).astype(bf16)
                if cfg["down_split"] == 2:
                    out_copy(c, t).start()
            if cfg["down_split"] == 1:
                out_copy(c).start()
            return nxt
        mlp = lax.dot_general(wd_v[...], hh, NT_DIMS, preferred_element_type=f32)
        h = out_v[:, cols(c)].astype(f32) if cur is None else cur[0]
        out_v[:, cols(c)] = (h + mlp.astype(bf16).astype(f32)).astype(bf16)
        out_copy(c).start()
        return nxt

    def fwd_tile(a):
        if cfg.get("dbg_nofwd") and a < 15:
            return
        if a % 2 == 0:
            dftd_e(a, 0)
            dftd_e(a, 1)
            dftd_o(a)
        else:
            dftd_o(a)
            dftd_e(a, 0)
            dftd_e(a, 1)

    if not cfg["fd_late"]:
        make_views()
    ln1(0)
    if cfg["fd_late"]:
        wait("fd")
        make_views()
    for a in range(1, NT):
        if a in xst:
            wait("x%d" % xst.index(a))
        if cfg["ln_first"]:
            ln1(a)
            fwd_tile(a - 1)
        else:
            fwd_tile(a - 1)
            ln1(a)
    fwd_tile(NT - 1)
    if cfg.get("dbg_stop") == 1:
        for n in order:
            if not (n[0] == "x" or n == "fd"):
                wait(n)
        out_v[0:8, 0:128] = X1[0].ld(15 * 256, 8).astype(bf16) + X1[1].ld(15 * 256, 8).astype(bf16)
        cp = pltpu.make_async_copy(out_v.at[:, pl.ds(0, 128)], out_hbm.at[:, pl.ds(0, 128)], osems.at[0])
        cp.start()
        cp.wait()
        return
    for j in range(15):
        rad_fwd(0, j)
    wait("g")
    for km in range(9):
        gsum(km)
    j = 0
    for k1 in range(16):
        if k1 == cfg["wr_at"]:
            wait("wr")
        dft128(0, k1)
        for _ in range(cfg["ro_per"] if k1 >= cfg["ro_at"] else 0):
            if j < 14:
                rad_fwd(1, j)
                j += 1
        if k1 >= cfg["wr_at"]:
            n = 16 - cfg["wr_at"]
            for a in range(16 * (k1 - cfg["wr_at"]) // n, 16 * (k1 - cfg["wr_at"] + 1) // n):
                wprep(wr_v, Wtr, a)
    while j < 14:
        rad_fwd(1, j)
        j += 1
    mc = cfg["m_c"]
    if cfg["wr_at"] >= 16:
        wait("wr")
        for k1 in range(cfg["wi_at"]):
            dft128(1, k1)
            n = cfg["wi_at"]
            for a in range(16 * k1 // n, 16 * (k1 + 1) // n):
                wprep(wr_v, Wtr, a)
    else:
        for k1 in range(cfg["wi_at"]):
            dft128(1, k1)
    if cfg["bd_early"] == 2:
        wait("wi", "bd")
    else:
        wait("wi")
    for k1 in range(cfg["wi_at"], mc):
        dft128(1, k1)
        n = mc - cfg["wi_at"]
        for a in range(16 * (k1 - cfg["wi_at"]) // n, 16 * (k1 - cfg["wi_at"] + 1) // n):
            wprep(wi_v, Wti, a)
    if cfg["bd_early"] == 1:
        wait("bd")
    for k1 in range(16):
        idft128(0, k1)
    j = 0
    for k1 in range(mc, 16):
        dft128(1, k1)
        for _ in range(cfg["gec_per"]):
            if j < cfg["gec_max"]:
                rad_inv(0, j)
                j += 1
    for k1 in range(16):
        idft128(1, k1)
        for _ in range(cfg["ge_per"] if k1 >= cfg["ge_at"] else 0):
            if j < 16:
                rad_inv(0, j)
                j += 1
    while j < 16:
        rad_inv(0, j)
        j += 1
    if not cfg["bd_early"]:
        wait("bd")
    j = 0
    loop = cfg["mlp_loop"]
    mem = loop > 0 or cfg["mlp_mem"]
    state = {"done": False}

    def first_prologue():
        state["nxt"] = prologue(0, mem)
        if loop == 3:
            for c in range(cfg["mlp_unroll"], cfg["nmlp"], cfg["mlp_unroll"]):
                prologue(c, True)
        state["done"] = True

    for a in range(16):
        if a == cfg["wgwu_at"]:
            wait("wg", "wu", *(("wd",) if cfg["wd_early"] else ()))
        if a == cfg["pro_at"]:
            while j < 16:
                rad_inv(1, j)
                j += 1
            first_prologue()
        HE.st(a * DH, idftd(0, a))
        for _ in range(cfg["go_per"] if a >= cfg["go_at"] else 0):
            if j < 16:
                rad_inv(1, j)
                j += 1
    while j < 16:
        rad_inv(1, j)
        j += 1
    if not state["done"]:
        first_prologue()
    NC = cfg["nmlp"]
    if cfg["wgwu_at"] >= 16:
        wait("wg", "wu", *(("wd",) if cfg["wd_early"] else ()))
    if loop == 0:
        cur = state["nxt"]
        for c in range(NC):
            fn = (lambda c=c: prologue(c + 1, mem)) if c + 1 < NC else None
            cur = mlp(c, cur, fn, wd_wait=(c == 0 and not cfg["wd_early"]))
    else:
        U = cfg["mlp_unroll"]
        if loop == 3:
            assert NC % U == 0

            def body(i, carry):
                cur = None
                for k in range(U):
                    c = i * U + k
                    fn = (lambda c=c: prologue(c + 1, False)) if k < U - 1 else None
                    cur = mlp(c, cur, fn, wd_wait=(i == 0) if (k == 0 and not cfg["wd_early"]) else False)
                return carry

            lax.fori_loop(0, NC // U, body, 0)
        elif loop == 1:
            assert NC % U == 0

            def body(i, carry):
                cur = None
                for k in range(U):
                    c = i * U + k
                    cn = jnp.minimum(c + 1, NC - 1) if k == U - 1 else c + 1
                    cur = mlp(c, cur, lambda: prologue(cn, k == U - 1 or not cfg["loop_ssa"]))
                return carry

            lax.fori_loop(0, NC // U, body, 0)
        else:
            peel = cfg["mlp_peel"]
            for c in range(peel):
                mlp(c, None, lambda c=c: prologue(c + 1, True))
            assert (NC - peel) % U == 0

            def body(i, carry):
                for k in range(U):
                    c = peel + i * U + k
                    cn = jnp.minimum(c + 1, NC - 1) if k == U - 1 else c + 1
                    mlp(c, None, lambda: prologue(cn, True))
                return carry

            lax.fori_loop(0, (NC - peel) // U, body, 0)
    with jax.named_scope("wait_out"):
        for c in range(NC):
            if cfg["down_split"] == 2:
                out_copy(c, 0).wait()
                out_copy(c, 1).wait()
            else:
                out_copy(c).wait()


@jax.jit
def pallas_sequential_preLN__spectral_gfnet__glu_gated_bilinear__prompt_kernel(
    A_x: jax.Array,
    A_w_r: jax.Array,
    A_w_i: jax.Array,
    B_x: jax.Array,
    B_w_gate: jax.Array,
    B_w_up: jax.Array,
    B_w_down: jax.Array,
):
    del B_x
    fd, G, bd = _make_consts()
    xT = A_x.reshape(S, D).T
    any_spec = pl.BlockSpec(memory_space=pl.ANY)
    outT = pl.pallas_call(
        _kernel,
        out_shape=jax.ShapeDtypeStruct((D, S), bf16),
        in_specs=[any_spec] * 9,
        out_specs=any_spec,
        scratch_shapes=[
            pltpu.VMEM((D, S), bf16),
            pltpu.VMEM((DH + 1, S), bf16),
            pltpu.VMEM((DH + 1, S), bf16),
            pltpu.VMEM((D, F), bf16),
            pltpu.VMEM((D, F), bf16),
            pltpu.VMEM((D, F), bf16),
            pltpu.VMEM((FD_ROWS, 128), u32),
            pltpu.VMEM((9, 128, 128), u32),
            pltpu.VMEM((9, 64, 128), u32),
            pltpu.VMEM((2, 2, DH // 2, 128), u32),
            pltpu.VMEM((16 * WP, 128), u32),
            pltpu.VMEM((16 * WP, 128), u32),
            pltpu.VMEM((D, S), bf16),
            pltpu.VMEM((D, S), bf16),
            pltpu.VMEM((S, D), bf16),
            pltpu.SemaphoreType.DMA((14,)),
            pltpu.SemaphoreType.DMA((16,)),
        ] + [pltpu.VMEM((n, 128), u32) for n in _layout()[2]],
        compiler_params=pltpu.CompilerParams(vmem_limit_bytes=100 * 2**20),
        name="gfnet_glu",
    )(xT, A_w_r.T, A_w_i.T, B_w_gate, B_w_up, B_w_down.T, fd, G, bd)
    return outT.T.reshape(1, S, D)
```

```python
import numpy as np
import jax
import jax.numpy as jnp
from jax import lax
from jax.experimental import pallas as pl
from jax.experimental.pallas import tpu as pltpu

S, D, F = 2048, 448, 1792
DH = D // 2
NT = S // 128
EPS = 1e-5
bf16 = jnp.bfloat16
f32 = jnp.float32
u32 = jnp.uint32
NT_DIMS = (((1,), (1,)), ((), ()))
TN_DIMS = (((0,), (0,)), ((), ()))
WP = 136

CFG = dict(xchunks=(4, 4, 4, 4), ro_per=1, ge_per=2, go_per=1, pro_at=16, tpc=2, nmlp=8,
           groups=[["YE", "YO"], ["ZE", "ZO"]], static=["EOE", "EOO"], ln_first=0,
           order=["wr", "wi", "wg", "wu", "wd"], re_at=0, ro_at=0, ge_at=0, go_at=0, wr_prep=(16, 8), wi_prep=(24, 8), wi_wait=24, h_early=0, bar_f=0, bar_g=0, bar_h=0, w_f32=0, ln2=0, g_barrier=0, m_c=16, gec_per=2, gec_max=16, mlp_loop=0, pre_t=0, down_split=0, loop_ssa=1, mlp_unroll=1, mlp_peel=2, mlp_mem=0, wd_early=0, wr_at=16, wi_at=8, bd_early=0, wgwu_at=16)
CFG.update(OPQ)
BUFS = dict(EOE=NT * 128, EOO=NT * 128, X1E=4096, X1O=4096, YE=4096, YO=4096, X2E=4096, X2O=4096,
            VE=4096, VO=4096, ZE=4096, ZO=4096, HE=NT * DH, HB1=NT * DH, HB2=NT * DH)


TRACE = []


def _layout():
    groups = [list(g) for g in CFG["groups"]]
    used = {b for g in groups for b in g}
    groups += [[b] for b in BUFS if b not in used]
    loc, sizes = {}, []
    for gi, g in enumerate(groups):
        off = 0
        for b in g:
            loc[b] = (gi, off)
            off += BUFS[b]
        sizes.append(off)
    return groups, loc, sizes


DQ = D // 4
FD_ROWS = 56 + 56 + 2 * 112


def _cis(n, period):
    nf = n.astype(f32)
    r = nf - jnp.floor(nf * np.float32(1.0 / period) + 0.5) * np.float32(period)
    ang = r * np.float32(2 * np.pi / period)
    return jnp.cos(ang), -jnp.sin(ang)


def _cmul(a, b):
    return a[0] * b[0] - a[1] * b[1], a[0] * b[1] + a[1] * b[0]


def _geom(base, step, n):
    out = [base]
    for _ in range(n - 1):
        out.append(_cmul(out[-1], step))
    return out


def _pack_rows(vregs):
    return pltpu.bitcast(jnp.concatenate(vregs, axis=0).astype(bf16), u32)


class V:
    __slots__ = ("a", "n")

    def __init__(self, a, n=False):
        self.a, self.n = a, n

    def __neg__(self):
        return V(self.a, not self.n)

    def __add__(self, o):
        if o.a is None:
            return self
        if self.a is None:
            return o
        if not self.n and not o.n:
            return V(self.a + o.a)
        if not self.n and o.n:
            return V(self.a - o.a)
        if self.n and not o.n:
            return V(o.a - self.a)
        return V(self.a + o.a, True)

    def __sub__(self, o):
        return self + (-o)

    def mul(self, c):
        if self.a is None:
            return self
        return V(self.a * np.float32(-c if self.n else c))

    def val(self, like):
        if self.a is None:
            return jnp.zeros_like(like)
        return -self.a if self.n else self.a


def _r4(x, sg):
    (x0r, x0i), (x1r, x1i), (x2r, x2i), (x3r, x3i) = x
    t0r, t0i = x0r + x2r, x0i + x2i
    t1r, t1i = x0r - x2r, x0i - x2i
    t2r, t2i = x1r + x3r, x1i + x3i
    t3r, t3i = x1r - x3r, x1i - x3i
    if sg > 0:
        ur, ui = -t3i, t3r
    else:
        ur, ui = t3i, -t3r
    return [(t0r + t2r, t0i + t2i), (t1r + ur, t1i + ui), (t0r - t2r, t0i - t2i), (t1r - ur, t1i - ui)]


def _tw(x, e, sg):
    xr, xi = x
    e = e % 16
    if e % 4 == 0:
        q = ((e // 4) if sg > 0 else (-(e // 4))) % 4
        if q == 0:
            return xr, xi
        if q == 1:
            return -xi, xr
        if q == 2:
            return -xr, -xi
        return xi, -xr
    c, s = np.cos(2 * np.pi * e / 16), sg * np.sin(2 * np.pi * e / 16)
    if e % 2 == 0:
        h = abs(c)
        a = xr if c > 0 else -xr
        b = xi if s > 0 else -xi
        re = (a - b).mul(h)
        a = xi if c > 0 else -xi
        b = xr if s > 0 else -xr
        im = (a + b).mul(h)
        return re, im
    return xr.mul(c) - xi.mul(s), xi.mul(c) + xr.mul(s)


def _fft16(re, im, sg):
    x = [(V(re[a]), V(im[a])) for a in range(16)]
    T = [_r4([x[4 * a1 + a0] for a1 in range(4)], sg) for a0 in range(4)]
    out_re, out_im = [None] * 16, [None] * 16
    for k0 in range(4):
        col = [_tw(T[a0][k0], a0 * k0, sg) for a0 in range(4)]
        y = _r4(col, sg)
        for k1 in range(4):
            out_re[k0 + 4 * k1] = y[k1][0].val(re[0])
            out_im[k0 + 4 * k1] = y[k1][1].val(re[0])
    return out_re, out_im


def _colsum(x):
    parts = [x[i:i + 8] for i in range(0, x.shape[0], 8)]
    while len(parts) > 1:
        nxt = [parts[i] + parts[i + 1] for i in range(0, len(parts) - 1, 2)]
        if len(parts) % 2:
            nxt.append(parts[-1])
        parts = nxt
    return jnp.sum(parts[0], axis=0, keepdims=True)


def _deilv16(x):
    a = jnp.concatenate([x[32 * j:32 * j + 16] for j in range(8)], axis=0)
    b = jnp.concatenate([x[32 * j + 16:32 * j + 32] for j in range(8)], axis=0)
    return a, b


def _pack16(x):
    return pltpu.pack_elementwise([x[0:8], x[8:16]], packed_dtype=bf16)


def _lo(w):
    return lax.bitcast_convert_type(lax.shift_left(w, np.uint32(16)), f32)


def _hi(w):
    return lax.bitcast_convert_type(w & np.uint32(0xFFFF0000), f32)


def _bf(x):
    return pltpu.bitcast(x, bf16)


class Arena:
    def __init__(self, ref, static=False):
        self.ref, self.static = ref, static
        self.sv = self.lv = ref if static else None

    def bind(self, zs, zl):
        self.zs, self.zl = zs, zl
        if not self.static:
            n = self.ref.shape[0]
            self.sv = self.ref.at[pl.ds(zs, n)]
            self.lv = self.ref.at[pl.ds(zl, n)]


class Buf:
    def __init__(self, arena, off):
        self.a, self.off = arena, off

    def sub(self, c, n):
        if isinstance(c, int):
            return Buf(self.a, self.off + c * n)
        ar = Arena(self.a.ref)
        base = pl.multiple_of(self.off + c * n, 8)
        ar.sv = self.a.ref.at[pl.ds(self.a.zs + base, n)]
        ar.lv = self.a.ref.at[pl.ds(self.a.zl + base, n)]
        return Buf(ar, 0)

    def st(self, row, val):
        if val.dtype != u32:
            val = lax.bitcast_convert_type(val, u32)
        row += self.off
        self.a.sv[row:row + val.shape[0], :] = val

    def st_strided(self, row, val, stride):
        if val.dtype != u32:
            val = lax.bitcast_convert_type(val, u32)
        row += self.off
        self.a.sv[pl.ds(row, val.shape[0], stride=stride), :] = val

    def ld(self, row, n, dtype=f32):
        row += self.off
        v = self.a.lv[row:row + n, :]
        return v if dtype == u32 else lax.bitcast_convert_type(v, dtype)


def _kernel(x_hbm, wr_hbm, wi_hbm, wg_hbm, wu_hbm, wd_hbm, z_hbm,
            out_hbm,
            x_v, wr_v, wi_v, wg_v, wu_v, wd_v, fd_v, g_v, gs_v, bd_v, z_v, zb_v,
            Wtr, Wti, out_v, hn_v, hn2_v, sems, *arenas):
    cfg = CFG
    xch = cfg["xchunks"]
    xst = [sum(xch[:c]) for c in range(len(xch) + 1)]
    x_cp = [pltpu.make_async_copy(x_hbm.at[:, pl.ds(128 * xst[c], 128 * xch[c])],
                                  x_v.at[:, pl.ds(128 * xst[c], 128 * xch[c])], sems.at[c])
            for c in range(len(xch))]
    nx = len(xch)
    cp_z = pltpu.make_async_copy(z_hbm, z_v, sems.at[0])
    cp_wr = pltpu.make_async_copy(wr_hbm, wr_v, sems.at[nx])
    cp_wi = pltpu.make_async_copy(wi_hbm, wi_v, sems.at[nx + 1])
    cp_wg = pltpu.make_async_copy(wg_hbm, wg_v, sems.at[nx + 2])
    cp_wu = pltpu.make_async_copy(wu_hbm, wu_v, sems.at[nx + 2])
    cp_wd = pltpu.make_async_copy(wd_hbm, wd_v, sems.at[nx + 2])
    assert cfg["wd_early"]
    bars = [n for n in ("bar_f", "bar_g", "bar_h") if cfg[n]]
    cps = dict(z=cp_z, wr=cp_wr, wi=cp_wi, wg=cp_wg, wu=cp_wu, wd=cp_wd)
    for c in range(len(xch)):
        cps["x%d" % c] = x_cp[c]
    for k, n in enumerate(bars):
        cps[n] = pltpu.make_async_copy(z_hbm.at[pl.ds(0, 8)], zb_v.at[k], sems.at[nx + 4 + k])
    order = ["z"] + bars + ["x0"] + ["x%d" % c for c in range(1, len(xch))] + cfg["order"]

    del TRACE[:]
    TRACE.append(("order", order, list(xch)))
    for n in order:
        cps[n].start()

    def make_tables():
        i = lax.broadcasted_iota(jnp.int32, (8, 128), 0)
        c = lax.broadcasted_iota(jnp.int32, (8, 128), 1)
        step = _cis(16 * c, 128)
        f = [_geom(_cis((2 * i + b) * c, 128), step, 8) for b in range(2)]
        t1 = _cis(c, S)
        t = t1
        for km in range(9):
            g = f
            if km:
                if km > 1:
                    t = _cmul(t, t1)
                g = [[_cmul(e, t) for e in fb] for fb in f]
            pk = lambda x, y: pltpu.pack_elementwise([x, y], packed_dtype=bf16)
            g_v[km, 0:64, :] = jnp.concatenate([pk(g[0][a][0], g[1][a][0]) for a in range(8)], axis=0)
            g_v[km, 64:128, :] = jnp.concatenate([pk(g[0][a][1], g[1][a][1]) for a in range(8)], axis=0)
            gs_v[km] = jnp.concatenate([pk(g[0][a][0] + g[0][a][1], g[1][a][0] + g[1][a][1]) for a in range(8)], axis=0)
        dq = (c & 0x70) | ((c & 1) << 3) | ((c >> 1) & 7)
        b0, st0 = _cis(4 * i * dq, D), _cis(32 * dq, D)
        e0 = _geom(b0, st0, 7)
        e2 = _geom(_cmul(b0, _cis(2 * dq, D)), st0, 7)
        nyq = (1 - 2 * (dq & 1)).astype(f32)
        im0 = [jnp.where(i == 0, nyq, e0[0][1])] + [e[1] for e in e0[1:]]
        fd_v[0:56, :] = _pack_rows([e[0] for e in e0] + im0)
        fd_v[56:112, :] = _pack_rows([e[0] for e in e2] + [e[1] for e in e2])
        for kt in range(2):
            dd = dq + 128 * kt
            eo = _geom(_cis((2 * i + 1) * dd, D), _cis(16 * dd, D), 14)
            fd_v[112 + 112 * kt:224 + 112 * kt, :] = _pack_rows([e[0] for e in eo] + [e[1] for e in eo])
        sc = np.float32(1.0 / (D * S))
        for p in range(2):
            kd = 2 * c + p
            if p == 0:
                wgt = jnp.where((c == 0) | (c == DQ), sc, jnp.where(c < DQ, 2 * sc, np.float32(0)))
            else:
                wgt = jnp.where(c < DQ, 2 * sc, np.float32(0))
            base, step = _cis(kd * i, D), _cis(8 * kd, D)
            if p == 0:
                base = (base[0], jnp.where(c == DQ, np.float32(0), base[1]))
                step = (step[0], jnp.where(c == DQ, np.float32(0), step[1]))
            e = _geom((base[0] * wgt, base[1] * wgt), step, DH // 8)
            bd_v[p, 0] = _pack_rows([x[0] for x in e])
            bd_v[p, 1] = _pack_rows([x[1] for x in e])

    def wait(*names):
        TRACE.append(("wait", names))
        if cfg.get("scopes"):
            with jax.named_scope("wait_" + names[0]):
                for n in names:
                    cps[n].wait()
            return
        for n in names:
            cps[n].wait()

    import contextlib
    scope = (lambda n: jax.named_scope(n)) if cfg.get("scopes") == 2 else (lambda n: contextlib.nullcontext())
    with scope("ph_tables"):
        make_tables()
    wait("z", "x0")
    groups, loc, _ = _layout()
    ars = [Arena(r, static=all(b in cfg["static"] for b in g)) for r, g in zip(arenas, groups)]
    bufs = {b: Buf(ars[gi], off) for b, (gi, off) in loc.items()}
    X1 = [bufs["X1E"], bufs["X1O"]]
    Yb = [bufs["YE"], bufs["YO"]]
    X2 = [bufs["X2E"], bufs["X2O"]]
    Vb = [bufs["VE"], bufs["VO"]]
    Zb = [bufs["ZE"], bufs["ZO"]]
    HE = bufs["HE"]

    def make_views():
        zz = z_v[0:16, :]
        z1 = pl.multiple_of(jnp.max(zz[0:8]), 8)
        z2 = pl.multiple_of(jnp.max(zz[8:16]), 8)
        for ar in ars:
            ar.bind(z1, z2)
    rstd = [None] * NT

    def ln1(a):
        if cfg.get("dbg_noln") and a < 15:
            return
        x = x_v[:, a * 128:(a + 1) * 128].astype(f32)
        a0, o_lo, o_hi, a2p = [], [], [], []
        accd, acca = [None, None], [None, None]

        def acc(l, i, v):
            l[i] = v if l[i] is None else l[i] + v

        for j in range(DQ // 16):
            x0, x1, x2, x3 = (x[q * DQ + 16 * j:q * DQ + 16 * j + 16] for q in range(4))
            s02, s13 = x0 + x2, x1 + x3
            d02, d13 = x0 - x2, x1 - x3
            a0.append(s02 + s13)
            a2 = s02 - s13
            o_lo.append(_pack16(d02))
            o_hi.append(_pack16(d13))
            a2p.append(_pack16(a2))
            acc(accd, 0, d02 * d02)
            acc(accd, 1, d13 * d13)
            acc(acca, 0, a2 * a2)
        m4 = _colsum(jnp.concatenate(a0, axis=0)) * (4.0 / D)
        a0p = []
        for j in range(DQ // 16):
            t = a0[j] - m4
            a0p.append(_pack16(t))
            acc(acca, 1, t * t)
        v = _colsum((accd[0] + accd[1]) * 2.0 + (acca[0] + acca[1])) * (0.25 / D)
        rstd[a] = lax.rsqrt(v + EPS)
        bufs["EOO"].st(a * 128, jnp.concatenate(o_lo + o_hi, axis=0))
        bufs["EOE"].st(a * 128, jnp.concatenate(a0p + a2p, axis=0))

    row0 = lax.broadcasted_iota(jnp.int32, (8, 128), 0) == 0

    def dftd_e(a, q):
        rhs = jnp.concatenate([bufs["EOE"].ld(a * 128 + 56 * q, 56, u32), jnp.zeros((8, 128), u32)], axis=0)
        r = jnp.dot(_bf(fd_v[56 * q:56 * q + 56, :]), _bf(rhs), preferred_element_type=f32) * rstd[a]
        for c in range(2):
            for v in range(7):
                t = r[56 * c + 8 * v:56 * c + 8 * v + 8]
                if q == 0 and c == 1 and v == 0:
                    X1[0].st(a * 256 + 112, jnp.where(row0, t, 0.0))
                    t = jnp.where(row0, 0.0, t)
                X1[0].st_strided(a * 256 + 128 * c + 16 * v + q, t, 2)

    def dftd_o(a):
        lhs = jnp.concatenate([_bf(fd_v[112:224, :]), _bf(fd_v[224:336, :])], axis=1)
        rhs = jnp.concatenate([bufs["EOO"].ld(a * 128, 112, u32), jnp.zeros((16, 128), u32)], axis=0)
        r = jnp.dot(lhs, _bf(rhs), preferred_element_type=f32) * rstd[a]
        X1[1].st(a * 256, r[:DQ])
        X1[1].st(a * 256 + 128, r[DQ:])

    def rad_fwd(p, j):
        r = 8 * j
        re = [X1[p].ld(a * 256 + r, 8) for a in range(16)]
        nyq = (p == 0 and j == 14)
        im = [None if nyq else X1[p].ld(a * 256 + 128 + r, 8) for a in range(16)]
        ore, oim = _fft16(re, im, -1)
        for k1 in range(16):
            Yb[p].st(k1 * 256 + r, ore[k1])
            Yb[p].st(k1 * 256 + 128 + r, oim[k1])

    def y_get(p, k1):
        n = 112 if p else 120
        z = jnp.zeros((128 - n, 128), f32)
        return (jnp.concatenate([Yb[p].ld(k1 * 256, n), z], axis=0),
                jnp.concatenate([Yb[p].ld(k1 * 256 + 128, n), z], axis=0))

    def gmat(k1):
        return (k1, 1) if k1 < 8 else (16 - k1, -1)

    def gparts(km):
        return _bf(g_v[km, 0:64, :]), _bf(g_v[km, 64:128, :]), _bf(gs_v[km])

    def cmul3(km, conj, a, b, dims):
        gr, gi, gs = gparts(km)
        t1 = lax.dot_general(gr, a.astype(bf16), dims, preferred_element_type=f32)
        t2 = lax.dot_general(gi, b.astype(bf16), dims, preferred_element_type=f32)
        if conj:
            t3 = lax.dot_general(gs, (b - a).astype(bf16), dims, preferred_element_type=f32)
            return t1 + t2, t3 + (t1 - t2)
        t3 = lax.dot_general(gs, (a + b).astype(bf16), dims, preferred_element_type=f32)
        return t1 - t2, t3 - (t1 + t2)

    def x2row(p, k1):
        return k1 * 256

    def dft128(p, k1):
        km, sg = gmat(k1)
        yr, yi = y_get(p, k1)
        xr, xi = cmul3(km, sg < 0, yr, yi, NT_DIMS)
        X2[p].st(x2row(p, k1), xr)
        X2[p].st(x2row(p, k1) + 128, xi)

    rows8 = lax.broadcasted_iota(jnp.int32, (8, 128), 0)

    def wprep(w_v, Wt, a):
        w32 = pltpu.bitcast(w_v[0:DH, a * 128:(a + 1) * 128], u32)
        ny = w_v[DH:DH + 1, a * 128:(a + 1) * 128].astype(f32)
        ny = jnp.broadcast_to(ny, (8, 128))
        nyu = lax.shift_right_logical(lax.bitcast_convert_type(ny, u32), np.uint32(16))
        nyu = jnp.where(rows8 == 0, nyu, np.uint32(0))
        t = jnp.concatenate([w32, nyu, jnp.zeros((8, 128), u32)], axis=0).T
        if cfg["w_f32"]:
            for p, tp in enumerate((_lo(t), _hi(t))):
                tp = lax.bitcast_convert_type(tp, u32)
                for j in range(8):
                    Wt[pl.ds(p * 16 * WP + a * WP + 17 * j, 8), :] = tp[16 * j:16 * j + 8, :]
                    Wt[pl.ds(p * 16 * WP + (15 - a) * WP + 17 * (7 - j) + 8, 8), :] = tp[16 * j + 8:16 * j + 16, :]
            return
        for j in range(8):
            Wt[pl.ds(a * WP + 17 * j, 8), :] = t[16 * j:16 * j + 8, :]
            Wt[pl.ds((15 - a) * WP + 17 * (7 - j) + 8, 8), :] = t[16 * j + 8:16 * j + 16, :]

    def idft128(p, k1, mid=None):
        km, sg = gmat(k1)
        if cfg["w_f32"]:
            o = p * 16 * WP + k1
            wr = jnp.concatenate([Wtr[pl.ds(o + A_ * WP, 8, stride=17), :] for A_ in range(16)], axis=0)
            wi = jnp.concatenate([Wti[pl.ds(o + A_ * WP, 8, stride=17), :] for A_ in range(16)], axis=0)
            wr, wi = lax.bitcast_convert_type(wr, f32), lax.bitcast_convert_type(wi, f32)
        else:
            wr32 = jnp.concatenate([Wtr[pl.ds(A_ * WP + k1, 8, stride=17), :] for A_ in range(16)], axis=0)
            wi32 = jnp.concatenate([Wti[pl.ds(A_ * WP + k1, 8, stride=17), :] for A_ in range(16)], axis=0)
            if p == 0:
                wr, wi = _lo(wr32), _lo(wi32)
            else:
                wr, wi = _hi(wr32), _hi(wi32)
        xr, xi = X2[p].ld(x2row(p, k1), 128), X2[p].ld(x2row(p, k1) + 128, 128)
        vr, vi = cmul3(km, sg > 0, xr * wr - xi * wi, xr * wi + xi * wr, TN_DIMS)
        if mid is not None:
            mid()
        Vb[p].st(k1 * 256, vr)
        Vb[p].st(k1 * 256 + 128, vi)

    def rad_inv(p, j):
        r = 8 * j
        re = [Vb[p].ld(k1 * 256 + r, 8) for k1 in range(16)]
        im = [Vb[p].ld(k1 * 256 + 128 + r, 8) for k1 in range(16)]
        ore, oim = _fft16(re, im, +1)
        for s1 in range(16):
            Zb[p].st(s1 * 256 + r, ore[s1])
            Zb[p].st(s1 * 256 + 128 + r, oim[s1])

    def idftd2(p, zb, t):
        z = jnp.concatenate([zb.ld(t * 256, 128), zb.ld(t * 256 + 128, 128)], axis=1).astype(bf16)
        lhs = jnp.concatenate([_bf(bd_v[p, 0]), _bf(bd_v[p, 1])], axis=1)
        return lax.dot_general(lhs, z, NT_DIMS, preferred_element_type=f32)

    def idftd(p, a):
        return idftd2(p, Zb[p], a)

    TPC = 2
    CW = TPC * 128

    def cols(c, t=0, n=CW):
        if isinstance(c, int):
            return pl.ds(c * CW + t * 128, n)
        return pl.ds(pl.multiple_of(c * CW, CW) + t * 128, n)

    def h_get(hb, t):
        w = hb.ld(t * DH, DH, u32)
        return jnp.concatenate([f(w[8 * j:8 * j + 8]) for j in range(D // 16) for f in (_lo, _hi)], axis=0)

    def prologue2(c, mem):
        zo, he = Zb[1].sub(c, TPC * 256), HE.sub(c, TPC * DH)
        hb1, hb2 = bufs["HB1"].sub(c, TPC * DH), bufs["HB2"].sub(c, TPC * DH)
        ms, rs = [], []
        for t in range(TPC):
            O = idftd2(1, zo, t)
            E = he.ld(t * DH, DH)
            x = x_v[:, cols(c, t, 128)].astype(f32)
            pk = [None] * (D // 16)
            for j in range(DH // 16):
                e, o = E[16 * j:16 * j + 16], O[16 * j:16 * j + 16]
                pk[j] = _pack16(x[16 * j:16 * j + 16] + (e + o))
                pk[DH // 16 + j] = _pack16(x[DH + 16 * j:DH + 16 * j + 16] + (e - o))
            w = jnp.concatenate(pk, axis=0)
            hb1.st(t * DH, w)
            hb2.st(t * DH, w)
            acc = [None] * 4
            for j, p_ in enumerate(pk):
                for k, f in enumerate((_lo, _hi)):
                    i = (2 * j + k) % 4
                    acc[i] = f(p_) if acc[i] is None else acc[i] + f(p_)
            ms.append(_colsum((acc[0] + acc[1]) + (acc[2] + acc[3])) * (1.0 / D))
        for t in range(TPC):
            w = hb2.ld(t * DH, DH, u32)
            acc = [None] * 4
            for j in range(D // 16):
                for k, f in enumerate((_lo, _hi)):
                    i = (2 * j + k) % 4
                    d = f(w[8 * j:8 * j + 8]) - ms[t]
                    acc[i] = d * d if acc[i] is None else acc[i] + d * d
            v = _colsum((acc[0] + acc[1]) + (acc[2] + acc[3])) * (1.0 / D)
            rs.append(lax.rsqrt(v + EPS))
        hns = [(h_get(hb1, t) - ms[t]) * rs[t] for t in range(TPC)]
        hn = jnp.concatenate(hns, axis=1).astype(bf16)
        if mem:
            hn_v[:, cols(c)] = hn
            return None
        return None, hn

    def prologue(c, mem):
        if cfg["ln2"] == 1:
            return prologue2(c, mem)
        zo, he = Zb[1].sub(c, TPC * 256), HE.sub(c, TPC * DH)
        hs, hns = [], []
        for t in range(TPC):
            O = idftd2(1, zo, t)
            E = he.ld(t * DH, DH)
            y = jnp.concatenate([E + O, E - O], axis=0)
            hb = (x_v[:, cols(c, t, 128)].astype(f32) + y).astype(bf16)
            hf = hb.astype(f32)
            m = _colsum(hf) * (1.0 / D)
            hc = hf - m
            v = _colsum(hc * hc) * (1.0 / D)
            hs.append(hf)
            hns.append(hc * lax.rsqrt(v + EPS))
            if mem:
                out_v[:, cols(c, t, 128)] = hb
        hn = jnp.concatenate(hns, axis=1).astype(bf16)
        if mem:
            hn_v[:, cols(c)] = hn
            return None
        return jnp.concatenate(hs, axis=1), hn

    def rows(c):
        if isinstance(c, int):
            return pl.ds(c * CW, CW)
        return pl.ds(pl.multiple_of(c * CW, CW), CW)

    def out_copy(c, t=None):
        if t is None:
            return pltpu.make_async_copy(out_v.at[:, cols(c)], out_hbm.at[:, cols(c)], sems.at[nx + 3])
        return pltpu.make_async_copy(out_v.at[:, cols(c, t, 128)], out_hbm.at[:, cols(c, t, 128)], sems.at[nx + 3])

    def mlp(c, cur, nxt_fn=None, wd_wait=False):
        hnT = hn_v[:, cols(c)] if cur is None else cur[1]
        nxt = nxt_fn() if nxt_fn is not None else None
        g = lax.dot_general(hnT, wg_v[...], TN_DIMS, preferred_element_type=f32)
        u = lax.dot_general(hnT, wu_v[...], TN_DIMS, preferred_element_type=f32)
        hh = (g * u).astype(bf16)
        if wd_wait is True:
            wait("wd")
        elif wd_wait is not False:
            @pl.when(wd_wait)
            def _():
                wait("wd")
        if cfg["down_split"]:
            for t in range(TPC):
                mlp = lax.dot_general(wd_v[...], hh[t * 128:(t + 1) * 128], NT_DIMS, preferred_element_type=f32)
                if cfg["ln2"] == 1:
                    h = h_get(bufs["HB1"].sub(c, TPC * DH), t)
                else:
                    h = out_v[:, cols(c, t, 128)].astype(f32) if cur is None else cur[0][:, t * 128:(t + 1) * 128]
                out_v[:, cols(c, t, 128)] = (h + mlp.astype(bf16).astype(f32)).astype(bf16)
                if cfg["down_split"] == 2:
                    out_copy(c, t).start()
            if cfg["down_split"] == 1:
                out_copy(c).start()
            return nxt
        mlp = lax.dot_general(wd_v[...], hh, NT_DIMS, preferred_element_type=f32)
        h = out_v[:, cols(c)].astype(f32) if cur is None else cur[0]
        out_v[:, cols(c)] = (h + mlp.astype(bf16).astype(f32)).astype(bf16)
        out_copy(c).start()
        return nxt

    def fwd_tile(a):
        if cfg.get("dbg_nofwd") and a < 15:
            return
        if a % 2 == 0:
            dftd_e(a, 0)
            dftd_e(a, 1)
            dftd_o(a)
        else:
            dftd_o(a)
            dftd_e(a, 0)
            dftd_e(a, 1)

    make_views()
    with scope("ph_fwd"):
        ln1(0)
        for a in range(1, NT):
            if a in xst:
                wait("x%d" % xst.index(a))
            fwd_tile(a - 1)
            ln1(a)
        fwd_tile(NT - 1)
    if cfg.get("dbg_stop") == 1:
        for n in order:
            if not (n[0] == "x" or n == "z"):
                wait(n)
        out_v[0:8, 0:128] = X1[0].ld(15 * 256, 8).astype(bf16) + X1[1].ld(15 * 256, 8).astype(bf16)
        cp = pltpu.make_async_copy(out_v.at[:, pl.ds(0, 128)], out_hbm.at[:, pl.ds(0, 128)], osems.at[0])
        cp.start()
        cp.wait()
        return
    for j in range(15):
        rad_fwd(0, j)
    wait("wr")
    def spread(k, k0, n, total, fn):
        if k0 <= k < k0 + n:
            for a in range(total * (k - k0) // n, total * (k - k0 + 1) // n):
                fn(a)

    j = 0
    wr0, wrn = cfg["wr_prep"]
    wi0, win = cfg["wi_prep"]
    for q in range(32):
        if q == cfg["wi_wait"]:
            wait("wi")
        dft128(q // 16, q % 16)
        if q >= cfg["ro_at"] and j < 14:
            rad_fwd(1, j)
            j += 1
        spread(q, wr0, wrn, 16, lambda a: wprep(wr_v, Wtr, a))
        spread(q, wi0, win, 16, lambda a: wprep(wi_v, Wti, a))
    assert j == 14 and cfg["ro_at"] <= 2 and wi0 >= cfg["wi_wait"]
    if cfg["bar_f"]:
        wait("bar_f")
    for k1 in range(16):
        idft128(0, k1)
    if cfg["bar_g"]:
        wait("bar_g")
    j = 0
    ne = cfg["h_early"]

    def early_h():
        for a in range(ne):
            HE.st(a * DH, idftd(0, a))

    for k1 in range(16):
        idft128(1, k1, early_h if (k1 == 15 and ne) else None)
        for _ in range(cfg["ge_per"] if k1 >= cfg["ge_at"] else 0):
            if j < 16:
                rad_inv(0, j)
                j += 1
    while j < 16:
        rad_inv(0, j)
        j += 1
    if cfg["bar_h"]:
        wait("bar_h")
    j = 0
    loop = cfg["mlp_loop"]
    mem = loop > 0 or cfg["mlp_mem"]
    state = {"done": False}

    def first_prologue():
        state["nxt"] = prologue(0, mem)
        if loop == 3:
            for c in range(cfg["mlp_unroll"], cfg["nmlp"], cfg["mlp_unroll"]):
                prologue(c, True)
        state["done"] = True

    for a in range(ne, 16):
        if a == cfg["wgwu_at"]:
            wait("wg", "wu", *(("wd",) if cfg["wd_early"] else ()))
        if a == cfg["pro_at"]:
            while j < 16:
                rad_inv(1, j)
                j += 1
            first_prologue()
        HE.st(a * DH, idftd(0, a))
        for _ in range(cfg["go_per"] if a >= cfg["go_at"] else 0):
            if j < 16:
                rad_inv(1, j)
                j += 1
    while j < 16:
        rad_inv(1, j)
        j += 1
    if not state["done"]:
        first_prologue()
    NC = cfg["nmlp"]
    if cfg["wgwu_at"] >= 16:
        wait("wg", "wu", *(("wd",) if cfg["wd_early"] else ()))
    if loop == 0:
        cur = state["nxt"]
        for c in range(NC):
            fn = (lambda c=c: prologue(c + 1, mem)) if c + 1 < NC else None
            cur = mlp(c, cur, fn, wd_wait=(c == 0 and not cfg["wd_early"]))
    else:
        U = cfg["mlp_unroll"]
        if loop == 3:
            assert NC % U == 0

            def body(i, carry):
                cur = None
                for k in range(U):
                    c = i * U + k
                    fn = (lambda c=c: prologue(c + 1, False)) if k < U - 1 else None
                    cur = mlp(c, cur, fn, wd_wait=(i == 0) if (k == 0 and not cfg["wd_early"]) else False)
                return carry

            with scope("ph_loop"):
                lax.fori_loop(0, NC // U, body, 0)
        elif loop == 1:
            assert NC % U == 0

            def body(i, carry):
                cur = None
                for k in range(U):
                    c = i * U + k
                    cn = jnp.minimum(c + 1, NC - 1) if k == U - 1 else c + 1
                    cur = mlp(c, cur, lambda: prologue(cn, k == U - 1 or not cfg["loop_ssa"]))
                return carry

            lax.fori_loop(0, NC // U, body, 0)
        else:
            peel = cfg["mlp_peel"]
            for c in range(peel):
                mlp(c, None, lambda c=c: prologue(c + 1, True))
            assert (NC - peel) % U == 0

            def body(i, carry):
                for k in range(U):
                    c = peel + i * U + k
                    cn = jnp.minimum(c + 1, NC - 1) if k == U - 1 else c + 1
                    mlp(c, None, lambda: prologue(cn, True))
                return carry

            lax.fori_loop(0, (NC - peel) // U, body, 0)
    pltpu.make_async_copy(out_v, out_hbm, sems.at[nx + 3]).wait()


@jax.jit
def pallas_sequential_preLN__spectral_gfnet__glu_gated_bilinear__prompt_kernel(
    A_x: jax.Array,
    A_w_r: jax.Array,
    A_w_i: jax.Array,
    B_x: jax.Array,
    B_w_gate: jax.Array,
    B_w_up: jax.Array,
    B_w_down: jax.Array,
):
    del B_x
    zc = np.zeros((24, 128), np.int32)
    zc[16:] = np.arange(128)
    xT = A_x.reshape(S, D).T
    any_spec = pl.BlockSpec(memory_space=pl.ANY)
    outT = pl.pallas_call(
        _kernel,
        out_shape=jax.ShapeDtypeStruct((D, S), bf16),
        in_specs=[any_spec] * 7,
        out_specs=any_spec,
        scratch_shapes=[
            pltpu.VMEM((D, S), bf16),
            pltpu.VMEM((DH + 1, S), bf16),
            pltpu.VMEM((DH + 1, S), bf16),
            pltpu.VMEM((D, F), bf16),
            pltpu.VMEM((D, F), bf16),
            pltpu.VMEM((D, F), bf16),
            pltpu.VMEM((FD_ROWS, 128), u32),
            pltpu.VMEM((9, 128, 128), u32),
            pltpu.VMEM((9, 64, 128), u32),
            pltpu.VMEM((2, 2, DH // 2, 128), u32),
            pltpu.VMEM((24, 128), jnp.int32),
            pltpu.VMEM((3, 8, 128), jnp.int32),
            pltpu.VMEM(((2 if CFG["w_f32"] else 1) * 16 * WP, 128), u32),
            pltpu.VMEM(((2 if CFG["w_f32"] else 1) * 16 * WP, 128), u32),
            pltpu.VMEM((D, S), bf16),
            pltpu.VMEM((D, S), bf16),
            pltpu.VMEM((S, D), bf16),
            pltpu.SemaphoreType.DMA((len(CFG["xchunks"]) + 4 + sum(bool(CFG[n]) for n in ("bar_f", "bar_g", "bar_h")),)),
        ] + [pltpu.VMEM((n, 128), u32) for n in _layout()[2]],
        compiler_params=pltpu.CompilerParams(vmem_limit_bytes=100 * 2**20),
        name="gfnet_glu",
    )(xT, A_w_r.T, A_w_i.T, B_w_gate, B_w_up, B_w_down.T, zc)
    return outT.T.reshape(1, S, D)
```

```python
import numpy as np
import jax
import jax.numpy as jnp
from jax import lax
from jax.experimental import pallas as pl
from jax.experimental.pallas import tpu as pltpu

S, D, F = 2048, 448, 1792
DH = D // 2
NT = S // 128
EPS = 1e-5
bf16 = jnp.bfloat16
f32 = jnp.float32
u32 = jnp.uint32
NT_DIMS = (((1,), (1,)), ((), ()))
TN_DIMS = (((0,), (0,)), ((), ()))
WP = 136

CFG = dict(xchunks=(4, 4, 4, 4), ro_per=1, ge_per=2, go_per=1, pro_at=16, tpc=2, nmlp=8,
           groups=[["YE", "YO"], ["ZE", "ZO"]], static=[], ln_first=0,
           order=["wr", "wi", "wg", "wu", "wd"], re_at=0, ro_at=0, ge_at=0, go_at=0, wr_prep=(16, 8), wi_prep=(24, 8), wi_wait=24, h_early=0, bar_f=0, bar_g=0, bar_h=0, w_f32=0, ln2=0, g_barrier=0, m_c=16, gec_per=2, gec_max=16, mlp_loop=0, pre_t=0, down_split=0, loop_ssa=1, mlp_unroll=1, mlp_peel=2, mlp_mem=0, wd_early=0, wr_at=16, wi_at=8, bd_early=0, wgwu_at=16)
CFG.update(OPQ)
BUFS = dict(X1E=4096, X1O=4096, YE=4096, YO=4096, X2E=4096, X2O=4096,
            VE=4096, VO=4096, ZE=4096, ZO=4096, HE=NT * DH)


TRACE = []


def _layout():
    groups = [list(g) for g in CFG["groups"]]
    used = {b for g in groups for b in g}
    groups += [[b] for b in BUFS if b not in used]
    loc, sizes = {}, []
    for gi, g in enumerate(groups):
        off = 0
        for b in g:
            loc[b] = (gi, off)
            off += BUFS[b]
        sizes.append(off)
    return groups, loc, sizes


DQ = D // 4
FD_ROWS = 56 + 56 + 2 * 112


def _cis(n, period):
    nf = n.astype(f32)
    r = nf - jnp.floor(nf * np.float32(1.0 / period) + 0.5) * np.float32(period)
    ang = r * np.float32(2 * np.pi / period)
    return jnp.cos(ang), -jnp.sin(ang)


def _cmul(a, b):
    return a[0] * b[0] - a[1] * b[1], a[0] * b[1] + a[1] * b[0]


def _geom(base, step, n):
    out = [base]
    for _ in range(n - 1):
        out.append(_cmul(out[-1], step))
    return out


def _pack_rows(vregs):
    return pltpu.bitcast(jnp.concatenate(vregs, axis=0).astype(bf16), u32)


class V:
    __slots__ = ("a", "n")

    def __init__(self, a, n=False):
        self.a, self.n = a, n

    def __neg__(self):
        return V(self.a, not self.n)

    def __add__(self, o):
        if o.a is None:
            return self
        if self.a is None:
            return o
        if not self.n and not o.n:
            return V(self.a + o.a)
        if not self.n and o.n:
            return V(self.a - o.a)
        if self.n and not o.n:
            return V(o.a - self.a)
        return V(self.a + o.a, True)

    def __sub__(self, o):
        return self + (-o)

    def mul(self, c):
        if self.a is None:
            return self
        return V(self.a * np.float32(-c if self.n else c))

    def val(self, like):
        if self.a is None:
            return jnp.zeros_like(like)
        return -self.a if self.n else self.a


def _r4(x, sg):
    (x0r, x0i), (x1r, x1i), (x2r, x2i), (x3r, x3i) = x
    t0r, t0i = x0r + x2r, x0i + x2i
    t1r, t1i = x0r - x2r, x0i - x2i
    t2r, t2i = x1r + x3r, x1i + x3i
    t3r, t3i = x1r - x3r, x1i - x3i
    if sg > 0:
        ur, ui = -t3i, t3r
    else:
        ur, ui = t3i, -t3r
    return [(t0r + t2r, t0i + t2i), (t1r + ur, t1i + ui), (t0r - t2r, t0i - t2i), (t1r - ur, t1i - ui)]


def _tw(x, e, sg):
    xr, xi = x
    e = e % 16
    if e % 4 == 0:
        q = ((e // 4) if sg > 0 else (-(e // 4))) % 4
        if q == 0:
            return xr, xi
        if q == 1:
            return -xi, xr
        if q == 2:
            return -xr, -xi
        return xi, -xr
    c, s = np.cos(2 * np.pi * e / 16), sg * np.sin(2 * np.pi * e / 16)
    if e % 2 == 0:
        h = abs(c)
        a = xr if c > 0 else -xr
        b = xi if s > 0 else -xi
        re = (a - b).mul(h)
        a = xi if c > 0 else -xi
        b = xr if s > 0 else -xr
        im = (a + b).mul(h)
        return re, im
    return xr.mul(c) - xi.mul(s), xi.mul(c) + xr.mul(s)


def _fft16(re, im, sg):
    x = [(V(re[a]), V(im[a])) for a in range(16)]
    T = [_r4([x[4 * a1 + a0] for a1 in range(4)], sg) for a0 in range(4)]
    out_re, out_im = [None] * 16, [None] * 16
    for k0 in range(4):
        col = [_tw(T[a0][k0], a0 * k0, sg) for a0 in range(4)]
        y = _r4(col, sg)
        for k1 in range(4):
            out_re[k0 + 4 * k1] = y[k1][0].val(re[0])
            out_im[k0 + 4 * k1] = y[k1][1].val(re[0])
    return out_re, out_im


def _colsum(x):
    parts = [x[i:i + 8] for i in range(0, x.shape[0], 8)]
    while len(parts) > 1:
        nxt = [parts[i] + parts[i + 1] for i in range(0, len(parts) - 1, 2)]
        if len(parts) % 2:
            nxt.append(parts[-1])
        parts = nxt
    return jnp.sum(parts[0], axis=0, keepdims=True)


def _deilv16(x):
    a = jnp.concatenate([x[32 * j:32 * j + 16] for j in range(8)], axis=0)
    b = jnp.concatenate([x[32 * j + 16:32 * j + 32] for j in range(8)], axis=0)
    return a, b


def _lo(w):
    return lax.bitcast_convert_type(lax.shift_left(w, np.uint32(16)), f32)


def _hi(w):
    return lax.bitcast_convert_type(w & np.uint32(0xFFFF0000), f32)


def _bf(x):
    return pltpu.bitcast(x, bf16)


class Arena:
    def __init__(self, ref, static=False):
        self.ref, self.static = ref, static
        self.sv = self.lv = ref if static else None

    def bind(self, zs, zl):
        self.zs, self.zl = zs, zl
        if not self.static:
            n = self.ref.shape[0]
            self.sv = self.ref.at[pl.ds(zs, n)]
            self.lv = self.ref.at[pl.ds(zl, n)]


class Buf:
    def __init__(self, arena, off):
        self.a, self.off = arena, off

    def sub(self, c, n):
        if isinstance(c, int):
            return Buf(self.a, self.off + c * n)
        ar = Arena(self.a.ref)
        base = pl.multiple_of(self.off + c * n, 8)
        ar.sv = self.a.ref.at[pl.ds(self.a.zs + base, n)]
        ar.lv = self.a.ref.at[pl.ds(self.a.zl + base, n)]
        return Buf(ar, 0)

    def st(self, row, val):
        if val.dtype != u32:
            val = lax.bitcast_convert_type(val, u32)
        row += self.off
        self.a.sv[row:row + val.shape[0], :] = val

    def st_strided(self, row, val, stride):
        if val.dtype != u32:
            val = lax.bitcast_convert_type(val, u32)
        row += self.off
        self.a.sv[pl.ds(row, val.shape[0], stride=stride), :] = val

    def ld(self, row, n, dtype=f32):
        row += self.off
        v = self.a.lv[row:row + n, :]
        return v if dtype == u32 else lax.bitcast_convert_type(v, dtype)


def _kernel(x_hbm, wr_hbm, wi_hbm, wg_hbm, wu_hbm, wd_hbm, z_hbm,
            out_hbm,
            x_v, wr_v, wi_v, wg_v, wu_v, wd_v, fd_v, g_v, gs_v, bd_v, z_v, zb_v,
            Wtr, Wti, out_v, hn_v, eoe_v, eoo_v, hb1_v, hb2_v, sems, *arenas):
    cfg = CFG
    xch = cfg["xchunks"]
    xst = [sum(xch[:c]) for c in range(len(xch) + 1)]
    x_cp = [pltpu.make_async_copy(x_hbm.at[:, pl.ds(128 * xst[c], 128 * xch[c])],
                                  x_v.at[:, pl.ds(128 * xst[c], 128 * xch[c])], sems.at[c])
            for c in range(len(xch))]
    nx = len(xch)
    cp_z = pltpu.make_async_copy(z_hbm, z_v, sems.at[0])
    cp_wr = pltpu.make_async_copy(wr_hbm, wr_v, sems.at[nx])
    cp_wi = pltpu.make_async_copy(wi_hbm, wi_v, sems.at[nx + 1])
    cp_wg = pltpu.make_async_copy(wg_hbm, wg_v, sems.at[nx + 2])
    cp_wu = pltpu.make_async_copy(wu_hbm, wu_v, sems.at[nx + 2])
    cp_wd = pltpu.make_async_copy(wd_hbm, wd_v, sems.at[nx + 2])
    assert cfg["wd_early"]
    bars = [n for n in ("bar_f", "bar_g", "bar_h") if cfg[n]]
    cps = dict(z=cp_z, wr=cp_wr, wi=cp_wi, wg=cp_wg, wu=cp_wu, wd=cp_wd)
    for c in range(len(xch)):
        cps["x%d" % c] = x_cp[c]
    for k, n in enumerate(bars):
        cps[n] = pltpu.make_async_copy(z_hbm.at[pl.ds(0, 8)], zb_v.at[k], sems.at[nx + 4 + k])
    order = ["z"] + bars + ["x0"] + ["x%d" % c for c in range(1, len(xch))] + cfg["order"]

    del TRACE[:]
    TRACE.append(("order", order, list(xch)))
    for n in order:
        cps[n].start()

    def make_tables():
        i = lax.broadcasted_iota(jnp.int32, (8, 128), 0)
        c = lax.broadcasted_iota(jnp.int32, (8, 128), 1)
        f = _geom(_cis(i * c, 128), _cis(8 * c, 128), 16)
        t1 = _cis(c, S)
        t = t1
        for km in range(9):
            g = f
            if km:
                if km > 1:
                    t = _cmul(t, t1)
                g = [_cmul(e, t) for e in f]
            g_v[km, 0:64, :] = _pack_rows([e[0] for e in g])
            g_v[km, 64:128, :] = _pack_rows([e[1] for e in g])
            gs_v[km] = _pack_rows([e[0] + e[1] for e in g])
        dq = c
        b0, st0 = _cis(4 * i * dq, D), _cis(32 * dq, D)
        e0 = _geom(b0, st0, 7)
        e2 = _geom(_cmul(b0, _cis(2 * dq, D)), st0, 7)
        nyq = (1 - 2 * (dq & 1)).astype(f32)
        im0 = [jnp.where(i == 0, nyq, e0[0][1])] + [e[1] for e in e0[1:]]
        fd_v[0:56, :] = _pack_rows([e[0] for e in e0] + im0)
        fd_v[56:112, :] = _pack_rows([e[0] for e in e2] + [e[1] for e in e2])
        for kt in range(2):
            dd = dq + 128 * kt
            eo = _geom(_cis((2 * i + 1) * dd, D), _cis(16 * dd, D), 14)
            fd_v[112 + 112 * kt:224 + 112 * kt, :] = _pack_rows([e[0] for e in eo] + [e[1] for e in eo])
        sc = np.float32(1.0 / (D * S))
        for p in range(2):
            kd = 2 * c + p
            if p == 0:
                wgt = jnp.where((c == 0) | (c == DQ), sc, jnp.where(c < DQ, 2 * sc, np.float32(0)))
            else:
                wgt = jnp.where(c < DQ, 2 * sc, np.float32(0))
            base, step = _cis(kd * i, D), _cis(8 * kd, D)
            if p == 0:
                base = (base[0], jnp.where(c == DQ, np.float32(0), base[1]))
                step = (step[0], jnp.where(c == DQ, np.float32(0), step[1]))
            e = _geom((base[0] * wgt, base[1] * wgt), step, DH // 8)
            bd_v[p, 0] = _pack_rows([x[0] for x in e])
            bd_v[p, 1] = _pack_rows([x[1] for x in e])

    def wait(*names):
        TRACE.append(("wait", names))
        if cfg.get("scopes"):
            with jax.named_scope("wait_" + names[0]):
                for n in names:
                    cps[n].wait()
            return
        for n in names:
            cps[n].wait()

    import contextlib
    scope = (lambda n: jax.named_scope(n)) if cfg.get("scopes") == 2 else (lambda n: contextlib.nullcontext())
    with scope("ph_tables"):
        make_tables()
        zpad = jnp.zeros((16, 128), bf16)
        for a in range(NT):
            eoe_v[a * 256 + DQ:a * 256 + 128, :] = zpad
            eoe_v[a * 256 + 128 + DQ:a * 256 + 256, :] = zpad
            eoo_v[a * 256 + DH:a * 256 + DH + 16, :] = zpad
            eoo_v[a * 256 + DH + 16:a * 256 + 256, :] = zpad
    wait("z", "x0")
    groups, loc, _ = _layout()
    ars = [Arena(r, static=all(b in cfg["static"] for b in g)) for r, g in zip(arenas, groups)]
    bufs = {b: Buf(ars[gi], off) for b, (gi, off) in loc.items()}
    X1 = [bufs["X1E"], bufs["X1O"]]
    Yb = [bufs["YE"], bufs["YO"]]
    X2 = [bufs["X2E"], bufs["X2O"]]
    Vb = [bufs["VE"], bufs["VO"]]
    Zb = [bufs["ZE"], bufs["ZO"]]
    HE = bufs["HE"]

    def make_views():
        zz = z_v[0:16, :]
        z1 = pl.multiple_of(jnp.max(zz[0:8]), 8)
        z2 = pl.multiple_of(jnp.max(zz[8:16]), 8)
        for ar in ars:
            ar.bind(z1, z2)
    rstd = [None] * NT

    def ln1(a):
        if cfg.get("dbg_noln") and a < 15:
            return
        x = x_v[:, a * 128:(a + 1) * 128].astype(f32)
        a0 = []
        accd, acca = [None, None], [None, None]

        def acc(l, i, v):
            l[i] = v if l[i] is None else l[i] + v

        for j in range(DQ // 16):
            x0, x1, x2, x3 = (x[q * DQ + 16 * j:q * DQ + 16 * j + 16] for q in range(4))
            s02, s13 = x0 + x2, x1 + x3
            d02, d13 = x0 - x2, x1 - x3
            a0.append(s02 + s13)
            a2 = s02 - s13
            eoo_v[a * 256 + 16 * j:a * 256 + 16 * j + 16, :] = d02.astype(bf16)
            eoo_v[a * 256 + DQ + 16 * j:a * 256 + DQ + 16 * j + 16, :] = d13.astype(bf16)
            eoe_v[a * 256 + 128 + 16 * j:a * 256 + 128 + 16 * j + 16, :] = a2.astype(bf16)
            acc(accd, 0, d02 * d02)
            acc(accd, 1, d13 * d13)
            acc(acca, 0, a2 * a2)
        m4 = _colsum(jnp.concatenate(a0, axis=0)) * (4.0 / D)
        for j in range(DQ // 16):
            t = a0[j] - m4
            eoe_v[a * 256 + 16 * j:a * 256 + 16 * j + 16, :] = t.astype(bf16)
            acc(acca, 1, t * t)
        v = _colsum((accd[0] + accd[1]) * 2.0 + (acca[0] + acca[1])) * (0.25 / D)
        rstd[a] = lax.rsqrt(v + EPS)

    row0 = lax.broadcasted_iota(jnp.int32, (8, 128), 0) == 0

    def dftd_e(a, q):
        rhs = eoe_v[a * 256 + 128 * q:a * 256 + 128 * q + 128, :]
        r = jnp.dot(_bf(fd_v[56 * q:56 * q + 56, :]), rhs, preferred_element_type=f32) * rstd[a]
        for c in range(2):
            for v in range(7):
                t = r[56 * c + 8 * v:56 * c + 8 * v + 8]
                if q == 0 and c == 1 and v == 0:
                    X1[0].st(a * 256 + 112, jnp.where(row0, t, 0.0))
                    t = jnp.where(row0, 0.0, t)
                X1[0].st_strided(a * 256 + 128 * c + 16 * v + q, t, 2)

    def dftd_o(a):
        lhs = jnp.concatenate([_bf(fd_v[112:224, :]), _bf(fd_v[224:336, :])], axis=1)
        rhs = eoo_v[a * 256:a * 256 + 256, :]
        r = jnp.dot(lhs, rhs, preferred_element_type=f32) * rstd[a]
        X1[1].st(a * 256, r[:DQ])
        X1[1].st(a * 256 + 128, r[DQ:])

    def rad_fwd(p, j):
        r = 8 * j
        re = [X1[p].ld(a * 256 + r, 8) for a in range(16)]
        nyq = (p == 0 and j == 14)
        im = [None if nyq else X1[p].ld(a * 256 + 128 + r, 8) for a in range(16)]
        ore, oim = _fft16(re, im, -1)
        for k1 in range(16):
            Yb[p].st(k1 * 256 + r, ore[k1])
            Yb[p].st(k1 * 256 + 128 + r, oim[k1])

    def y_get(p, k1):
        n = 112 if p else 120
        z = jnp.zeros((128 - n, 128), f32)
        return (jnp.concatenate([Yb[p].ld(k1 * 256, n), z], axis=0),
                jnp.concatenate([Yb[p].ld(k1 * 256 + 128, n), z], axis=0))

    def gmat(k1):
        return (k1, 1) if k1 < 8 else (16 - k1, -1)

    def gparts(km):
        return _bf(g_v[km, 0:64, :]), _bf(g_v[km, 64:128, :]), _bf(gs_v[km])

    def cmul3(km, conj, a, b, dims):
        gr, gi, gs = gparts(km)
        t1 = lax.dot_general(gr, a.astype(bf16), dims, preferred_element_type=f32)
        t2 = lax.dot_general(gi, b.astype(bf16), dims, preferred_element_type=f32)
        if conj:
            t3 = lax.dot_general(gs, (b - a).astype(bf16), dims, preferred_element_type=f32)
            return t1 + t2, t3 + (t1 - t2)
        t3 = lax.dot_general(gs, (a + b).astype(bf16), dims, preferred_element_type=f32)
        return t1 - t2, t3 - (t1 + t2)

    def x2row(p, k1):
        return k1 * 256

    def dft128(p, k1):
        km, sg = gmat(k1)
        yr, yi = y_get(p, k1)
        xr, xi = cmul3(km, sg < 0, yr, yi, NT_DIMS)
        X2[p].st(x2row(p, k1), xr)
        X2[p].st(x2row(p, k1) + 128, xi)

    rows8 = lax.broadcasted_iota(jnp.int32, (8, 128), 0)

    def wprep(w_v, Wt, a):
        w32 = pltpu.bitcast(w_v[0:DH, a * 128:(a + 1) * 128], u32)
        ny = w_v[DH:DH + 1, a * 128:(a + 1) * 128].astype(f32)
        ny = jnp.broadcast_to(ny, (8, 128))
        nyu = lax.shift_right_logical(lax.bitcast_convert_type(ny, u32), np.uint32(16))
        nyu = jnp.where(rows8 == 0, nyu, np.uint32(0))
        t = jnp.concatenate([w32, nyu, jnp.zeros((8, 128), u32)], axis=0).T
        if cfg["w_f32"]:
            for p, tp in enumerate((_lo(t), _hi(t))):
                tp = lax.bitcast_convert_type(tp, u32)
                for j in range(8):
                    Wt[pl.ds(p * 16 * WP + a * WP + 17 * j, 8), :] = tp[16 * j:16 * j + 8, :]
                    Wt[pl.ds(p * 16 * WP + (15 - a) * WP + 17 * (7 - j) + 8, 8), :] = tp[16 * j + 8:16 * j + 16, :]
            return
        for j in range(8):
            Wt[pl.ds(a * WP + 17 * j, 8), :] = t[16 * j:16 * j + 8, :]
            Wt[pl.ds((15 - a) * WP + 17 * (7 - j) + 8, 8), :] = t[16 * j + 8:16 * j + 16, :]

    def idft128(p, k1, mid=None):
        km, sg = gmat(k1)
        if cfg["w_f32"]:
            o = p * 16 * WP + k1
            wr = jnp.concatenate([Wtr[pl.ds(o + A_ * WP, 8, stride=17), :] for A_ in range(16)], axis=0)
            wi = jnp.concatenate([Wti[pl.ds(o + A_ * WP, 8, stride=17), :] for A_ in range(16)], axis=0)
            wr, wi = lax.bitcast_convert_type(wr, f32), lax.bitcast_convert_type(wi, f32)
        else:
            wr32 = jnp.concatenate([Wtr[pl.ds(A_ * WP + k1, 8, stride=17), :] for A_ in range(16)], axis=0)
            wi32 = jnp.concatenate([Wti[pl.ds(A_ * WP + k1, 8, stride=17), :] for A_ in range(16)], axis=0)
            if p == 0:
                wr, wi = _lo(wr32), _lo(wi32)
            else:
                wr, wi = _hi(wr32), _hi(wi32)
        xr, xi = X2[p].ld(x2row(p, k1), 128), X2[p].ld(x2row(p, k1) + 128, 128)
        vr, vi = cmul3(km, sg > 0, xr * wr - xi * wi, xr * wi + xi * wr, TN_DIMS)
        if mid is not None:
            mid()
        Vb[p].st(k1 * 256, vr)
        Vb[p].st(k1 * 256 + 128, vi)

    def rad_inv(p, j):
        r = 8 * j
        re = [Vb[p].ld(k1 * 256 + r, 8) for k1 in range(16)]
        im = [Vb[p].ld(k1 * 256 + 128 + r, 8) for k1 in range(16)]
        ore, oim = _fft16(re, im, +1)
        for s1 in range(16):
            Zb[p].st(s1 * 256 + r, ore[s1])
            Zb[p].st(s1 * 256 + 128 + r, oim[s1])

    def idftd2(p, zb, t):
        z = jnp.concatenate([zb.ld(t * 256, 128), zb.ld(t * 256 + 128, 128)], axis=1).astype(bf16)
        lhs = jnp.concatenate([_bf(bd_v[p, 0]), _bf(bd_v[p, 1])], axis=1)
        return lax.dot_general(lhs, z, NT_DIMS, preferred_element_type=f32)

    def idftd(p, a):
        return idftd2(p, Zb[p], a)

    TPC = 2
    CW = TPC * 128

    def cols(c, t=0, n=CW):
        if isinstance(c, int):
            return pl.ds(c * CW + t * 128, n)
        return pl.ds(pl.multiple_of(c * CW, CW) + t * 128, n)

    def hrows(c, t, r=0, n=D):
        if isinstance(c, int):
            return pl.ds((c * TPC + t) * D + r, n)
        return pl.ds(pl.multiple_of(c * (TPC * D), 16) + (t * D + r), n)

    def prologue2(c, mem):
        zo, he = Zb[1].sub(c, TPC * 256), HE.sub(c, TPC * DH)
        ms, rs = [], []
        for t in range(TPC):
            O = idftd2(1, zo, t)
            E = he.ld(t * DH, DH)
            x = x_v[:, cols(c, t, 128)].astype(f32)
            acc = [None] * 4
            for j in range(DH // 16):
                e, o = E[16 * j:16 * j + 16], O[16 * j:16 * j + 16]
                for k, (r, v) in enumerate(((16 * j, e + o), (DH + 16 * j, e - o))):
                    hb = (x[r:r + 16] + v).astype(bf16)
                    hb1_v[hrows(c, t, r, 16), :] = hb
                    hb2_v[hrows(c, t, r, 16), :] = hb
                    i = (2 * j + k) % 4
                    hf = hb.astype(f32)
                    acc[i] = hf if acc[i] is None else acc[i] + hf
            ms.append(_colsum((acc[0] + acc[1]) + (acc[2] + acc[3])) * (1.0 / D))
        for t in range(TPC):
            acc = [None] * 4
            for j in range(D // 16):
                d = hb2_v[hrows(c, t, 16 * j, 16), :].astype(f32) - ms[t]
                acc[j % 4] = d * d if acc[j % 4] is None else acc[j % 4] + d * d
            v = _colsum((acc[0] + acc[1]) + (acc[2] + acc[3])) * (1.0 / D)
            rs.append(lax.rsqrt(v + EPS))
        hns = [(hb1_v[hrows(c, t), :].astype(f32) - ms[t]) * rs[t] for t in range(TPC)]
        hn = jnp.concatenate(hns, axis=1).astype(bf16)
        if mem:
            hn_v[:, cols(c)] = hn
            return None
        return None, hn

    def prologue(c, mem):
        if cfg["ln2"] == 1:
            return prologue2(c, mem)
        zo, he = Zb[1].sub(c, TPC * 256), HE.sub(c, TPC * DH)
        hs, hns = [], []
        for t in range(TPC):
            O = idftd2(1, zo, t)
            E = he.ld(t * DH, DH)
            y = jnp.concatenate([E + O, E - O], axis=0)
            hb = (x_v[:, cols(c, t, 128)].astype(f32) + y).astype(bf16)
            hf = hb.astype(f32)
            m = _colsum(hf) * (1.0 / D)
            hc = hf - m
            v = _colsum(hc * hc) * (1.0 / D)
            hs.append(hf)
            hns.append(hc * lax.rsqrt(v + EPS))
            if mem:
                out_v[:, cols(c, t, 128)] = hb
        hn = jnp.concatenate(hns, axis=1).astype(bf16)
        if mem:
            hn_v[:, cols(c)] = hn
            return None
        return jnp.concatenate(hs, axis=1), hn

    def rows(c):
        if isinstance(c, int):
            return pl.ds(c * CW, CW)
        return pl.ds(pl.multiple_of(c * CW, CW), CW)

    def out_copy(c, t=None):
        if t is None:
            return pltpu.make_async_copy(out_v.at[:, cols(c)], out_hbm.at[:, cols(c)], sems.at[nx + 3])
        return pltpu.make_async_copy(out_v.at[:, cols(c, t, 128)], out_hbm.at[:, cols(c, t, 128)], sems.at[nx + 3])

    def mlp(c, cur, nxt_fn=None, wd_wait=False):
        hnT = hn_v[:, cols(c)] if cur is None else cur[1]
        nxt = nxt_fn() if nxt_fn is not None else None
        g = lax.dot_general(hnT, wg_v[...], TN_DIMS, preferred_element_type=f32)
        u = lax.dot_general(hnT, wu_v[...], TN_DIMS, preferred_element_type=f32)
        hh = (g * u).astype(bf16)
        if wd_wait is True:
            wait("wd")
        elif wd_wait is not False:
            @pl.when(wd_wait)
            def _():
                wait("wd")
        if cfg["down_split"]:
            for t in range(TPC):
                mlp = lax.dot_general(wd_v[...], hh[t * 128:(t + 1) * 128], NT_DIMS, preferred_element_type=f32)
                if cfg["ln2"] == 1:
                    h = hb1_v[hrows(c, t), :].astype(f32)
                else:
                    h = out_v[:, cols(c, t, 128)].astype(f32) if cur is None else cur[0][:, t * 128:(t + 1) * 128]
                out_v[:, cols(c, t, 128)] = (h + mlp.astype(bf16).astype(f32)).astype(bf16)
                if cfg["down_split"] == 2:
                    out_copy(c, t).start()
            if cfg["down_split"] == 1:
                out_copy(c).start()
            return nxt
        mlp = lax.dot_general(wd_v[...], hh, NT_DIMS, preferred_element_type=f32)
        h = out_v[:, cols(c)].astype(f32) if cur is None else cur[0]
        out_v[:, cols(c)] = (h + mlp.astype(bf16).astype(f32)).astype(bf16)
        out_copy(c).start()
        return nxt

    def fwd_tile(a):
        if cfg.get("dbg_nofwd") and a < 15:
            return
        if a % 2 == 0:
            dftd_e(a, 0)
            dftd_e(a, 1)
            dftd_o(a)
        else:
            dftd_o(a)
            dftd_e(a, 0)
            dftd_e(a, 1)

    make_views()
    with scope("ph_fwd"):
        ln1(0)
        for a in range(1, NT):
            if a in xst:
                wait("x%d" % xst.index(a))
            fwd_tile(a - 1)
            ln1(a)
        fwd_tile(NT - 1)
    if cfg.get("dbg_stop") == 1:
        for n in order:
            if not (n[0] == "x" or n == "z"):
                wait(n)
        out_v[0:8, 0:128] = X1[0].ld(15 * 256, 8).astype(bf16) + X1[1].ld(15 * 256, 8).astype(bf16)
        cp = pltpu.make_async_copy(out_v.at[:, pl.ds(0, 128)], out_hbm.at[:, pl.ds(0, 128)], osems.at[0])
        cp.start()
        cp.wait()
        return
    for j in range(15):
        rad_fwd(0, j)
    wait("wr")
    def spread(k, k0, n, total, fn):
        if k0 <= k < k0 + n:
            for a in range(total * (k - k0) // n, total * (k - k0 + 1) // n):
                fn(a)

    j = 0
    wr0, wrn = cfg["wr_prep"]
    wi0, win = cfg["wi_prep"]
    for q in range(32):
        if q == cfg["wi_wait"]:
            wait("wi")
        dft128(q // 16, q % 16)
        if q >= cfg["ro_at"] and j < 14:
            rad_fwd(1, j)
            j += 1
        spread(q, wr0, wrn, 16, lambda a: wprep(wr_v, Wtr, a))
        spread(q, wi0, win, 16, lambda a: wprep(wi_v, Wti, a))
    assert j == 14 and cfg["ro_at"] <= 2 and wi0 >= cfg["wi_wait"]
    if cfg["bar_f"]:
        wait("bar_f")
    for k1 in range(16):
        idft128(0, k1)
    if cfg["bar_g"]:
        wait("bar_g")
    j = 0
    ne = cfg["h_early"]

    def early_h():
        for a in range(ne):
            HE.st(a * DH, idftd(0, a))

    for k1 in range(16):
        idft128(1, k1, early_h if (k1 == 15 and ne) else None)
        for _ in range(cfg["ge_per"] if k1 >= cfg["ge_at"] else 0):
            if j < 16:
                rad_inv(0, j)
                j += 1
    while j < 16:
        rad_inv(0, j)
        j += 1
    if cfg["bar_h"]:
        wait("bar_h")
    j = 0
    loop = cfg["mlp_loop"]
    mem = loop > 0 or cfg["mlp_mem"]
    state = {"done": False}

    def first_prologue():
        state["nxt"] = prologue(0, mem)
        if loop == 3:
            for c in range(cfg["mlp_unroll"], cfg["nmlp"], cfg["mlp_unroll"]):
                prologue(c, True)
        state["done"] = True

    for a in range(ne, 16):
        if a == cfg["wgwu_at"]:
            wait("wg", "wu", *(("wd",) if cfg["wd_early"] else ()))
        if a == cfg["pro_at"]:
            while j < 16:
                rad_inv(1, j)
                j += 1
            first_prologue()
        HE.st(a * DH, idftd(0, a))
        for _ in range(cfg["go_per"] if a >= cfg["go_at"] else 0):
            if j < 16:
                rad_inv(1, j)
                j += 1
    while j < 16:
        rad_inv(1, j)
        j += 1
    if not state["done"]:
        first_prologue()
    NC = cfg["nmlp"]
    if cfg["wgwu_at"] >= 16:
        wait("wg", "wu", *(("wd",) if cfg["wd_early"] else ()))
    if loop == 0:
        cur = state["nxt"]
        for c in range(NC):
            fn = (lambda c=c: prologue(c + 1, mem)) if c + 1 < NC else None
            cur = mlp(c, cur, fn, wd_wait=(c == 0 and not cfg["wd_early"]))
    else:
        U = cfg["mlp_unroll"]
        if loop == 3:
            assert NC % U == 0

            def body(i, carry):
                cur = None
                for k in range(U):
                    c = i * U + k
                    fn = (lambda c=c: prologue(c + 1, False)) if k < U - 1 else None
                    cur = mlp(c, cur, fn, wd_wait=(i == 0) if (k == 0 and not cfg["wd_early"]) else False)
                return carry

            with scope("ph_loop"):
                lax.fori_loop(0, NC // U, body, 0)
        elif loop == 1:
            assert NC % U == 0

            def body(i, carry):
                cur = None
                for k in range(U):
                    c = i * U + k
                    cn = jnp.minimum(c + 1, NC - 1) if k == U - 1 else c + 1
                    cur = mlp(c, cur, lambda: prologue(cn, k == U - 1 or not cfg["loop_ssa"]))
                return carry

            lax.fori_loop(0, NC // U, body, 0)
        else:
            peel = cfg["mlp_peel"]
            for c in range(peel):
                mlp(c, None, lambda c=c: prologue(c + 1, True))
            assert (NC - peel) % U == 0

            def body(i, carry):
                for k in range(U):
                    c = peel + i * U + k
                    cn = jnp.minimum(c + 1, NC - 1) if k == U - 1 else c + 1
                    mlp(c, None, lambda: prologue(cn, True))
                return carry

            lax.fori_loop(0, (NC - peel) // U, body, 0)
    pltpu.make_async_copy(out_v, out_hbm, sems.at[nx + 3]).wait()


@jax.jit
def pallas_sequential_preLN__spectral_gfnet__glu_gated_bilinear__prompt_kernel(
    A_x: jax.Array,
    A_w_r: jax.Array,
    A_w_i: jax.Array,
    B_x: jax.Array,
    B_w_gate: jax.Array,
    B_w_up: jax.Array,
    B_w_down: jax.Array,
):
    del B_x
    zc = np.zeros((24, 128), np.int32)
    zc[16:] = np.arange(128)
    xT = A_x.reshape(S, D).T
    any_spec = pl.BlockSpec(memory_space=pl.ANY)
    outT = pl.pallas_call(
        _kernel,
        out_shape=jax.ShapeDtypeStruct((D, S), bf16),
        in_specs=[any_spec] * 7,
        out_specs=any_spec,
        scratch_shapes=[
            pltpu.VMEM((D, S), bf16),
            pltpu.VMEM((DH + 1, S), bf16),
            pltpu.VMEM((DH + 1, S), bf16),
            pltpu.VMEM((D, F), bf16),
            pltpu.VMEM((D, F), bf16),
            pltpu.VMEM((D, F), bf16),
            pltpu.VMEM((FD_ROWS, 128), u32),
            pltpu.VMEM((9, 128, 128), u32),
            pltpu.VMEM((9, 64, 128), u32),
            pltpu.VMEM((2, 2, DH // 2, 128), u32),
            pltpu.VMEM((24, 128), jnp.int32),
            pltpu.VMEM((3, 8, 128), jnp.int32),
            pltpu.VMEM(((2 if CFG["w_f32"] else 1) * 16 * WP, 128), u32),
            pltpu.VMEM(((2 if CFG["w_f32"] else 1) * 16 * WP, 128), u32),
            pltpu.VMEM((D, S), bf16),
            pltpu.VMEM((D, S), bf16),
            pltpu.VMEM((NT * 256, 128), bf16),
            pltpu.VMEM((NT * 256, 128), bf16),
            pltpu.VMEM((NT * D, 128), bf16),
            pltpu.VMEM((NT * D, 128), bf16),
            pltpu.SemaphoreType.DMA((len(CFG["xchunks"]) + 4 + sum(bool(CFG[n]) for n in ("bar_f", "bar_g", "bar_h")),)),
        ] + [pltpu.VMEM((n, 128), u32) for n in _layout()[2]],
        compiler_params=pltpu.CompilerParams(vmem_limit_bytes=100 * 2**20),
        name="gfnet_glu",
    )(xT, A_w_r.T, A_w_i.T, B_w_gate, B_w_up, B_w_down.T, zc)
    return outT.T.reshape(1, S, D)
```

```python
import numpy as np
import jax
import jax.numpy as jnp
from jax import lax
from jax.experimental import pallas as pl
from jax.experimental.pallas import tpu as pltpu

S, D, F = 2048, 448, 1792
DH = D // 2
NT = S // 128
EPS = 1e-5
bf16 = jnp.bfloat16
f32 = jnp.float32
u32 = jnp.uint32
NT_DIMS = (((1,), (1,)), ((), ()))
TN_DIMS = (((0,), (0,)), ((), ()))
WP = 136

CFG = dict(xchunks=(4, 4, 4, 4), ro_per=1, ge_per=2, go_per=1, pro_at=16, tpc=2, nmlp=8,
           groups=[["YE", "YO"], ["ZE", "ZO"]], static=[], ln_first=0,
           order=["wr", "wi", "wg", "wu", "wd"], re_at=0, ro_at=0, ge_at=0, go_at=0, wr_prep=(16, 8), wi_prep=(24, 8), wi_wait=24, h_early=0, bar_f=0, bar_g=0, bar_h=0, w_f32=0, ln2=0, g_barrier=0, m_c=16, gec_per=2, gec_max=16, mlp_loop=0, pre_t=0, down_split=0, loop_ssa=1, mlp_unroll=1, mlp_peel=2, mlp_mem=0, wd_early=0, wr_at=16, wi_at=8, bd_early=0, wgwu_at=16)
CFG.update(OPQ)
BUFS = dict(X1E=4096, X1O=4096, YE=4096, YO=4096, X2E=4096, X2O=4096,
            VE=4096, VO=4096, ZE=4096, ZO=4096, HE=NT * DH)


TRACE = []


def _layout():
    groups = [list(g) for g in CFG["groups"]]
    used = {b for g in groups for b in g}
    groups += [[b] for b in BUFS if b not in used]
    loc, sizes = {}, []
    for gi, g in enumerate(groups):
        off = 0
        for b in g:
            loc[b] = (gi, off)
            off += BUFS[b]
        sizes.append(off)
    return groups, loc, sizes


DQ = D // 4
FD_ROWS = 112 + 112 + 2 * 224


def _cis(n, period):
    nf = n.astype(f32)
    r = nf - jnp.floor(nf * np.float32(1.0 / period) + 0.5) * np.float32(period)
    ang = r * np.float32(2 * np.pi / period)
    return jnp.cos(ang), -jnp.sin(ang)


def _cmul(a, b):
    return a[0] * b[0] - a[1] * b[1], a[0] * b[1] + a[1] * b[0]


def _geom(base, step, n):
    out = [base]
    for _ in range(n - 1):
        out.append(_cmul(out[-1], step))
    return out


def _pack_rows(vregs):
    return jnp.concatenate(vregs, axis=0).astype(bf16)


def _ldw(ref, row, n):
    return pltpu.bitcast(ref.bitcast(u32)[row // 2:(row + n) // 2, :], bf16)


class V:
    __slots__ = ("a", "n")

    def __init__(self, a, n=False):
        self.a, self.n = a, n

    def __neg__(self):
        return V(self.a, not self.n)

    def __add__(self, o):
        if o.a is None:
            return self
        if self.a is None:
            return o
        if not self.n and not o.n:
            return V(self.a + o.a)
        if not self.n and o.n:
            return V(self.a - o.a)
        if self.n and not o.n:
            return V(o.a - self.a)
        return V(self.a + o.a, True)

    def __sub__(self, o):
        return self + (-o)

    def mul(self, c):
        if self.a is None:
            return self
        return V(self.a * np.float32(-c if self.n else c))

    def val(self, like):
        if self.a is None:
            return jnp.zeros_like(like)
        return -self.a if self.n else self.a


def _r4(x, sg):
    (x0r, x0i), (x1r, x1i), (x2r, x2i), (x3r, x3i) = x
    t0r, t0i = x0r + x2r, x0i + x2i
    t1r, t1i = x0r - x2r, x0i - x2i
    t2r, t2i = x1r + x3r, x1i + x3i
    t3r, t3i = x1r - x3r, x1i - x3i
    if sg > 0:
        ur, ui = -t3i, t3r
    else:
        ur, ui = t3i, -t3r
    return [(t0r + t2r, t0i + t2i), (t1r + ur, t1i + ui), (t0r - t2r, t0i - t2i), (t1r - ur, t1i - ui)]


def _tw(x, e, sg):
    xr, xi = x
    e = e % 16
    if e % 4 == 0:
        q = ((e // 4) if sg > 0 else (-(e // 4))) % 4
        if q == 0:
            return xr, xi
        if q == 1:
            return -xi, xr
        if q == 2:
            return -xr, -xi
        return xi, -xr
    c, s = np.cos(2 * np.pi * e / 16), sg * np.sin(2 * np.pi * e / 16)
    if e % 2 == 0:
        h = abs(c)
        a = xr if c > 0 else -xr
        b = xi if s > 0 else -xi
        re = (a - b).mul(h)
        a = xi if c > 0 else -xi
        b = xr if s > 0 else -xr
        im = (a + b).mul(h)
        return re, im
    return xr.mul(c) - xi.mul(s), xi.mul(c) + xr.mul(s)


def _fft16(re, im, sg):
    x = [(V(re[a]), V(im[a])) for a in range(16)]
    T = [_r4([x[4 * a1 + a0] for a1 in range(4)], sg) for a0 in range(4)]
    out_re, out_im = [None] * 16, [None] * 16
    for k0 in range(4):
        col = [_tw(T[a0][k0], a0 * k0, sg) for a0 in range(4)]
        y = _r4(col, sg)
        for k1 in range(4):
            out_re[k0 + 4 * k1] = y[k1][0].val(re[0])
            out_im[k0 + 4 * k1] = y[k1][1].val(re[0])
    return out_re, out_im


def _colsum(x):
    parts = [x[i:i + 8] for i in range(0, x.shape[0], 8)]
    while len(parts) > 1:
        nxt = [parts[i] + parts[i + 1] for i in range(0, len(parts) - 1, 2)]
        if len(parts) % 2:
            nxt.append(parts[-1])
        parts = nxt
    return jnp.sum(parts[0], axis=0, keepdims=True)


def _deilv16(x):
    a = jnp.concatenate([x[32 * j:32 * j + 16] for j in range(8)], axis=0)
    b = jnp.concatenate([x[32 * j + 16:32 * j + 32] for j in range(8)], axis=0)
    return a, b


def _lo(w):
    return lax.bitcast_convert_type(lax.shift_left(w, np.uint32(16)), f32)


def _hi(w):
    return lax.bitcast_convert_type(w & np.uint32(0xFFFF0000), f32)


def _bf(x):
    return pltpu.bitcast(x, bf16)


class Arena:
    def __init__(self, ref, static=False):
        self.ref, self.static = ref, static
        self.sv = self.lv = ref if static else None

    def bind(self, zs, zl):
        self.zs, self.zl = zs, zl
        if not self.static:
            n = self.ref.shape[0]
            self.sv = self.ref.at[pl.ds(zs, n)]
            self.lv = self.ref.at[pl.ds(zl, n)]


class Buf:
    def __init__(self, arena, off):
        self.a, self.off = arena, off

    def sub(self, c, n):
        if isinstance(c, int):
            return Buf(self.a, self.off + c * n)
        ar = Arena(self.a.ref)
        base = pl.multiple_of(self.off + c * n, 8)
        ar.sv = self.a.ref.at[pl.ds(self.a.zs + base, n)]
        ar.lv = self.a.ref.at[pl.ds(self.a.zl + base, n)]
        return Buf(ar, 0)

    def st(self, row, val):
        if val.dtype != u32:
            val = lax.bitcast_convert_type(val, u32)
        row += self.off
        self.a.sv[row:row + val.shape[0], :] = val

    def st_strided(self, row, val, stride):
        if val.dtype != u32:
            val = lax.bitcast_convert_type(val, u32)
        row += self.off
        self.a.sv[pl.ds(row, val.shape[0], stride=stride), :] = val

    def ld(self, row, n, dtype=f32):
        row += self.off
        v = self.a.lv[row:row + n, :]
        return v if dtype == u32 else lax.bitcast_convert_type(v, dtype)


def _kernel(x_hbm, wr_hbm, wi_hbm, wg_hbm, wu_hbm, wd_hbm, z_hbm,
            out_hbm,
            x_v, wr_v, wi_v, wg_v, wu_v, wd_v, fd_v, g_v, bd_v, z_v, zb_v,
            Wtr, Wti, out_v, hn_v, eoe_v, eoo_v, hb1_v, hb2_v, sems, *arenas):
    cfg = CFG
    xch = cfg["xchunks"]
    xst = [sum(xch[:c]) for c in range(len(xch) + 1)]
    x_cp = [pltpu.make_async_copy(x_hbm.at[:, pl.ds(128 * xst[c], 128 * xch[c])],
                                  x_v.at[:, pl.ds(128 * xst[c], 128 * xch[c])], sems.at[c])
            for c in range(len(xch))]
    nx = len(xch)
    cp_z = pltpu.make_async_copy(z_hbm, z_v, sems.at[0])
    cp_wr = pltpu.make_async_copy(wr_hbm, wr_v, sems.at[nx])
    cp_wi = pltpu.make_async_copy(wi_hbm, wi_v, sems.at[nx + 1])
    cp_wg = pltpu.make_async_copy(wg_hbm, wg_v, sems.at[nx + 2])
    cp_wu = pltpu.make_async_copy(wu_hbm, wu_v, sems.at[nx + 2])
    cp_wd = pltpu.make_async_copy(wd_hbm, wd_v, sems.at[nx + 2])
    assert cfg["wd_early"]
    bars = [n for n in ("bar_f", "bar_g", "bar_h") if cfg[n]]
    cps = dict(z=cp_z, wr=cp_wr, wi=cp_wi, wg=cp_wg, wu=cp_wu, wd=cp_wd)
    for c in range(len(xch)):
        cps["x%d" % c] = x_cp[c]
    for k, n in enumerate(bars):
        cps[n] = pltpu.make_async_copy(z_hbm.at[pl.ds(0, 8)], zb_v.at[k], sems.at[nx + 4 + k])
    order = ["z"] + bars + ["x0"] + ["x%d" % c for c in range(1, len(xch))] + cfg["order"]

    del TRACE[:]
    TRACE.append(("order", order, list(xch)))
    for n in order:
        cps[n].start()

    def make_tables():
        i = lax.broadcasted_iota(jnp.int32, (8, 128), 0)
        c = lax.broadcasted_iota(jnp.int32, (8, 128), 1)
        f = _geom(_cis(i * c, 128), _cis(8 * c, 128), 16)
        t1 = _cis(c, S)
        t = t1
        for km in range(9):
            g = f
            if km:
                if km > 1:
                    t = _cmul(t, t1)
                g = [_cmul(e, t) for e in f]
            g_v[km * 384:km * 384 + 128, :] = _pack_rows([e[0] for e in g])
            g_v[km * 384 + 128:km * 384 + 256, :] = _pack_rows([e[1] for e in g])
            g_v[km * 384 + 256:km * 384 + 384, :] = _pack_rows([e[0] + e[1] for e in g])
        dq = c
        b0, st0 = _cis(4 * i * dq, D), _cis(32 * dq, D)
        e0 = _geom(b0, st0, 7)
        e2 = _geom(_cmul(b0, _cis(2 * dq, D)), st0, 7)
        nyq = (1 - 2 * (dq & 1)).astype(f32)
        im0 = [jnp.where(i == 0, nyq, e0[0][1])] + [e[1] for e in e0[1:]]
        fd_v[0:112, :] = _pack_rows([e[0] for e in e0] + im0)
        fd_v[112:224, :] = _pack_rows([e[0] for e in e2] + [e[1] for e in e2])
        for kt in range(2):
            dd = dq + 128 * kt
            eo = _geom(_cis((2 * i + 1) * dd, D), _cis(16 * dd, D), 14)
            fd_v[224 + 224 * kt:448 + 224 * kt, :] = _pack_rows([e[0] for e in eo] + [e[1] for e in eo])
        sc = np.float32(1.0 / (D * S))
        for p in range(2):
            kd = 2 * c + p
            if p == 0:
                wgt = jnp.where((c == 0) | (c == DQ), sc, jnp.where(c < DQ, 2 * sc, np.float32(0)))
            else:
                wgt = jnp.where(c < DQ, 2 * sc, np.float32(0))
            base, step = _cis(kd * i, D), _cis(8 * kd, D)
            if p == 0:
                base = (base[0], jnp.where(c == DQ, np.float32(0), base[1]))
                step = (step[0], jnp.where(c == DQ, np.float32(0), step[1]))
            e = _geom((base[0] * wgt, base[1] * wgt), step, DH // 8)
            bd_v[p * 448:p * 448 + DH, :] = _pack_rows([x[0] for x in e])
            bd_v[p * 448 + DH:p * 448 + 448, :] = _pack_rows([x[1] for x in e])

    def wait(*names):
        TRACE.append(("wait", names))
        if cfg.get("scopes"):
            with jax.named_scope("wait_" + names[0]):
                for n in names:
                    cps[n].wait()
            return
        for n in names:
            cps[n].wait()

    import contextlib
    scope = (lambda n: jax.named_scope(n)) if cfg.get("scopes") == 2 else (lambda n: contextlib.nullcontext())
    with scope("ph_tables"):
        make_tables()
        zpad = jnp.zeros((16, 128), bf16)
        for a in range(NT):
            eoe_v[a * 256 + DQ:a * 256 + 128, :] = zpad
            eoe_v[a * 256 + 128 + DQ:a * 256 + 256, :] = zpad
            eoo_v[a * 256 + DH:a * 256 + DH + 16, :] = zpad
            eoo_v[a * 256 + DH + 16:a * 256 + 256, :] = zpad
    wait("z", "x0")
    groups, loc, _ = _layout()
    ars = [Arena(r, static=all(b in cfg["static"] for b in g)) for r, g in zip(arenas, groups)]
    bufs = {b: Buf(ars[gi], off) for b, (gi, off) in loc.items()}
    X1 = [bufs["X1E"], bufs["X1O"]]
    Yb = [bufs["YE"], bufs["YO"]]
    X2 = [bufs["X2E"], bufs["X2O"]]
    Vb = [bufs["VE"], bufs["VO"]]
    Zb = [bufs["ZE"], bufs["ZO"]]
    HE = bufs["HE"]

    def make_views():
        zz = z_v[0:16, :]
        z1 = pl.multiple_of(jnp.max(zz[0:8]), 8)
        z2 = pl.multiple_of(jnp.max(zz[8:16]), 8)
        for ar in ars:
            ar.bind(z1, z2)
    rstd = [None] * NT

    def ln1(a):
        if cfg.get("dbg_noln") and a < 15:
            return
        x = x_v[:, a * 128:(a + 1) * 128].astype(f32)
        a0 = []
        accd, acca = [None, None], [None, None]

        def acc(l, i, v):
            l[i] = v if l[i] is None else l[i] + v

        for j in range(DQ // 16):
            x0, x1, x2, x3 = (x[q * DQ + 16 * j:q * DQ + 16 * j + 16] for q in range(4))
            s02, s13 = x0 + x2, x1 + x3
            d02, d13 = x0 - x2, x1 - x3
            a0.append(s02 + s13)
            a2 = s02 - s13
            eoo_v[a * 256 + 16 * j:a * 256 + 16 * j + 16, :] = d02.astype(bf16)
            eoo_v[a * 256 + DQ + 16 * j:a * 256 + DQ + 16 * j + 16, :] = d13.astype(bf16)
            eoe_v[a * 256 + 128 + 16 * j:a * 256 + 128 + 16 * j + 16, :] = a2.astype(bf16)
            acc(accd, 0, d02 * d02)
            acc(accd, 1, d13 * d13)
            acc(acca, 0, a2 * a2)
        m4 = _colsum(jnp.concatenate(a0, axis=0)) * (4.0 / D)
        for j in range(DQ // 16):
            t = a0[j] - m4
            eoe_v[a * 256 + 16 * j:a * 256 + 16 * j + 16, :] = t.astype(bf16)
            acc(acca, 1, t * t)
        v = _colsum((accd[0] + accd[1]) * 2.0 + (acca[0] + acca[1])) * (0.25 / D)
        rstd[a] = lax.rsqrt(v + EPS)

    row0 = lax.broadcasted_iota(jnp.int32, (8, 128), 0) == 0

    def dftd_e(a, q):
        rhs = _ldw(eoe_v, a * 256 + 128 * q, 128)
        r = jnp.dot(_ldw(fd_v, 112 * q, 112), rhs, preferred_element_type=f32) * rstd[a]
        for c in range(2):
            for v in range(7):
                t = r[56 * c + 8 * v:56 * c + 8 * v + 8]
                if q == 0 and c == 1 and v == 0:
                    X1[0].st(a * 256 + 112, jnp.where(row0, t, 0.0))
                    t = jnp.where(row0, 0.0, t)
                X1[0].st_strided(a * 256 + 128 * c + 16 * v + q, t, 2)

    def dftd_o(a):
        lhs = jnp.concatenate([_ldw(fd_v, 224, 224), _ldw(fd_v, 448, 224)], axis=1)
        rhs = _ldw(eoo_v, a * 256, 256)
        r = jnp.dot(lhs, rhs, preferred_element_type=f32) * rstd[a]
        X1[1].st(a * 256, r[:DQ])
        X1[1].st(a * 256 + 128, r[DQ:])

    def rad_fwd(p, j):
        r = 8 * j
        re = [X1[p].ld(a * 256 + r, 8) for a in range(16)]
        nyq = (p == 0 and j == 14)
        im = [None if nyq else X1[p].ld(a * 256 + 128 + r, 8) for a in range(16)]
        ore, oim = _fft16(re, im, -1)
        for k1 in range(16):
            Yb[p].st(k1 * 256 + r, ore[k1])
            Yb[p].st(k1 * 256 + 128 + r, oim[k1])

    def y_get(p, k1):
        n = 112 if p else 120
        z = jnp.zeros((128 - n, 128), f32)
        return (jnp.concatenate([Yb[p].ld(k1 * 256, n), z], axis=0),
                jnp.concatenate([Yb[p].ld(k1 * 256 + 128, n), z], axis=0))

    def gmat(k1):
        return (k1, 1) if k1 < 8 else (16 - k1, -1)

    def gparts(km):
        return tuple(_ldw(g_v, km * 384 + 128 * k, 128) for k in range(3))

    def cmul3(km, conj, a, b, dims):
        gr, gi, gs = gparts(km)
        t1 = lax.dot_general(gr, a.astype(bf16), dims, preferred_element_type=f32)
        t2 = lax.dot_general(gi, b.astype(bf16), dims, preferred_element_type=f32)
        if conj:
            t3 = lax.dot_general(gs, (b - a).astype(bf16), dims, preferred_element_type=f32)
            return t1 + t2, t3 + (t1 - t2)
        t3 = lax.dot_general(gs, (a + b).astype(bf16), dims, preferred_element_type=f32)
        return t1 - t2, t3 - (t1 + t2)

    def x2row(p, k1):
        return k1 * 256

    def dft128(p, k1):
        km, sg = gmat(k1)
        yr, yi = y_get(p, k1)
        xr, xi = cmul3(km, sg < 0, yr, yi, NT_DIMS)
        X2[p].st(x2row(p, k1), xr)
        X2[p].st(x2row(p, k1) + 128, xi)

    rows8 = lax.broadcasted_iota(jnp.int32, (8, 128), 0)

    def wprep(w_v, Wt, a):
        w32 = pltpu.bitcast(w_v[0:DH, a * 128:(a + 1) * 128], u32)
        ny = w_v[DH:DH + 1, a * 128:(a + 1) * 128].astype(f32)
        ny = jnp.broadcast_to(ny, (8, 128))
        nyu = lax.shift_right_logical(lax.bitcast_convert_type(ny, u32), np.uint32(16))
        nyu = jnp.where(rows8 == 0, nyu, np.uint32(0))
        t = jnp.concatenate([w32, nyu, jnp.zeros((8, 128), u32)], axis=0).T
        if cfg["w_f32"]:
            for p, tp in enumerate((_lo(t), _hi(t))):
                tp = lax.bitcast_convert_type(tp, u32)
                for j in range(8):
                    Wt[pl.ds(p * 16 * WP + a * WP + 17 * j, 8), :] = tp[16 * j:16 * j + 8, :]
                    Wt[pl.ds(p * 16 * WP + (15 - a) * WP + 17 * (7 - j) + 8, 8), :] = tp[16 * j + 8:16 * j + 16, :]
            return
        for j in range(8):
            Wt[pl.ds(a * WP + 17 * j, 8), :] = t[16 * j:16 * j + 8, :]
            Wt[pl.ds((15 - a) * WP + 17 * (7 - j) + 8, 8), :] = t[16 * j + 8:16 * j + 16, :]

    def idft128(p, k1, mid=None):
        km, sg = gmat(k1)
        if cfg["w_f32"]:
            o = p * 16 * WP + k1
            wr = jnp.concatenate([Wtr[pl.ds(o + A_ * WP, 8, stride=17), :] for A_ in range(16)], axis=0)
            wi = jnp.concatenate([Wti[pl.ds(o + A_ * WP, 8, stride=17), :] for A_ in range(16)], axis=0)
            wr, wi = lax.bitcast_convert_type(wr, f32), lax.bitcast_convert_type(wi, f32)
        else:
            wr32 = jnp.concatenate([Wtr[pl.ds(A_ * WP + k1, 8, stride=17), :] for A_ in range(16)], axis=0)
            wi32 = jnp.concatenate([Wti[pl.ds(A_ * WP + k1, 8, stride=17), :] for A_ in range(16)], axis=0)
            if p == 0:
                wr, wi = _lo(wr32), _lo(wi32)
            else:
                wr, wi = _hi(wr32), _hi(wi32)
        xr, xi = X2[p].ld(x2row(p, k1), 128), X2[p].ld(x2row(p, k1) + 128, 128)
        vr, vi = cmul3(km, sg > 0, xr * wr - xi * wi, xr * wi + xi * wr, TN_DIMS)
        if mid is not None:
            mid()
        Vb[p].st(k1 * 256, vr)
        Vb[p].st(k1 * 256 + 128, vi)

    def rad_inv(p, j):
        r = 8 * j
        re = [Vb[p].ld(k1 * 256 + r, 8) for k1 in range(16)]
        im = [Vb[p].ld(k1 * 256 + 128 + r, 8) for k1 in range(16)]
        ore, oim = _fft16(re, im, +1)
        for s1 in range(16):
            Zb[p].st(s1 * 256 + r, ore[s1])
            Zb[p].st(s1 * 256 + 128 + r, oim[s1])

    def idftd2(p, zb, t):
        z = jnp.concatenate([zb.ld(t * 256, 128), zb.ld(t * 256 + 128, 128)], axis=1).astype(bf16)
        lhs = jnp.concatenate([_ldw(bd_v, p * 448, DH), _ldw(bd_v, p * 448 + DH, DH)], axis=1)
        return lax.dot_general(lhs, z, NT_DIMS, preferred_element_type=f32)

    def idftd(p, a):
        return idftd2(p, Zb[p], a)

    TPC = 2
    CW = TPC * 128

    def cols(c, t=0, n=CW):
        if isinstance(c, int):
            return pl.ds(c * CW + t * 128, n)
        return pl.ds(pl.multiple_of(c * CW, CW) + t * 128, n)

    def hrows(c, t, r=0, n=D):
        if isinstance(c, int):
            return pl.ds((c * TPC + t) * D + r, n)
        return pl.ds(pl.multiple_of(c * (TPC * D), 16) + (t * D + r), n)

    def h_ld(ref, c, t, r, n):
        if isinstance(c, int):
            return _ldw(ref, (c * TPC + t) * D + r, n).astype(f32)
        base = pl.multiple_of(c * (TPC * D // 2), 8)
        w = ref.bitcast(u32)[pl.ds(base + (t * D + r) // 2, n // 2), :]
        return pltpu.bitcast(w, bf16).astype(f32)

    def prologue2(c, mem):
        zo, he = Zb[1].sub(c, TPC * 256), HE.sub(c, TPC * DH)
        ms, rs = [], []
        for t in range(TPC):
            O = idftd2(1, zo, t)
            E = he.ld(t * DH, DH)
            x = x_v[:, cols(c, t, 128)].astype(f32)
            acc = [None] * 4
            for j in range(DH // 16):
                e, o = E[16 * j:16 * j + 16], O[16 * j:16 * j + 16]
                for k, (r, v) in enumerate(((16 * j, e + o), (DH + 16 * j, e - o))):
                    hb = (x[r:r + 16] + v).astype(bf16)
                    hb1_v[hrows(c, t, r, 16), :] = hb
                    hb2_v[hrows(c, t, r, 16), :] = hb
                    i = (2 * j + k) % 4
                    hf = hb.astype(f32)
                    acc[i] = hf if acc[i] is None else acc[i] + hf
            ms.append(_colsum((acc[0] + acc[1]) + (acc[2] + acc[3])) * (1.0 / D))
        for t in range(TPC):
            acc = [None] * 4
            for j in range(D // 16):
                d = h_ld(hb2_v, c, t, 16 * j, 16) - ms[t]
                acc[j % 4] = d * d if acc[j % 4] is None else acc[j % 4] + d * d
            v = _colsum((acc[0] + acc[1]) + (acc[2] + acc[3])) * (1.0 / D)
            rs.append(lax.rsqrt(v + EPS))
        hns = [(h_ld(hb1_v, c, t, 0, D) - ms[t]) * rs[t] for t in range(TPC)]
        hn = jnp.concatenate(hns, axis=1).astype(bf16)
        if mem:
            hn_v[:, cols(c)] = hn
            return None
        return None, hn

    def prologue(c, mem):
        if cfg["ln2"] == 1:
            return prologue2(c, mem)
        zo, he = Zb[1].sub(c, TPC * 256), HE.sub(c, TPC * DH)
        hs, hns = [], []
        for t in range(TPC):
            O = idftd2(1, zo, t)
            E = he.ld(t * DH, DH)
            y = jnp.concatenate([E + O, E - O], axis=0)
            hb = (x_v[:, cols(c, t, 128)].astype(f32) + y).astype(bf16)
            hf = hb.astype(f32)
            m = _colsum(hf) * (1.0 / D)
            hc = hf - m
            v = _colsum(hc * hc) * (1.0 / D)
            hs.append(hf)
            hns.append(hc * lax.rsqrt(v + EPS))
            if mem:
                out_v[:, cols(c, t, 128)] = hb
        hn = jnp.concatenate(hns, axis=1).astype(bf16)
        if mem:
            hn_v[:, cols(c)] = hn
            return None
        return jnp.concatenate(hs, axis=1), hn

    def rows(c):
        if isinstance(c, int):
            return pl.ds(c * CW, CW)
        return pl.ds(pl.multiple_of(c * CW, CW), CW)

    def out_copy(c, t=None):
        if t is None:
            return pltpu.make_async_copy(out_v.at[:, cols(c)], out_hbm.at[:, cols(c)], sems.at[nx + 3])
        return pltpu.make_async_copy(out_v.at[:, cols(c, t, 128)], out_hbm.at[:, cols(c, t, 128)], sems.at[nx + 3])

    def mlp(c, cur, nxt_fn=None, wd_wait=False):
        hnT = hn_v[:, cols(c)] if cur is None else cur[1]
        nxt = nxt_fn() if nxt_fn is not None else None
        g = lax.dot_general(hnT, wg_v[...], TN_DIMS, preferred_element_type=f32)
        u = lax.dot_general(hnT, wu_v[...], TN_DIMS, preferred_element_type=f32)
        hh = (g * u).astype(bf16)
        if wd_wait is True:
            wait("wd")
        elif wd_wait is not False:
            @pl.when(wd_wait)
            def _():
                wait("wd")
        if cfg["down_split"]:
            for t in range(TPC):
                mlp = lax.dot_general(wd_v[...], hh[t * 128:(t + 1) * 128], NT_DIMS, preferred_element_type=f32)
                if cfg["ln2"] == 1:
                    h = h_ld(hb1_v, c, t, 0, D)
                else:
                    h = out_v[:, cols(c, t, 128)].astype(f32) if cur is None else cur[0][:, t * 128:(t + 1) * 128]
                out_v[:, cols(c, t, 128)] = (h + mlp.astype(bf16).astype(f32)).astype(bf16)
                if cfg["down_split"] == 2:
                    out_copy(c, t).start()
            if cfg["down_split"] == 1:
                out_copy(c).start()
            return nxt
        mlp = lax.dot_general(wd_v[...], hh, NT_DIMS, preferred_element_type=f32)
        h = out_v[:, cols(c)].astype(f32) if cur is None else cur[0]
        out_v[:, cols(c)] = (h + mlp.astype(bf16).astype(f32)).astype(bf16)
        out_copy(c).start()
        return nxt

    def fwd_tile(a):
        if cfg.get("dbg_nofwd") and a < 15:
            return
        if a % 2 == 0:
            dftd_e(a, 0)
            dftd_e(a, 1)
            dftd_o(a)
        else:
            dftd_o(a)
            dftd_e(a, 0)
            dftd_e(a, 1)

    make_views()
    with scope("ph_fwd"):
        ln1(0)
        for a in range(1, NT):
            if a in xst:
                wait("x%d" % xst.index(a))
            fwd_tile(a - 1)
            ln1(a)
        fwd_tile(NT - 1)
    if cfg.get("dbg_stop") == 1:
        for n in order:
            if not (n[0] == "x" or n == "z"):
                wait(n)
        out_v[0:8, 0:128] = X1[0].ld(15 * 256, 8).astype(bf16) + X1[1].ld(15 * 256, 8).astype(bf16)
        cp = pltpu.make_async_copy(out_v.at[:, pl.ds(0, 128)], out_hbm.at[:, pl.ds(0, 128)], osems.at[0])
        cp.start()
        cp.wait()
        return
    for j in range(15):
        rad_fwd(0, j)
    wait("wr")
    def spread(k, k0, n, total, fn):
        if k0 <= k < k0 + n:
            for a in range(total * (k - k0) // n, total * (k - k0 + 1) // n):
                fn(a)

    j = 0
    wr0, wrn = cfg["wr_prep"]
    wi0, win = cfg["wi_prep"]
    for q in range(32):
        if q == cfg["wi_wait"]:
            wait("wi")
        dft128(q // 16, q % 16)
        if q >= cfg["ro_at"] and j < 14:
            rad_fwd(1, j)
            j += 1
        spread(q, wr0, wrn, 16, lambda a: wprep(wr_v, Wtr, a))
        spread(q, wi0, win, 16, lambda a: wprep(wi_v, Wti, a))
    assert j == 14 and cfg["ro_at"] <= 2 and wi0 >= cfg["wi_wait"]
    if cfg["bar_f"]:
        wait("bar_f")
    for k1 in range(16):
        idft128(0, k1)
    if cfg["bar_g"]:
        wait("bar_g")
    j = 0
    ne = cfg["h_early"]

    def early_h():
        for a in range(ne):
            HE.st(a * DH, idftd(0, a))

    for k1 in range(16):
        idft128(1, k1, early_h if (k1 == 15 and ne) else None)
        for _ in range(cfg["ge_per"] if k1 >= cfg["ge_at"] else 0):
            if j < 16:
                rad_inv(0, j)
                j += 1
    while j < 16:
        rad_inv(0, j)
        j += 1
    if cfg["bar_h"]:
        wait("bar_h")
    j = 0
    loop = cfg["mlp_loop"]
    mem = loop > 0 or cfg["mlp_mem"]
    state = {"done": False}

    def first_prologue():
        state["nxt"] = prologue(0, mem)
        if loop == 3:
            for c in range(cfg["mlp_unroll"], cfg["nmlp"], cfg["mlp_unroll"]):
                prologue(c, True)
        state["done"] = True

    for a in range(ne, 16):
        if a == cfg["wgwu_at"]:
            wait("wg", "wu", *(("wd",) if cfg["wd_early"] else ()))
        if a == cfg["pro_at"]:
            while j < 16:
                rad_inv(1, j)
                j += 1
            first_prologue()
        HE.st(a * DH, idftd(0, a))
        for _ in range(cfg["go_per"] if a >= cfg["go_at"] else 0):
            if j < 16:
                rad_inv(1, j)
                j += 1
    while j < 16:
        rad_inv(1, j)
        j += 1
    if not state["done"]:
        first_prologue()
    NC = cfg["nmlp"]
    if cfg["wgwu_at"] >= 16:
        wait("wg", "wu", *(("wd",) if cfg["wd_early"] else ()))
    if loop == 0:
        cur = state["nxt"]
        for c in range(NC):
            fn = (lambda c=c: prologue(c + 1, mem)) if c + 1 < NC else None
            cur = mlp(c, cur, fn, wd_wait=(c == 0 and not cfg["wd_early"]))
    else:
        U = cfg["mlp_unroll"]
        if loop == 3:
            assert NC % U == 0

            def body(i, carry):
                cur = None
                for k in range(U):
                    c = i * U + k
                    fn = (lambda c=c: prologue(c + 1, False)) if k < U - 1 else None
                    cur = mlp(c, cur, fn, wd_wait=(i == 0) if (k == 0 and not cfg["wd_early"]) else False)
                return carry

            with scope("ph_loop"):
                lax.fori_loop(0, NC // U, body, 0)
        elif loop == 1:
            assert NC % U == 0

            def body(i, carry):
                cur = None
                for k in range(U):
                    c = i * U + k
                    cn = jnp.minimum(c + 1, NC - 1) if k == U - 1 else c + 1
                    cur = mlp(c, cur, lambda: prologue(cn, k == U - 1 or not cfg["loop_ssa"]))
                return carry

            lax.fori_loop(0, NC // U, body, 0)
        else:
            peel = cfg["mlp_peel"]
            for c in range(peel):
                mlp(c, None, lambda c=c: prologue(c + 1, True))
            assert (NC - peel) % U == 0

            def body(i, carry):
                for k in range(U):
                    c = peel + i * U + k
                    cn = jnp.minimum(c + 1, NC - 1) if k == U - 1 else c + 1
                    mlp(c, None, lambda: prologue(cn, True))
                return carry

            lax.fori_loop(0, (NC - peel) // U, body, 0)
    pltpu.make_async_copy(out_v, out_hbm, sems.at[nx + 3]).wait()


@jax.jit
def pallas_sequential_preLN__spectral_gfnet__glu_gated_bilinear__prompt_kernel(
    A_x: jax.Array,
    A_w_r: jax.Array,
    A_w_i: jax.Array,
    B_x: jax.Array,
    B_w_gate: jax.Array,
    B_w_up: jax.Array,
    B_w_down: jax.Array,
):
    del B_x
    zc = np.zeros((24, 128), np.int32)
    zc[16:] = np.arange(128)
    xT = A_x.reshape(S, D).T
    any_spec = pl.BlockSpec(memory_space=pl.ANY)
    outT = pl.pallas_call(
        _kernel,
        out_shape=jax.ShapeDtypeStruct((D, S), bf16),
        in_specs=[any_spec] * 7,
        out_specs=any_spec,
        scratch_shapes=[
            pltpu.VMEM((D, S), bf16),
            pltpu.VMEM((DH + 1, S), bf16),
            pltpu.VMEM((DH + 1, S), bf16),
            pltpu.VMEM((D, F), bf16),
            pltpu.VMEM((D, F), bf16),
            pltpu.VMEM((D, F), bf16),
            pltpu.VMEM((FD_ROWS, 128), bf16),
            pltpu.VMEM((9 * 384, 128), bf16),
            pltpu.VMEM((2 * 448, 128), bf16),
            pltpu.VMEM((24, 128), jnp.int32),
            pltpu.VMEM((3, 8, 128), jnp.int32),
            pltpu.VMEM(((2 if CFG["w_f32"] else 1) * 16 * WP, 128), u32),
            pltpu.VMEM(((2 if CFG["w_f32"] else 1) * 16 * WP, 128), u32),
            pltpu.VMEM((D, S), bf16),
            pltpu.VMEM((D, S), bf16),
            pltpu.VMEM((NT * 256, 128), bf16),
            pltpu.VMEM((NT * 256, 128), bf16),
            pltpu.VMEM((NT * D, 128), bf16),
            pltpu.VMEM((NT * D, 128), bf16),
            pltpu.SemaphoreType.DMA((len(CFG["xchunks"]) + 4 + sum(bool(CFG[n]) for n in ("bar_f", "bar_g", "bar_h")),)),
        ] + [pltpu.VMEM((n, 128), u32) for n in _layout()[2]],
        compiler_params=pltpu.CompilerParams(vmem_limit_bytes=100 * 2**20),
        name="gfnet_glu",
    )(xT, A_w_r.T, A_w_i.T, B_w_gate, B_w_up, B_w_down.T, zc)
    return outT.T.reshape(1, S, D)
```

```python
import numpy as np
import jax
import jax.numpy as jnp
from jax import lax
from jax.experimental import pallas as pl
from jax.experimental.pallas import tpu as pltpu

S, D, F = 2048, 448, 1792
DH, DQ = D // 2, D // 4
NT = S // 128
EPS = 1e-5
bf16, f32, u32 = jnp.bfloat16, jnp.float32, jnp.uint32
NT_DIMS = (((1,), (1,)), ((), ()))
TN_DIMS = (((0,), (0,)), ((), ()))
XC = 4
WP = 136
TPC = 2
CW = TPC * 128
UNROLL = 4
NVOB = 2
FD_ROWS = 56 + 56 + 2 * 112

_GROUPS = (("YE", "YO"), ("VO", "ZE", "ZO"), ("X1E",), ("X1O",), ("X2E",), ("X2O",), ("VE",), ("VOB",), ("HE",))
_ROWS = dict(X1E=4096, X1O=4096, YE=4096, YO=4096, X2E=4096, X2O=4096, VE=4096, VO=4096, ZE=4096, ZO=4096,
             VOB=NVOB * 256, HE=NT * DH)


def _cis(n, period):
    nf = n.astype(f32)
    r = nf - jnp.floor(nf * np.float32(1.0 / period) + 0.5) * np.float32(period)
    ang = r * np.float32(2 * np.pi / period)
    return jnp.cos(ang), -jnp.sin(ang)


def _cmul(a, b):
    return a[0] * b[0] - a[1] * b[1], a[0] * b[1] + a[1] * b[0]


def _geom(base, step, n):
    out = [base]
    for _ in range(n - 1):
        out.append(_cmul(out[-1], step))
    return out


def _pack_rows(vregs):
    return pltpu.bitcast(jnp.concatenate(vregs, axis=0).astype(bf16), u32)


def _bf(w):
    return pltpu.bitcast(w, bf16)


def _lo(w):
    return lax.bitcast_convert_type(lax.shift_left(w, np.uint32(16)), f32)


def _hi(w):
    return lax.bitcast_convert_type(w & np.uint32(0xFFFF0000), f32)


class _V:
    __slots__ = ("a", "n")

    def __init__(self, a, n=False):
        self.a, self.n = a, n

    def __neg__(self):
        return _V(self.a, not self.n)

    def __add__(self, o):
        if o.a is None:
            return self
        if self.a is None:
            return o
        if self.n == o.n:
            return _V(self.a + o.a, self.n)
        return _V(o.a - self.a) if self.n else _V(self.a - o.a)

    def __sub__(self, o):
        return self + (-o)

    def mul(self, c):
        return self if self.a is None else _V(self.a * np.float32(-c if self.n else c))

    def val(self, like):
        if self.a is None:
            return jnp.zeros_like(like)
        return -self.a if self.n else self.a


def _r4(x, sg):
    (x0r, x0i), (x1r, x1i), (x2r, x2i), (x3r, x3i) = x
    t0r, t0i, t1r, t1i = x0r + x2r, x0i + x2i, x0r - x2r, x0i - x2i
    t2r, t2i, t3r, t3i = x1r + x3r, x1i + x3i, x1r - x3r, x1i - x3i
    ur, ui = (-t3i, t3r) if sg > 0 else (t3i, -t3r)
    return [(t0r + t2r, t0i + t2i), (t1r + ur, t1i + ui), (t0r - t2r, t0i - t2i), (t1r - ur, t1i - ui)]


def _tw(x, e, sg):
    xr, xi = x
    if e % 4 == 0:
        q = (sg * (e // 4)) % 4
        return [(xr, xi), (-xi, xr), (-xr, -xi), (xi, -xr)][q]
    c, s = np.cos(2 * np.pi * e / 16), sg * np.sin(2 * np.pi * e / 16)
    if e % 2 == 0:
        sc = (lambda v: v) if c > 0 else (lambda v: -v)
        ss = (lambda v: v) if s > 0 else (lambda v: -v)
        return (sc(xr) - ss(xi)).mul(abs(c)), (sc(xi) + ss(xr)).mul(abs(c))
    return xr.mul(c) - xi.mul(s), xi.mul(c) + xr.mul(s)


def _fft16(re, im, sg):
    x = [(_V(re[a]), _V(im[a])) for a in range(16)]
    t = [_r4([x[4 * a1 + a0] for a1 in range(4)], sg) for a0 in range(4)]
    out_re, out_im = [None] * 16, [None] * 16
    for k0 in range(4):
        y = _r4([_tw(t[a0][k0], a0 * k0, sg) for a0 in range(4)], sg)
        for k1 in range(4):
            out_re[k0 + 4 * k1] = y[k1][0].val(re[0])
            out_im[k0 + 4 * k1] = y[k1][1].val(re[0])
    return out_re, out_im


def _colsum(x):
    parts = [x[i:i + 8] for i in range(0, x.shape[0], 8)]
    while len(parts) > 1:
        nxt = [parts[i] + parts[i + 1] for i in range(0, len(parts) - 1, 2)]
        if len(parts) % 2:
            nxt.append(parts[-1])
        parts = nxt
    return jnp.sum(parts[0], axis=0, keepdims=True)


class _Buf:
    def __init__(self, ref, zs, zl, off=0, n=None, views=None):
        self.ref, self.zs, self.zl, self.off = ref, zs, zl, off
        self.sv, self.lv = views or (ref.at[pl.ds(zs, n)], ref.at[pl.ds(zl, n)])

    def at_rows(self, start, n):
        if isinstance(start, int):
            return _Buf(self.ref, self.zs, self.zl, self.off + start, views=(self.sv, self.lv))
        base = pl.multiple_of(self.off + start, 8)
        return _Buf(self.ref, self.zs + base, self.zl + base, n=n)

    def st(self, row, val, stride=None):
        row += self.off
        idx = pl.ds(row, val.shape[0]) if stride is None else pl.ds(row, val.shape[0], stride=stride)
        self.sv[idx, :] = lax.bitcast_convert_type(val, u32)

    def ld(self, row, n):
        row += self.off
        return lax.bitcast_convert_type(self.lv[row:row + n, :], f32)


def _kernel(x_hbm, wr_hbm, wi_hbm, wg_hbm, wu_hbm, wd_hbm, z_hbm, out_hbm,
            x_v, wr_v, wi_v, wg_v, wu_v, wd_v, z_v, zb_v, fd_v, g_v, gs_v, bd_v,
            wtr_v, wti_v, out_v, hn_v, hb_v, sems, *arenas):
    xw = S // XC
    x_cp = [pltpu.make_async_copy(x_hbm.at[:, pl.ds(c * xw, xw)], x_v.at[:, pl.ds(c * xw, xw)], sems.at[c])
            for c in range(XC)]
    cp_z = pltpu.make_async_copy(z_hbm, z_v, sems.at[0])
    cp_wr = pltpu.make_async_copy(wr_hbm, wr_v, sems.at[XC])
    cp_wi = pltpu.make_async_copy(wi_hbm, wi_v, sems.at[XC + 1])
    cp_mlp = [pltpu.make_async_copy(h, v, sems.at[XC + 2]) for h, v in ((wg_hbm, wg_v), (wu_hbm, wu_v), (wd_hbm, wd_v))]
    out_sem = sems.at[XC + 3]
    cp_bar = pltpu.make_async_copy(z_hbm.at[pl.ds(0, 8)], zb_v, sems.at[XC + 4])
    for cp in [cp_z, cp_bar] + x_cp + [cp_wr, cp_wi] + cp_mlp:
        cp.start()

    i = lax.broadcasted_iota(jnp.int32, (8, 128), 0)
    c = lax.broadcasted_iota(jnp.int32, (8, 128), 1)
    f = _geom(_cis(i * c, 128), _cis(8 * c, 128), 16)
    t1 = _cis(c, S)
    t = t1
    for km in range(9):
        g = f
        if km:
            if km > 1:
                t = _cmul(t, t1)
            g = [_cmul(e, t) for e in f]
        g_v[km, 0:64, :] = _pack_rows([e[0] for e in g])
        g_v[km, 64:128, :] = _pack_rows([e[1] for e in g])
        gs_v[km] = _pack_rows([e[0] + e[1] for e in g])
    b0, st0 = _cis(4 * i * c, D), _cis(32 * c, D)
    e0 = _geom(b0, st0, 7)
    e2 = _geom(_cmul(b0, _cis(2 * c, D)), st0, 7)
    nyq = (1 - 2 * (c & 1)).astype(f32)
    fd_v[0:56, :] = _pack_rows([e[0] for e in e0] + [jnp.where(i == 0, nyq, e0[0][1])] + [e[1] for e in e0[1:]])
    fd_v[56:112, :] = _pack_rows([e[0] for e in e2] + [e[1] for e in e2])
    for kt in range(2):
        dd = c + 128 * kt
        eo = _geom(_cis((2 * i + 1) * dd, D), _cis(16 * dd, D), 14)
        fd_v[112 + 112 * kt:224 + 112 * kt, :] = _pack_rows([e[0] for e in eo] + [e[1] for e in eo])
    sc = np.float32(1.0 / (D * S))
    for p in range(2):
        kd = 2 * c + p
        if p == 0:
            wgt = jnp.where((c == 0) | (c == DQ), sc, jnp.where(c < DQ, 2 * sc, np.float32(0)))
        else:
            wgt = jnp.where(c < DQ, 2 * sc, np.float32(0))
        base, step = _cis(kd * i, D), _cis(8 * kd, D)
        if p == 0:
            base = (base[0], jnp.where(c == DQ, np.float32(0), base[1]))
            step = (step[0], jnp.where(c == DQ, np.float32(0), step[1]))
        e = _geom((base[0] * wgt, base[1] * wgt), step, DH // 8)
        bd_v[p, 0] = _pack_rows([v[0] for v in e])
        bd_v[p, 1] = _pack_rows([v[1] for v in e])

    cp_z.wait()
    x_cp[0].wait()
    zz = z_v[0:16, :]
    z1 = pl.multiple_of(jnp.max(zz[0:8]), 8)
    z2 = pl.multiple_of(jnp.max(zz[8:16]), 8)
    bufs = {}
    for ref, group in zip(arenas, _GROUPS):
        whole = _Buf(ref, z1, z2, n=ref.shape[0])
        off = 0
        for name in group:
            bufs[name] = whole.at_rows(off, _ROWS[name])
            off += _ROWS[name]
    X1, Y = (bufs["X1E"], bufs["X1O"]), (bufs["YE"], bufs["YO"])
    X2, Z, HE = (bufs["X2E"], bufs["X2O"]), (bufs["ZE"], bufs["ZO"]), bufs["HE"]

    def vbuf(p, k1):
        if p == 0:
            return bufs["VE"], k1 * 256
        if k1 >= 16 - NVOB:
            return bufs["VOB"], (k1 - (16 - NVOB)) * 256
        return bufs["VO"], k1 * 256

    rstd, eos = [None] * NT, [None] * NT

    def ln1(a):
        x = x_v[:, a * 128:(a + 1) * 128].astype(f32)
        a0, a2s, dl, dh = [], [], [], []
        acc = [None] * 4

        def add(k, v):
            acc[k] = v if acc[k] is None else acc[k] + v

        for j in range(DQ // 16):
            x0, x1, x2, x3 = (x[q * DQ + 16 * j:q * DQ + 16 * j + 16] for q in range(4))
            s02, s13, d02, d13 = x0 + x2, x1 + x3, x0 - x2, x1 - x3
            a2 = s02 - s13
            a0.append(s02 + s13)
            a2s.append(a2)
            dl.append(d02)
            dh.append(d13)
            add(0, d02 * d02)
            add(1, d13 * d13)
            add(2, a2 * a2)
        m4 = _colsum(jnp.concatenate(a0, axis=0)) * (4.0 / D)
        a0c = [v - m4 for v in a0]
        for v in a0c:
            add(3, v * v)
        var = _colsum((acc[0] + acc[1]) * 2.0 + (acc[2] + acc[3])) * (0.25 / D)
        rstd[a] = lax.rsqrt(var + EPS)
        eos[a] = (a0c, a2s, dl + dh)

    row0 = lax.broadcasted_iota(jnp.int32, (8, 128), 0) == 0

    def dftd_e(a, q):
        rhs = jnp.concatenate(eos[a][q] + [jnp.zeros((16, 128), f32)], axis=0).astype(bf16)
        r = jnp.dot(_bf(fd_v[56 * q:56 * q + 56, :]), rhs, preferred_element_type=f32) * rstd[a]
        for part in range(2):
            for v in range(7):
                blk = r[56 * part + 8 * v:56 * part + 8 * v + 8]
                if q == 0 and part == 1 and v == 0:
                    X1[0].st(a * 256 + 112, jnp.where(row0, blk, 0.0))
                    blk = jnp.where(row0, 0.0, blk)
                X1[0].st(a * 256 + 128 * part + 16 * v + q, blk, stride=2)

    def dftd_o(a):
        lhs = jnp.concatenate([_bf(fd_v[112:224, :]), _bf(fd_v[224:336, :])], axis=1)
        rhs = jnp.concatenate(eos[a][2] + [jnp.zeros((32, 128), f32)], axis=0).astype(bf16)
        r = jnp.dot(lhs, rhs, preferred_element_type=f32) * rstd[a]
        X1[1].st(a * 256, r[:DQ])
        X1[1].st(a * 256 + 128, r[DQ:])

    def fwd_tile(a):
        if a % 2 == 0:
            dftd_e(a, 0)
            dftd_e(a, 1)
            dftd_o(a)
        else:
            dftd_o(a)
            dftd_e(a, 0)
            dftd_e(a, 1)

    def rad_fwd(p, j):
        r = 8 * j
        re = [X1[p].ld(a * 256 + r, 8) for a in range(16)]
        only_nyq = p == 0 and j == 14
        im = [None if only_nyq else X1[p].ld(a * 256 + 128 + r, 8) for a in range(16)]
        ore, oim = _fft16(re, im, -1)
        for k1 in range(16):
            Y[p].st(k1 * 256 + r, ore[k1])
            Y[p].st(k1 * 256 + 128 + r, oim[k1])

    def cmul3(km, conj, a, b, dims):
        gr, gi, gs = _bf(g_v[km, 0:64, :]), _bf(g_v[km, 64:128, :]), _bf(gs_v[km])
        m1 = lax.dot_general(gr, a.astype(bf16), dims, preferred_element_type=f32)
        m2 = lax.dot_general(gi, b.astype(bf16), dims, preferred_element_type=f32)
        if conj:
            m3 = lax.dot_general(gs, (b - a).astype(bf16), dims, preferred_element_type=f32)
            return m1 + m2, m3 + (m1 - m2)
        m3 = lax.dot_general(gs, (a + b).astype(bf16), dims, preferred_element_type=f32)
        return m1 - m2, m3 - (m1 + m2)

    def dft128(p, k1):
        n = 112 if p else 120
        pad = jnp.zeros((128 - n, 128), f32)
        yr = jnp.concatenate([Y[p].ld(k1 * 256, n), pad], axis=0)
        yi = jnp.concatenate([Y[p].ld(k1 * 256 + 128, n), pad], axis=0)
        xr, xi = cmul3(k1 if k1 < 8 else 16 - k1, k1 >= 8, yr, yi, NT_DIMS)
        X2[p].st(k1 * 256, xr)
        X2[p].st(k1 * 256 + 128, xi)

    def wprep(w_v, wt_v, a):
        w32 = pltpu.bitcast(w_v[0:DH, a * 128:(a + 1) * 128], u32)
        ny = jnp.broadcast_to(w_v[DH:DH + 1, a * 128:(a + 1) * 128].astype(f32), (8, 128))
        ny = lax.shift_right_logical(lax.bitcast_convert_type(ny, u32), np.uint32(16))
        tile = jnp.concatenate([w32, jnp.where(row0, ny, np.uint32(0)), jnp.zeros((8, 128), u32)], axis=0).T
        for j in range(8):
            wt_v[pl.ds(a * WP + 17 * j, 8), :] = tile[16 * j:16 * j + 8, :]
            wt_v[pl.ds((15 - a) * WP + 17 * (7 - j) + 8, 8), :] = tile[16 * j + 8:16 * j + 16, :]

    def idft128(p, k1):
        wr32 = jnp.concatenate([wtr_v[pl.ds(a * WP + k1, 8, stride=17), :] for a in range(16)], axis=0)
        wi32 = jnp.concatenate([wti_v[pl.ds(a * WP + k1, 8, stride=17), :] for a in range(16)], axis=0)
        wr, wi = (_hi(wr32), _hi(wi32)) if p else (_lo(wr32), _lo(wi32))
        xr, xi = X2[p].ld(k1 * 256, 128), X2[p].ld(k1 * 256 + 128, 128)
        vr, vi = cmul3(k1 if k1 < 8 else 16 - k1, k1 < 8, xr * wr - xi * wi, xr * wi + xi * wr, TN_DIMS)
        vb, r0 = vbuf(p, k1)
        vb.st(r0, vr)
        vb.st(r0 + 128, vi)

    def rad_inv(p, j):
        r = 8 * j
        src = [vbuf(p, k1) for k1 in range(16)]
        re = [vb.ld(r0 + r, 8) for vb, r0 in src]
        im = [vb.ld(r0 + 128 + r, 8) for vb, r0 in src]
        ore, oim = _fft16(re, im, +1)
        for s1 in range(16):
            Z[p].st(s1 * 256 + r, ore[s1])
            Z[p].st(s1 * 256 + 128 + r, oim[s1])

    def idftd(p, zb, a):
        z = jnp.concatenate([zb.ld(a * 256, 128), zb.ld(a * 256 + 128, 128)], axis=1).astype(bf16)
        lhs = jnp.concatenate([_bf(bd_v[p, 0]), _bf(bd_v[p, 1])], axis=1)
        return lax.dot_general(lhs, z, NT_DIMS, preferred_element_type=f32)

    def cols(ch, t=0, n=CW):
        if isinstance(ch, int):
            return pl.ds(ch * CW + t * 128, n)
        return pl.ds(pl.multiple_of(ch * CW, CW) + t * 128, n)

    def hrows(ch, t, r=0, n=D):
        if isinstance(ch, int):
            return pl.ds((ch * TPC + t) * D + r, n)
        return pl.ds(pl.multiple_of(ch * (TPC * D), 16) + (t * D + r), n)

    def prologue(ch, to_mem):
        zo, he = Z[1].at_rows(ch * (TPC * 256), TPC * 256), HE.at_rows(ch * (TPC * DH), TPC * DH)
        means, scales = [], []
        for t in range(TPC):
            o = idftd(1, zo, t)
            e = he.ld(t * DH, DH)
            x = x_v[:, cols(ch, t, 128)].astype(f32)
            acc = [None] * 4
            for j in range(DH // 16):
                ej, oj = e[16 * j:16 * j + 16], o[16 * j:16 * j + 16]
                for k, (r, y) in enumerate(((16 * j, ej + oj), (DH + 16 * j, ej - oj))):
                    hb = (x[r:r + 16] + y).astype(bf16)
                    hb_v[hrows(ch, t, r, 16), :] = hb
                    q = (2 * j + k) % 4
                    acc[q] = hb.astype(f32) if acc[q] is None else acc[q] + hb.astype(f32)
            means.append(_colsum((acc[0] + acc[1]) + (acc[2] + acc[3])) * (1.0 / D))
        for t in range(TPC):
            acc = [None] * 4
            for j in range(D // 16):
                d = hb_v[hrows(ch, t, 16 * j, 16), :].astype(f32) - means[t]
                acc[j % 4] = d * d if acc[j % 4] is None else acc[j % 4] + d * d
            scales.append(lax.rsqrt(_colsum((acc[0] + acc[1]) + (acc[2] + acc[3])) * (1.0 / D) + EPS))
        hn = [(hb_v[hrows(ch, t), :].astype(f32) - means[t]) * scales[t] for t in range(TPC)]
        hn = jnp.concatenate(hn, axis=1).astype(bf16)
        if to_mem:
            hn_v[:, cols(ch)] = hn
            return None
        return hn

    def mlp(ch, hn, with_next):
        if hn is None:
            hn = hn_v[:, cols(ch)]
        nxt = prologue(ch + 1, False) if with_next else None
        g = lax.dot_general(hn, wg_v[...], TN_DIMS, preferred_element_type=f32)
        u = lax.dot_general(hn, wu_v[...], TN_DIMS, preferred_element_type=f32)
        hh = (g * u).astype(bf16)
        for t in range(TPC):
            y = lax.dot_general(wd_v[...], hh[t * 128:(t + 1) * 128], NT_DIMS, preferred_element_type=f32)
            h = hb_v[hrows(ch, t), :].astype(f32)
            out_v[:, cols(ch, t, 128)] = (h + y.astype(bf16).astype(f32)).astype(bf16)
            pltpu.make_async_copy(out_v.at[:, cols(ch, t, 128)], out_hbm.at[:, cols(ch, t, 128)], out_sem).start()
        return nxt

    ln1(0)
    for a in range(1, NT):
        if a % (NT // XC) == 0:
            x_cp[a // (NT // XC)].wait()
        fwd_tile(a - 1)
        ln1(a)
    fwd_tile(NT - 1)
    for j in range(15):
        rad_fwd(0, j)
    cp_wr.wait()
    for q in range(32):
        if q == 24:
            cp_wi.wait()
        dft128(q // 16, q % 16)
        if 1 <= q < 15:
            rad_fwd(1, q - 1)
        if q >= 16:
            for a in (2 * (q % 8), 2 * (q % 8) + 1):
                wprep(*((wr_v, wtr_v) if q < 24 else (wi_v, wti_v)), a)
    cp_bar.wait()
    for k1 in range(16):
        idft128(0, k1)
    for k1 in range(16):
        idft128(1, k1)
        if k1 < 8:
            rad_inv(0, 2 * k1)
            rad_inv(0, 2 * k1 + 1)
    for a in range(NT):
        HE.st(a * DH, idftd(0, Z[0], a))
        rad_inv(1, a)
    for ch in range(0, NT // TPC, UNROLL):
        prologue(ch, True)
    for cp in cp_mlp:
        cp.wait()

    def body(it, carry):
        hn = None
        for k in range(UNROLL):
            hn = mlp(it * UNROLL + k, hn, k < UNROLL - 1)
        return carry

    lax.fori_loop(0, NT // TPC // UNROLL, body, 0)
    pltpu.make_async_copy(out_v, out_hbm, out_sem).wait()


@jax.jit
def pallas_sequential_preLN__spectral_gfnet__glu_gated_bilinear__prompt_kernel(
    A_x: jax.Array,
    A_w_r: jax.Array,
    A_w_i: jax.Array,
    B_x: jax.Array,
    B_w_gate: jax.Array,
    B_w_up: jax.Array,
    B_w_down: jax.Array,
):
    del B_x
    zc = np.zeros((24, 128), np.int32)
    zc[16:] = np.arange(128)
    any_spec = pl.BlockSpec(memory_space=pl.ANY)
    vm = pltpu.VMEM
    out_t = pl.pallas_call(
        _kernel,
        out_shape=jax.ShapeDtypeStruct((D, S), bf16),
        in_specs=[any_spec] * 7,
        out_specs=any_spec,
        scratch_shapes=[
            vm((D, S), bf16), vm((DH + 1, S), bf16), vm((DH + 1, S), bf16),
            vm((D, F), bf16), vm((D, F), bf16), vm((D, F), bf16),
            vm((24, 128), jnp.int32), vm((8, 128), jnp.int32),
            vm((FD_ROWS, 128), u32), vm((9, 128, 128), u32), vm((9, 64, 128), u32), vm((2, 2, DH // 2, 128), u32),
            vm((16 * WP, 128), u32), vm((16 * WP, 128), u32),
            vm((D, S), bf16), vm((D, S), bf16), vm((NT * D, 128), bf16),
            pltpu.SemaphoreType.DMA((XC + 5,)),
        ] + [vm((sum(_ROWS[n] for n in group), 128), u32) for group in _GROUPS],
        compiler_params=pltpu.CompilerParams(vmem_limit_bytes=100 * 2**20),
        name="gfnet_glu",
    )(A_x.reshape(S, D).T, A_w_r.T, A_w_i.T, B_w_gate, B_w_up, B_w_down.T, zc)
    return out_t.T.reshape(1, S, D)
```

```python
import numpy as np
import jax
import jax.numpy as jnp
from jax import lax
from jax.experimental import pallas as pl
from jax.experimental.pallas import tpu as pltpu

S, D, F = 2048, 448, 1792
DH, DQ = D // 2, D // 4
NT = S // 128
EPS = 1e-5
bf16, f32, u32 = jnp.bfloat16, jnp.float32, jnp.uint32
NT_DIMS = (((1,), (1,)), ((), ()))
TN_DIMS = (((0,), (0,)), ((), ()))
XC = 4
WP = 136
TPC = 2
CW = TPC * 128
UNROLL = 4
NVOB = 2
FD_ROWS = 56 + 56 + 2 * 112

PA, PB = 1, 0
_GROUPS = (("YE", "YO"), ("V2", "ZE", "ZO"), ("X1E",), ("X1O",), ("X2E",), ("X2O",), ("V1",), ("VOB",), ("HE",))
_ROWS = dict(X1E=4096, X1O=4096, YE=4096, YO=4096, X2E=4096, X2O=4096, V1=4096, V2=4096, ZE=4096, ZO=4096,
             VOB=NVOB * 256, HE=NT * DH)


def _cis(n, period):
    nf = n.astype(f32)
    r = nf - jnp.floor(nf * np.float32(1.0 / period) + 0.5) * np.float32(period)
    ang = r * np.float32(2 * np.pi / period)
    return jnp.cos(ang), -jnp.sin(ang)


def _cmul(a, b):
    return a[0] * b[0] - a[1] * b[1], a[0] * b[1] + a[1] * b[0]


def _geom(base, step, n):
    out = [base]
    for _ in range(n - 1):
        out.append(_cmul(out[-1], step))
    return out


def _pack_rows(vregs):
    return pltpu.bitcast(jnp.concatenate(vregs, axis=0).astype(bf16), u32)


def _bf(w):
    return pltpu.bitcast(w, bf16)


def _lo(w):
    return lax.bitcast_convert_type(lax.shift_left(w, np.uint32(16)), f32)


def _hi(w):
    return lax.bitcast_convert_type(w & np.uint32(0xFFFF0000), f32)


class _V:
    __slots__ = ("a", "n")

    def __init__(self, a, n=False):
        self.a, self.n = a, n

    def __neg__(self):
        return _V(self.a, not self.n)

    def __add__(self, o):
        if o.a is None:
            return self
        if self.a is None:
            return o
        if self.n == o.n:
            return _V(self.a + o.a, self.n)
        return _V(o.a - self.a) if self.n else _V(self.a - o.a)

    def __sub__(self, o):
        return self + (-o)

    def mul(self, c):
        return self if self.a is None else _V(self.a * np.float32(-c if self.n else c))

    def val(self, like):
        if self.a is None:
            return jnp.zeros_like(like)
        return -self.a if self.n else self.a


def _r4(x, sg):
    (x0r, x0i), (x1r, x1i), (x2r, x2i), (x3r, x3i) = x
    t0r, t0i, t1r, t1i = x0r + x2r, x0i + x2i, x0r - x2r, x0i - x2i
    t2r, t2i, t3r, t3i = x1r + x3r, x1i + x3i, x1r - x3r, x1i - x3i
    ur, ui = (-t3i, t3r) if sg > 0 else (t3i, -t3r)
    return [(t0r + t2r, t0i + t2i), (t1r + ur, t1i + ui), (t0r - t2r, t0i - t2i), (t1r - ur, t1i - ui)]


def _tw(x, e, sg):
    xr, xi = x
    if e % 4 == 0:
        q = (sg * (e // 4)) % 4
        return [(xr, xi), (-xi, xr), (-xr, -xi), (xi, -xr)][q]
    c, s = np.cos(2 * np.pi * e / 16), sg * np.sin(2 * np.pi * e / 16)
    if e % 2 == 0:
        sc = (lambda v: v) if c > 0 else (lambda v: -v)
        ss = (lambda v: v) if s > 0 else (lambda v: -v)
        return (sc(xr) - ss(xi)).mul(abs(c)), (sc(xi) + ss(xr)).mul(abs(c))
    return xr.mul(c) - xi.mul(s), xi.mul(c) + xr.mul(s)


def _fft16(re, im, sg):
    x = [(_V(re[a]), _V(im[a])) for a in range(16)]
    t = [_r4([x[4 * a1 + a0] for a1 in range(4)], sg) for a0 in range(4)]
    out_re, out_im = [None] * 16, [None] * 16
    for k0 in range(4):
        y = _r4([_tw(t[a0][k0], a0 * k0, sg) for a0 in range(4)], sg)
        for k1 in range(4):
            out_re[k0 + 4 * k1] = y[k1][0].val(re[0])
            out_im[k0 + 4 * k1] = y[k1][1].val(re[0])
    return out_re, out_im


def _colsum(x):
    parts = [x[i:i + 8] for i in range(0, x.shape[0], 8)]
    while len(parts) > 1:
        nxt = [parts[i] + parts[i + 1] for i in range(0, len(parts) - 1, 2)]
        if len(parts) % 2:
            nxt.append(parts[-1])
        parts = nxt
    return jnp.sum(parts[0], axis=0, keepdims=True)


class _Buf:
    def __init__(self, ref, zs, zl, off=0, n=None, views=None):
        self.ref, self.zs, self.zl, self.off = ref, zs, zl, off
        self.sv, self.lv = views or (ref.at[pl.ds(zs, n)], ref.at[pl.ds(zl, n)])

    def at_rows(self, start, n):
        if isinstance(start, int):
            return _Buf(self.ref, self.zs, self.zl, self.off + start, views=(self.sv, self.lv))
        base = pl.multiple_of(self.off + start, 8)
        return _Buf(self.ref, self.zs + base, self.zl + base, n=n)

    def st(self, row, val, stride=None):
        row += self.off
        idx = pl.ds(row, val.shape[0]) if stride is None else pl.ds(row, val.shape[0], stride=stride)
        self.sv[idx, :] = lax.bitcast_convert_type(val, u32)

    def ld(self, row, n):
        row += self.off
        return lax.bitcast_convert_type(self.lv[row:row + n, :], f32)


def _kernel(x_hbm, wr_hbm, wi_hbm, wg_hbm, wu_hbm, wd_hbm, z_hbm, out_hbm,
            x_v, wr_v, wi_v, wg_v, wu_v, wd_v, z_v, zb_v, fd_v, g_v, gs_v, bd_v,
            wtr_v, wti_v, out_v, hn_v, hb_v, sems, *arenas):
    xw = S // XC
    x_cp = [pltpu.make_async_copy(x_hbm.at[:, pl.ds(c * xw, xw)], x_v.at[:, pl.ds(c * xw, xw)], sems.at[c])
            for c in range(XC)]
    cp_z = pltpu.make_async_copy(z_hbm, z_v, sems.at[0])
    cp_wr = pltpu.make_async_copy(wr_hbm, wr_v, sems.at[XC])
    cp_wi = pltpu.make_async_copy(wi_hbm, wi_v, sems.at[XC + 1])
    cp_mlp = [pltpu.make_async_copy(h, v, sems.at[XC + 2]) for h, v in ((wg_hbm, wg_v), (wu_hbm, wu_v), (wd_hbm, wd_v))]
    out_sem = sems.at[XC + 3]
    cp_bar = pltpu.make_async_copy(z_hbm.at[pl.ds(0, 8)], zb_v, sems.at[XC + 4])
    for cp in [cp_z, cp_bar] + x_cp + [cp_wr, cp_wi] + cp_mlp:
        cp.start()

    i = lax.broadcasted_iota(jnp.int32, (8, 128), 0)
    c = lax.broadcasted_iota(jnp.int32, (8, 128), 1)
    f = _geom(_cis(i * c, 128), _cis(8 * c, 128), 16)
    t1 = _cis(c, S)
    t = t1
    for km in range(9):
        g = f
        if km:
            if km > 1:
                t = _cmul(t, t1)
            g = [_cmul(e, t) for e in f]
        g_v[km, 0:64, :] = _pack_rows([e[0] for e in g])
        g_v[km, 64:128, :] = _pack_rows([e[1] for e in g])
        gs_v[km] = _pack_rows([e[0] + e[1] for e in g])
    b0, st0 = _cis(4 * i * c, D), _cis(32 * c, D)
    e0 = _geom(b0, st0, 7)
    e2 = _geom(_cmul(b0, _cis(2 * c, D)), st0, 7)
    nyq = (1 - 2 * (c & 1)).astype(f32)
    fd_v[0:56, :] = _pack_rows([e[0] for e in e0] + [jnp.where(i == 0, nyq, e0[0][1])] + [e[1] for e in e0[1:]])
    fd_v[56:112, :] = _pack_rows([e[0] for e in e2] + [e[1] for e in e2])
    for kt in range(2):
        dd = c + 128 * kt
        eo = _geom(_cis((2 * i + 1) * dd, D), _cis(16 * dd, D), 14)
        fd_v[112 + 112 * kt:224 + 112 * kt, :] = _pack_rows([e[0] for e in eo] + [e[1] for e in eo])
    sc = np.float32(1.0 / (D * S))
    for p in range(2):
        kd = 2 * c + p
        if p == 0:
            wgt = jnp.where((c == 0) | (c == DQ), sc, jnp.where(c < DQ, 2 * sc, np.float32(0)))
        else:
            wgt = jnp.where(c < DQ, 2 * sc, np.float32(0))
        base, step = _cis(kd * i, D), _cis(8 * kd, D)
        if p == 0:
            base = (base[0], jnp.where(c == DQ, np.float32(0), base[1]))
            step = (step[0], jnp.where(c == DQ, np.float32(0), step[1]))
        e = _geom((base[0] * wgt, base[1] * wgt), step, DH // 8)
        bd_v[p, 0] = _pack_rows([v[0] for v in e])
        bd_v[p, 1] = _pack_rows([v[1] for v in e])

    cp_z.wait()
    x_cp[0].wait()
    zz = z_v[0:16, :]
    z1 = pl.multiple_of(jnp.max(zz[0:8]), 8)
    z2 = pl.multiple_of(jnp.max(zz[8:16]), 8)
    bufs = {}
    for ref, group in zip(arenas, _GROUPS):
        whole = _Buf(ref, z1, z2, n=ref.shape[0])
        off = 0
        for name in group:
            bufs[name] = whole.at_rows(off, _ROWS[name])
            off += _ROWS[name]
    X1, Y = (bufs["X1E"], bufs["X1O"]), (bufs["YE"], bufs["YO"])
    X2, Z, HE = (bufs["X2E"], bufs["X2O"]), (bufs["ZE"], bufs["ZO"]), bufs["HE"]

    def vbuf(p, k1):
        if p == PA:
            return bufs["V1"], k1 * 256
        if k1 >= 16 - NVOB:
            return bufs["VOB"], (k1 - (16 - NVOB)) * 256
        return bufs["V2"], k1 * 256

    rstd, eos = [None] * NT, [None] * NT

    def ln1(a):
        x = x_v[:, a * 128:(a + 1) * 128].astype(f32)
        a0, a2s, dl, dh = [], [], [], []
        acc = [None] * 4

        def add(k, v):
            acc[k] = v if acc[k] is None else acc[k] + v

        for j in range(DQ // 16):
            x0, x1, x2, x3 = (x[q * DQ + 16 * j:q * DQ + 16 * j + 16] for q in range(4))
            s02, s13, d02, d13 = x0 + x2, x1 + x3, x0 - x2, x1 - x3
            a2 = s02 - s13
            a0.append(s02 + s13)
            a2s.append(a2)
            dl.append(d02)
            dh.append(d13)
            add(0, d02 * d02)
            add(1, d13 * d13)
            add(2, a2 * a2)
        m4 = _colsum(jnp.concatenate(a0, axis=0)) * (4.0 / D)
        a0c = [v - m4 for v in a0]
        for v in a0c:
            add(3, v * v)
        var = _colsum((acc[0] + acc[1]) * 2.0 + (acc[2] + acc[3])) * (0.25 / D)
        rstd[a] = lax.rsqrt(var + EPS)
        eos[a] = (a0c, a2s, dl + dh)

    row0 = lax.broadcasted_iota(jnp.int32, (8, 128), 0) == 0

    def dftd_e(a, q):
        rhs = jnp.concatenate(eos[a][q] + [jnp.zeros((16, 128), f32)], axis=0).astype(bf16)
        r = jnp.dot(_bf(fd_v[56 * q:56 * q + 56, :]), rhs, preferred_element_type=f32) * rstd[a]
        for part in range(2):
            for v in range(7):
                blk = r[56 * part + 8 * v:56 * part + 8 * v + 8]
                if q == 0 and part == 1 and v == 0:
                    X1[0].st(a * 256 + 112, jnp.where(row0, blk, 0.0))
                    blk = jnp.where(row0, 0.0, blk)
                X1[0].st(a * 256 + 128 * part + 16 * v + q, blk, stride=2)

    def dftd_o(a):
        lhs = jnp.concatenate([_bf(fd_v[112:224, :]), _bf(fd_v[224:336, :])], axis=1)
        rhs = jnp.concatenate(eos[a][2] + [jnp.zeros((32, 128), f32)], axis=0).astype(bf16)
        r = jnp.dot(lhs, rhs, preferred_element_type=f32) * rstd[a]
        X1[1].st(a * 256, r[:DQ])
        X1[1].st(a * 256 + 128, r[DQ:])

    def fwd_tile(a):
        if a % 2 == 0:
            dftd_e(a, 0)
            dftd_e(a, 1)
            dftd_o(a)
        else:
            dftd_o(a)
            dftd_e(a, 0)
            dftd_e(a, 1)

    def rad_fwd(p, j):
        r = 8 * j
        re = [X1[p].ld(a * 256 + r, 8) for a in range(16)]
        only_nyq = p == 0 and j == 14
        im = [None if only_nyq else X1[p].ld(a * 256 + 128 + r, 8) for a in range(16)]
        ore, oim = _fft16(re, im, -1)
        for k1 in range(16):
            Y[p].st(k1 * 256 + r, ore[k1])
            Y[p].st(k1 * 256 + 128 + r, oim[k1])

    def cmul3(km, conj, a, b, dims):
        gr, gi, gs = _bf(g_v[km, 0:64, :]), _bf(g_v[km, 64:128, :]), _bf(gs_v[km])
        m1 = lax.dot_general(gr, a.astype(bf16), dims, preferred_element_type=f32)
        m2 = lax.dot_general(gi, b.astype(bf16), dims, preferred_element_type=f32)
        if conj:
            m3 = lax.dot_general(gs, (b - a).astype(bf16), dims, preferred_element_type=f32)
            return m1 + m2, m3 + (m1 - m2)
        m3 = lax.dot_general(gs, (a + b).astype(bf16), dims, preferred_element_type=f32)
        return m1 - m2, m3 - (m1 + m2)

    def dft128(p, k1):
        n = 112 if p else 120
        pad = jnp.zeros((128 - n, 128), f32)
        yr = jnp.concatenate([Y[p].ld(k1 * 256, n), pad], axis=0)
        yi = jnp.concatenate([Y[p].ld(k1 * 256 + 128, n), pad], axis=0)
        xr, xi = cmul3(k1 if k1 < 8 else 16 - k1, k1 >= 8, yr, yi, NT_DIMS)
        X2[p].st(k1 * 256, xr)
        X2[p].st(k1 * 256 + 128, xi)

    def wprep(w_v, wt_v, a):
        w32 = pltpu.bitcast(w_v[0:DH, a * 128:(a + 1) * 128], u32)
        ny = jnp.broadcast_to(w_v[DH:DH + 1, a * 128:(a + 1) * 128].astype(f32), (8, 128))
        ny = lax.shift_right_logical(lax.bitcast_convert_type(ny, u32), np.uint32(16))
        tile = jnp.concatenate([w32, jnp.where(row0, ny, np.uint32(0)), jnp.zeros((8, 128), u32)], axis=0).T
        for j in range(8):
            wt_v[pl.ds(a * WP + 17 * j, 8), :] = tile[16 * j:16 * j + 8, :]
            wt_v[pl.ds((15 - a) * WP + 17 * (7 - j) + 8, 8), :] = tile[16 * j + 8:16 * j + 16, :]

    def idft128(p, k1):
        wr32 = jnp.concatenate([wtr_v[pl.ds(a * WP + k1, 8, stride=17), :] for a in range(16)], axis=0)
        wi32 = jnp.concatenate([wti_v[pl.ds(a * WP + k1, 8, stride=17), :] for a in range(16)], axis=0)
        wr, wi = (_hi(wr32), _hi(wi32)) if p else (_lo(wr32), _lo(wi32))
        xr, xi = X2[p].ld(k1 * 256, 128), X2[p].ld(k1 * 256 + 128, 128)
        vr, vi = cmul3(k1 if k1 < 8 else 16 - k1, k1 < 8, xr * wr - xi * wi, xr * wi + xi * wr, TN_DIMS)
        vb, r0 = vbuf(p, k1)
        vb.st(r0, vr)
        vb.st(r0 + 128, vi)

    def rad_inv(p, j):
        r = 8 * j
        src = [vbuf(p, k1) for k1 in range(16)]
        re = [vb.ld(r0 + r, 8) for vb, r0 in src]
        im = [vb.ld(r0 + 128 + r, 8) for vb, r0 in src]
        ore, oim = _fft16(re, im, +1)
        for s1 in range(16):
            Z[p].st(s1 * 256 + r, ore[s1])
            Z[p].st(s1 * 256 + 128 + r, oim[s1])

    def idftd(p, zb, a):
        z = jnp.concatenate([zb.ld(a * 256, 128), zb.ld(a * 256 + 128, 128)], axis=1).astype(bf16)
        lhs = jnp.concatenate([_bf(bd_v[p, 0]), _bf(bd_v[p, 1])], axis=1)
        return lax.dot_general(lhs, z, NT_DIMS, preferred_element_type=f32)

    def cols(ch, t=0, n=CW):
        if isinstance(ch, int):
            return pl.ds(ch * CW + t * 128, n)
        return pl.ds(pl.multiple_of(ch * CW, CW) + t * 128, n)

    def hrows(ch, t, r=0, n=D):
        if isinstance(ch, int):
            return pl.ds((ch * TPC + t) * D + r, n)
        return pl.ds(pl.multiple_of(ch * (TPC * D), 16) + (t * D + r), n)

    def prologue(ch, to_mem):
        zo, he = Z[PB].at_rows(ch * (TPC * 256), TPC * 256), HE.at_rows(ch * (TPC * DH), TPC * DH)
        means, scales = [], []
        for t in range(TPC):
            e = idftd(PB, zo, t)
            o = he.ld(t * DH, DH)
            x = x_v[:, cols(ch, t, 128)].astype(f32)
            acc = [None] * 4
            for j in range(DH // 16):
                ej, oj = e[16 * j:16 * j + 16], o[16 * j:16 * j + 16]
                for k, (r, y) in enumerate(((16 * j, ej + oj), (DH + 16 * j, ej - oj))):
                    hb = (x[r:r + 16] + y).astype(bf16)
                    hb_v[hrows(ch, t, r, 16), :] = hb
                    q = (2 * j + k) % 4
                    acc[q] = hb.astype(f32) if acc[q] is None else acc[q] + hb.astype(f32)
            means.append(_colsum((acc[0] + acc[1]) + (acc[2] + acc[3])) * (1.0 / D))
        for t in range(TPC):
            acc = [None] * 4
            for j in range(D // 16):
                d = hb_v[hrows(ch, t, 16 * j, 16), :].astype(f32) - means[t]
                acc[j % 4] = d * d if acc[j % 4] is None else acc[j % 4] + d * d
            scales.append(lax.rsqrt(_colsum((acc[0] + acc[1]) + (acc[2] + acc[3])) * (1.0 / D) + EPS))
        hn = [(hb_v[hrows(ch, t), :].astype(f32) - means[t]) * scales[t] for t in range(TPC)]
        hn = jnp.concatenate(hn, axis=1).astype(bf16)
        if to_mem:
            hn_v[:, cols(ch)] = hn
            return None
        return hn

    def mlp(ch, hn, with_next):
        if hn is None:
            hn = hn_v[:, cols(ch)]
        nxt = prologue(ch + 1, False) if with_next else None
        g = lax.dot_general(hn, wg_v[...], TN_DIMS, preferred_element_type=f32)
        u = lax.dot_general(hn, wu_v[...], TN_DIMS, preferred_element_type=f32)
        hh = (g * u).astype(bf16)
        for t in range(TPC):
            y = lax.dot_general(wd_v[...], hh[t * 128:(t + 1) * 128], NT_DIMS, preferred_element_type=f32)
            h = hb_v[hrows(ch, t), :].astype(f32)
            out_v[:, cols(ch, t, 128)] = (h + y.astype(bf16).astype(f32)).astype(bf16)
            pltpu.make_async_copy(out_v.at[:, cols(ch, t, 128)], out_hbm.at[:, cols(ch, t, 128)], out_sem).start()
        return nxt

    last = NT - NT // XC
    ln1(0)
    for a in range(1, last):
        if a % (NT // XC) == 0:
            x_cp[a // (NT // XC)].wait()
        fwd_tile(a - 1)
        ln1(a)
    x_cp[XC - 1].wait()
    for a in range(last, NT):
        ln1(a)
    for a in range(last - 1, NT):
        dftd_o(a)
    for a in range(last - 1, NT):
        dftd_e(a, 0)
        dftd_e(a, 1)
    for j in range(14):
        rad_fwd(1, j)
    cp_wr.wait()
    for q in range(32):
        if q == 24:
            cp_wi.wait()
        dft128((PA, PB)[q // 16], q % 16)
        if 1 <= q < 16:
            rad_fwd(0, q - 1)
        if q >= 16:
            for a in (2 * (q % 8), 2 * (q % 8) + 1):
                wprep(*((wr_v, wtr_v) if q < 24 else (wi_v, wti_v)), a)
    cp_bar.wait()
    for k1 in range(16):
        idft128(PA, k1)
    for k1 in range(16):
        idft128(PB, k1)
        if k1 < 8:
            rad_inv(PA, 2 * k1)
            rad_inv(PA, 2 * k1 + 1)
    for a in range(NT):
        HE.st(a * DH, idftd(PA, Z[PA], a))
        rad_inv(PB, a)
    for ch in range(0, NT // TPC, UNROLL):
        prologue(ch, True)
    for cp in cp_mlp:
        cp.wait()

    def body(it, carry):
        hn = None
        for k in range(UNROLL):
            hn = mlp(it * UNROLL + k, hn, k < UNROLL - 1)
        return carry

    lax.fori_loop(0, NT // TPC // UNROLL, body, 0)
    pltpu.make_async_copy(out_v, out_hbm, out_sem).wait()


@jax.jit
def pallas_sequential_preLN__spectral_gfnet__glu_gated_bilinear__prompt_kernel(
    A_x: jax.Array,
    A_w_r: jax.Array,
    A_w_i: jax.Array,
    B_x: jax.Array,
    B_w_gate: jax.Array,
    B_w_up: jax.Array,
    B_w_down: jax.Array,
):
    del B_x
    zc = np.zeros((24, 128), np.int32)
    zc[16:] = np.arange(128)
    any_spec = pl.BlockSpec(memory_space=pl.ANY)
    vm = pltpu.VMEM
    out_t = pl.pallas_call(
        _kernel,
        out_shape=jax.ShapeDtypeStruct((D, S), bf16),
        in_specs=[any_spec] * 7,
        out_specs=any_spec,
        scratch_shapes=[
            vm((D, S), bf16), vm((DH + 1, S), bf16), vm((DH + 1, S), bf16),
            vm((D, F), bf16), vm((D, F), bf16), vm((D, F), bf16),
            vm((24, 128), jnp.int32), vm((8, 128), jnp.int32),
            vm((FD_ROWS, 128), u32), vm((9, 128, 128), u32), vm((9, 64, 128), u32), vm((2, 2, DH // 2, 128), u32),
            vm((16 * WP + 16, 128), u32), vm((16 * WP + 16, 128), u32),
            vm((D, S), bf16), vm((D, S), bf16), vm((NT * D, 128), bf16),
            pltpu.SemaphoreType.DMA((XC + 5,)),
        ] + [vm((sum(_ROWS[n] for n in group), 128), u32) for group in _GROUPS],
        compiler_params=pltpu.CompilerParams(vmem_limit_bytes=100 * 2**20),
        name="gfnet_glu",
    )(A_x.reshape(S, D).T, A_w_r.T, A_w_i.T, B_w_gate, B_w_up, B_w_down.T, zc)
    return out_t.T.reshape(1, S, D)
```

```python
import numpy as np
import jax
import jax.numpy as jnp
from jax import lax
from jax.experimental import pallas as pl
from jax.experimental.pallas import tpu as pltpu

S, D, F = 2048, 448, 1792
DH, DQ = D // 2, D // 4
NT = S // 128
EPS = 1e-5
bf16, f32, u32 = jnp.bfloat16, jnp.float32, jnp.uint32
NT_DIMS = (((1,), (1,)), ((), ()))
TN_DIMS = (((0,), (0,)), ((), ()))
XC = 4
WP = 136
TPC = 2
CW = TPC * 128
UNROLL = 4
NVOB = 2
FD_ROWS = 56 + 56 + 2 * 112

PA, PB = 1, 0
_GROUPS = (("YE", "YO"), ("V2", "ZE", "ZO"), ("X1E",), ("X1O",), ("X2E",), ("X2O",), ("V1",), ("VOB",), ("HE",))
_ROWS = dict(X1E=4096, X1O=4096, YE=4096, YO=4096, X2E=4096, X2O=4096, V1=4096, V2=4096, ZE=4096, ZO=4096,
             VOB=NVOB * 256, HE=NT * DH)


def _cis(n, period):
    nf = n.astype(f32)
    r = nf - jnp.floor(nf * np.float32(1.0 / period) + 0.5) * np.float32(period)
    ang = r * np.float32(2 * np.pi / period)
    return jnp.cos(ang), -jnp.sin(ang)


def _cmul(a, b):
    return a[0] * b[0] - a[1] * b[1], a[0] * b[1] + a[1] * b[0]


def _geom(base, step, n):
    out = [base]
    for _ in range(n - 1):
        out.append(_cmul(out[-1], step))
    return out


def _pack_rows(vregs):
    return pltpu.bitcast(jnp.concatenate(vregs, axis=0).astype(bf16), u32)


def _bf(w):
    return pltpu.bitcast(w, bf16)


def _lo(w):
    return lax.bitcast_convert_type(lax.shift_left(w, np.uint32(16)), f32)


def _hi(w):
    return lax.bitcast_convert_type(w & np.uint32(0xFFFF0000), f32)


class _V:
    __slots__ = ("a", "n")

    def __init__(self, a, n=False):
        self.a, self.n = a, n

    def __neg__(self):
        return _V(self.a, not self.n)

    def __add__(self, o):
        if o.a is None:
            return self
        if self.a is None:
            return o
        if self.n == o.n:
            return _V(self.a + o.a, self.n)
        return _V(o.a - self.a) if self.n else _V(self.a - o.a)

    def __sub__(self, o):
        return self + (-o)

    def mul(self, c):
        return self if self.a is None else _V(self.a * np.float32(-c if self.n else c))

    def val(self, like):
        if self.a is None:
            return jnp.zeros_like(like)
        return -self.a if self.n else self.a


def _r4(x, sg):
    (x0r, x0i), (x1r, x1i), (x2r, x2i), (x3r, x3i) = x
    t0r, t0i, t1r, t1i = x0r + x2r, x0i + x2i, x0r - x2r, x0i - x2i
    t2r, t2i, t3r, t3i = x1r + x3r, x1i + x3i, x1r - x3r, x1i - x3i
    ur, ui = (-t3i, t3r) if sg > 0 else (t3i, -t3r)
    return [(t0r + t2r, t0i + t2i), (t1r + ur, t1i + ui), (t0r - t2r, t0i - t2i), (t1r - ur, t1i - ui)]


def _tw(x, e, sg):
    xr, xi = x
    if e % 4 == 0:
        q = (sg * (e // 4)) % 4
        return [(xr, xi), (-xi, xr), (-xr, -xi), (xi, -xr)][q]
    c, s = np.cos(2 * np.pi * e / 16), sg * np.sin(2 * np.pi * e / 16)
    if e % 2 == 0:
        sc = (lambda v: v) if c > 0 else (lambda v: -v)
        ss = (lambda v: v) if s > 0 else (lambda v: -v)
        return (sc(xr) - ss(xi)).mul(abs(c)), (sc(xi) + ss(xr)).mul(abs(c))
    return xr.mul(c) - xi.mul(s), xi.mul(c) + xr.mul(s)


def _fft16(re, im, sg):
    x = [(_V(re[a]), _V(im[a])) for a in range(16)]
    t = [_r4([x[4 * a1 + a0] for a1 in range(4)], sg) for a0 in range(4)]
    out_re, out_im = [None] * 16, [None] * 16
    for k0 in range(4):
        y = _r4([_tw(t[a0][k0], a0 * k0, sg) for a0 in range(4)], sg)
        for k1 in range(4):
            out_re[k0 + 4 * k1] = y[k1][0].val(re[0])
            out_im[k0 + 4 * k1] = y[k1][1].val(re[0])
    return out_re, out_im


def _colsum(x):
    parts = [x[i:i + 8] for i in range(0, x.shape[0], 8)]
    while len(parts) > 1:
        nxt = [parts[i] + parts[i + 1] for i in range(0, len(parts) - 1, 2)]
        if len(parts) % 2:
            nxt.append(parts[-1])
        parts = nxt
    return jnp.sum(parts[0], axis=0, keepdims=True)


class _Buf:
    def __init__(self, ref, zs, zl, off=0, n=None, views=None):
        self.ref, self.zs, self.zl, self.off = ref, zs, zl, off
        self.sv, self.lv = views or (ref.at[pl.ds(zs, n)], ref.at[pl.ds(zl, n)])

    def at_rows(self, start, n):
        if isinstance(start, int):
            return _Buf(self.ref, self.zs, self.zl, self.off + start, views=(self.sv, self.lv))
        base = pl.multiple_of(self.off + start, 8)
        return _Buf(self.ref, self.zs + base, self.zl + base, n=n)

    def st(self, row, val, stride=None):
        row += self.off
        idx = pl.ds(row, val.shape[0]) if stride is None else pl.ds(row, val.shape[0], stride=stride)
        self.sv[idx, :] = lax.bitcast_convert_type(val, u32)

    def ld(self, row, n):
        row += self.off
        return lax.bitcast_convert_type(self.lv[row:row + n, :], f32)


def _kernel(x_hbm, wr_hbm, wi_hbm, wg_hbm, wu_hbm, wd_hbm, z_hbm, out_hbm,
            x_v, wr_v, wi_v, wg_v, wu_v, wd_v, z_v, zb_v, fd_v, g_v, gs_v, bd_v,
            wtr_v, wti_v, out_v, hn_v, hb_v, sems, *arenas):
    xw = S // XC
    x_cp = [pltpu.make_async_copy(x_hbm.at[:, pl.ds(c * xw, xw)], x_v.at[:, pl.ds(c * xw, xw)], sems.at[c])
            for c in range(XC)]
    cp_z = pltpu.make_async_copy(z_hbm, z_v, sems.at[0])
    cp_wr = pltpu.make_async_copy(wr_hbm, wr_v, sems.at[XC])
    cp_wi = pltpu.make_async_copy(wi_hbm, wi_v, sems.at[XC + 1])
    cp_mlp = [pltpu.make_async_copy(h, v, sems.at[XC + 2]) for h, v in ((wg_hbm, wg_v), (wu_hbm, wu_v), (wd_hbm, wd_v))]
    out_sem = sems.at[XC + 3]
    cp_bar = pltpu.make_async_copy(z_hbm.at[pl.ds(0, 8)], zb_v, sems.at[XC + 4])
    for cp in [cp_z, cp_bar] + x_cp + [cp_wr, cp_wi] + cp_mlp:
        cp.start()

    i = lax.broadcasted_iota(jnp.int32, (8, 128), 0)
    c = lax.broadcasted_iota(jnp.int32, (8, 128), 1)
    f = _geom(_cis(i * c, 128), _cis(8 * c, 128), 16)
    t1 = _cis(c, S)
    t = t1
    for km in range(9):
        g = f
        if km:
            if km > 1:
                t = _cmul(t, t1)
            g = [_cmul(e, t) for e in f]
        g_v[km, 0:64, :] = _pack_rows([e[0] for e in g])
        g_v[km, 64:128, :] = _pack_rows([e[1] for e in g])
        gs_v[km] = _pack_rows([e[0] + e[1] for e in g])
    b0, st0 = _cis(4 * i * c, D), _cis(32 * c, D)
    e0 = _geom(b0, st0, 7)
    e2 = _geom(_cmul(b0, _cis(2 * c, D)), st0, 7)
    nyq = (1 - 2 * (c & 1)).astype(f32)
    fd_v[0:56, :] = _pack_rows([e[0] for e in e0] + [jnp.where(i == 0, nyq, e0[0][1])] + [e[1] for e in e0[1:]])
    fd_v[56:112, :] = _pack_rows([e[0] for e in e2] + [e[1] for e in e2])
    for kt in range(2):
        dd = c + 128 * kt
        eo = _geom(_cis((2 * i + 1) * dd, D), _cis(16 * dd, D), 14)
        fd_v[112 + 112 * kt:224 + 112 * kt, :] = _pack_rows([e[0] for e in eo] + [e[1] for e in eo])
    sc = np.float32(1.0 / (D * S))
    for p in range(2):
        kd = 2 * c + p
        if p == 0:
            wgt = jnp.where((c == 0) | (c == DQ), sc, jnp.where(c < DQ, 2 * sc, np.float32(0)))
        else:
            wgt = jnp.where(c < DQ, 2 * sc, np.float32(0))
        base, step = _cis(kd * i, D), _cis(8 * kd, D)
        if p == 0:
            base = (base[0], jnp.where(c == DQ, np.float32(0), base[1]))
            step = (step[0], jnp.where(c == DQ, np.float32(0), step[1]))
        e = _geom((base[0] * wgt, base[1] * wgt), step, DH // 8)
        bd_v[p, 0] = _pack_rows([v[0] for v in e])
        bd_v[p, 1] = _pack_rows([v[1] for v in e])

    cp_z.wait()
    x_cp[0].wait()
    zz = z_v[0:16, :]
    z1 = pl.multiple_of(jnp.max(zz[0:8]), 8)
    z2 = pl.multiple_of(jnp.max(zz[8:16]), 8)
    bufs = {}
    for ref, group in zip(arenas, _GROUPS):
        whole = _Buf(ref, z1, z2, n=ref.shape[0])
        off = 0
        for name in group:
            bufs[name] = whole.at_rows(off, _ROWS[name])
            off += _ROWS[name]
    X1, Y = (bufs["X1E"], bufs["X1O"]), (bufs["YE"], bufs["YO"])
    X2, Z, HE = (bufs["X2E"], bufs["X2O"]), (bufs["ZE"], bufs["ZO"]), bufs["HE"]

    def vbuf(p, k1):
        if p == PA:
            return bufs["V1"], k1 * 256
        if k1 >= 16 - NVOB:
            return bufs["VOB"], (k1 - (16 - NVOB)) * 256
        return bufs["V2"], k1 * 256

    rstd, eos = [None] * NT, [None] * NT

    def ln1(a):
        x = x_v[:, a * 128:(a + 1) * 128].astype(f32)
        a0, a2s, dl, dh = [], [], [], []
        acc = [None] * 4

        def add(k, v):
            acc[k] = v if acc[k] is None else acc[k] + v

        for j in range(DQ // 16):
            x0, x1, x2, x3 = (x[q * DQ + 16 * j:q * DQ + 16 * j + 16] for q in range(4))
            s02, s13, d02, d13 = x0 + x2, x1 + x3, x0 - x2, x1 - x3
            a2 = s02 - s13
            a0.append(s02 + s13)
            a2s.append(a2)
            dl.append(d02)
            dh.append(d13)
            add(0, d02 * d02)
            add(1, d13 * d13)
            add(2, a2 * a2)
        m4 = _colsum(jnp.concatenate(a0, axis=0)) * (4.0 / D)
        a0c = [v - m4 for v in a0]
        for v in a0c:
            add(3, v * v)
        var = _colsum((acc[0] + acc[1]) * 2.0 + (acc[2] + acc[3])) * (0.25 / D)
        rstd[a] = lax.rsqrt(var + EPS)
        eos[a] = (a0c, a2s, dl + dh)

    row0 = lax.broadcasted_iota(jnp.int32, (8, 128), 0) == 0

    def dftd_e(a, q):
        rhs = jnp.concatenate(eos[a][q] + [jnp.zeros((16, 128), f32)], axis=0).astype(bf16)
        r = jnp.dot(_bf(fd_v[56 * q:56 * q + 56, :]), rhs, preferred_element_type=f32) * rstd[a]
        for part in range(2):
            for v in range(7):
                blk = r[56 * part + 8 * v:56 * part + 8 * v + 8]
                if q == 0 and part == 1 and v == 0:
                    X1[0].st(a * 256 + 112, jnp.where(row0, blk, 0.0))
                    blk = jnp.where(row0, 0.0, blk)
                X1[0].st(a * 256 + 128 * part + 16 * v + q, blk, stride=2)

    def dftd_o(a):
        lhs = jnp.concatenate([_bf(fd_v[112:224, :]), _bf(fd_v[224:336, :])], axis=1)
        rhs = jnp.concatenate(eos[a][2] + [jnp.zeros((32, 128), f32)], axis=0).astype(bf16)
        r = jnp.dot(lhs, rhs, preferred_element_type=f32) * rstd[a]
        X1[1].st(a * 256, r[:DQ])
        X1[1].st(a * 256 + 128, r[DQ:])

    def fwd_tile(a):
        if a % 2 == 0:
            dftd_e(a, 0)
            dftd_e(a, 1)
            dftd_o(a)
        else:
            dftd_o(a)
            dftd_e(a, 0)
            dftd_e(a, 1)

    def rad_fwd(p, j):
        r = 8 * j
        re = [X1[p].ld(a * 256 + r, 8) for a in range(16)]
        only_nyq = p == 0 and j == 14
        im = [None if only_nyq else X1[p].ld(a * 256 + 128 + r, 8) for a in range(16)]
        ore, oim = _fft16(re, im, -1)
        for k1 in range(16):
            Y[p].st(k1 * 256 + r, ore[k1])
            Y[p].st(k1 * 256 + 128 + r, oim[k1])

    def cmul3(km, conj, a, b, dims):
        gr, gi, gs = _bf(g_v[km, 0:64, :]), _bf(g_v[km, 64:128, :]), _bf(gs_v[km])
        m1 = lax.dot_general(gr, a.astype(bf16), dims, preferred_element_type=f32)
        m2 = lax.dot_general(gi, b.astype(bf16), dims, preferred_element_type=f32)
        if conj:
            m3 = lax.dot_general(gs, (b - a).astype(bf16), dims, preferred_element_type=f32)
            return m1 + m2, m3 + (m1 - m2)
        m3 = lax.dot_general(gs, (a + b).astype(bf16), dims, preferred_element_type=f32)
        return m1 - m2, m3 - (m1 + m2)

    def dft128(p, k1):
        n = 112 if p else 120
        pad = jnp.zeros((128 - n, 128), f32)
        yr = jnp.concatenate([Y[p].ld(k1 * 256, n), pad], axis=0)
        yi = jnp.concatenate([Y[p].ld(k1 * 256 + 128, n), pad], axis=0)
        xr, xi = cmul3(k1 if k1 < 8 else 16 - k1, k1 >= 8, yr, yi, NT_DIMS)
        X2[p].st(k1 * 256, xr)
        X2[p].st(k1 * 256 + 128, xi)

    def wprep(w_v, wt_v, a):
        w32 = pltpu.bitcast(w_v[0:DH, a * 128:(a + 1) * 128], u32)
        ny = jnp.broadcast_to(w_v[DH:DH + 1, a * 128:(a + 1) * 128].astype(f32), (8, 128))
        ny = lax.shift_right_logical(lax.bitcast_convert_type(ny, u32), np.uint32(16))
        tile = jnp.concatenate([w32, jnp.where(row0, ny, np.uint32(0)), jnp.zeros((8, 128), u32)], axis=0).T
        for j in range(8):
            wt_v[pl.ds(a * WP + 17 * j, 8), :] = tile[16 * j:16 * j + 8, :]
            wt_v[pl.ds((15 - a) * WP + 17 * (7 - j) + 8, 8), :] = tile[16 * j + 8:16 * j + 16, :]

    def idft128(p, k1):
        wr32 = jnp.concatenate([wtr_v[pl.ds(a * WP + k1, 8, stride=17), :] for a in range(16)], axis=0)
        wi32 = jnp.concatenate([wti_v[pl.ds(a * WP + k1, 8, stride=17), :] for a in range(16)], axis=0)
        wr, wi = (_hi(wr32), _hi(wi32)) if p else (_lo(wr32), _lo(wi32))
        xr, xi = X2[p].ld(k1 * 256, 128), X2[p].ld(k1 * 256 + 128, 128)
        vr, vi = cmul3(k1 if k1 < 8 else 16 - k1, k1 < 8, xr * wr - xi * wi, xr * wi + xi * wr, TN_DIMS)
        vb, r0 = vbuf(p, k1)
        vb.st(r0, vr)
        vb.st(r0 + 128, vi)

    def rad_inv(p, j):
        r = 8 * j
        src = [vbuf(p, k1) for k1 in range(16)]
        re = [vb.ld(r0 + r, 8) for vb, r0 in src]
        im = [vb.ld(r0 + 128 + r, 8) for vb, r0 in src]
        ore, oim = _fft16(re, im, +1)
        for s1 in range(16):
            Z[p].st(s1 * 256 + r, ore[s1])
            Z[p].st(s1 * 256 + 128 + r, oim[s1])

    def idftd(p, zb, a):
        z = jnp.concatenate([zb.ld(a * 256, 128), zb.ld(a * 256 + 128, 128)], axis=1).astype(bf16)
        lhs = jnp.concatenate([_bf(bd_v[p, 0]), _bf(bd_v[p, 1])], axis=1)
        return lax.dot_general(lhs, z, NT_DIMS, preferred_element_type=f32)

    def cols(ch, t=0, n=CW):
        if isinstance(ch, int):
            return pl.ds(ch * CW + t * 128, n)
        return pl.ds(pl.multiple_of(ch * CW, CW) + t * 128, n)

    def prologue(ch, to_mem):
        zo, he = Z[PB].at_rows(ch * (TPC * 256), TPC * 256), HE.at_rows(ch * (TPC * DH), TPC * DH)
        e = jnp.concatenate([idftd(PB, zo, t) for t in range(TPC)], axis=1)
        o = jnp.concatenate([he.ld(t * DH, DH) for t in range(TPC)], axis=1)
        acc = [None] * 4
        for j in range(DH // 16):
            ej, oj = e[16 * j:16 * j + 16], o[16 * j:16 * j + 16]
            for k, (r, y) in enumerate(((16 * j, ej + oj), (DH + 16 * j, ej - oj))):
                hs = x_v[r:r + 16, cols(ch)].astype(f32) + y
                hb_v[r:r + 16, cols(ch)] = hs.astype(bf16)
                q = (2 * j + k) % 4
                acc[q] = hs if acc[q] is None else acc[q] + hs
        mean = _colsum((acc[0] + acc[1]) + (acc[2] + acc[3])) * (1.0 / D)
        acc = [None] * 4
        for j in range(D // 16):
            d = hb_v[16 * j:16 * j + 16, cols(ch)].astype(f32) - mean
            acc[j % 4] = d * d if acc[j % 4] is None else acc[j % 4] + d * d
        scale = lax.rsqrt(_colsum((acc[0] + acc[1]) + (acc[2] + acc[3])) * (1.0 / D) + EPS)
        hn = ((hb_v[:, cols(ch)].astype(f32) - mean) * scale).astype(bf16)
        if to_mem:
            hn_v[:, cols(ch)] = hn
            return None
        return hn

    def mlp(ch, hn, with_next):
        if hn is None:
            hn = hn_v[:, cols(ch)]
        nxt = prologue(ch + 1, False) if with_next else None
        g = lax.dot_general(hn, wg_v[...], TN_DIMS, preferred_element_type=f32)
        u = lax.dot_general(hn, wu_v[...], TN_DIMS, preferred_element_type=f32)
        hh = (g * u).astype(bf16)
        for t in range(TPC):
            y = lax.dot_general(wd_v[...], hh[t * 128:(t + 1) * 128], NT_DIMS, preferred_element_type=f32)
            h = hb_v[:, cols(ch, t, 128)].astype(f32)
            out_v[:, cols(ch, t, 128)] = (h + y.astype(bf16).astype(f32)).astype(bf16)
            pltpu.make_async_copy(out_v.at[:, cols(ch, t, 128)], out_hbm.at[:, cols(ch, t, 128)], out_sem).start()
        return nxt

    last = NT - NT // XC
    ln1(0)
    for a in range(1, last):
        if a % (NT // XC) == 0:
            x_cp[a // (NT // XC)].wait()
        fwd_tile(a - 1)
        ln1(a)
    x_cp[XC - 1].wait()
    for a in range(last, NT):
        ln1(a)
    for a in range(last - 1, NT):
        dftd_o(a)
    for a in range(last - 1, NT):
        dftd_e(a, 0)
        dftd_e(a, 1)
    for j in range(14):
        rad_fwd(1, j)
    cp_wr.wait()
    for q in range(32):
        if q == 24:
            cp_wi.wait()
        dft128((PA, PB)[q // 16], q % 16)
        if 1 <= q < 16:
            rad_fwd(0, q - 1)
        if q >= 16:
            for a in (2 * (q % 8), 2 * (q % 8) + 1):
                wprep(*((wr_v, wtr_v) if q < 24 else (wi_v, wti_v)), a)
    cp_bar.wait()
    for k1 in range(16):
        idft128(PA, k1)
    for k1 in range(16):
        idft128(PB, k1)
        if k1 < 8:
            rad_inv(PA, 2 * k1)
            rad_inv(PA, 2 * k1 + 1)
    for a in range(NT):
        HE.st(a * DH, idftd(PA, Z[PA], a))
        rad_inv(PB, a)
    for ch in range(0, NT // TPC, UNROLL):
        prologue(ch, True)
    for cp in cp_mlp:
        cp.wait()

    def body(it, carry):
        hn = None
        for k in range(UNROLL):
            hn = mlp(it * UNROLL + k, hn, k < UNROLL - 1)
        return carry

    lax.fori_loop(0, NT // TPC // UNROLL, body, 0)
    pltpu.make_async_copy(out_v, out_hbm, out_sem).wait()


@jax.jit
def pallas_sequential_preLN__spectral_gfnet__glu_gated_bilinear__prompt_kernel(
    A_x: jax.Array,
    A_w_r: jax.Array,
    A_w_i: jax.Array,
    B_x: jax.Array,
    B_w_gate: jax.Array,
    B_w_up: jax.Array,
    B_w_down: jax.Array,
):
    del B_x
    zc = np.zeros((24, 128), np.int32)
    zc[16:] = np.arange(128)
    any_spec = pl.BlockSpec(memory_space=pl.ANY)
    vm = pltpu.VMEM
    out_t = pl.pallas_call(
        _kernel,
        out_shape=jax.ShapeDtypeStruct((D, S), bf16),
        in_specs=[any_spec] * 7,
        out_specs=any_spec,
        scratch_shapes=[
            vm((D, S), bf16), vm((DH + 1, S), bf16), vm((DH + 1, S), bf16),
            vm((D, F), bf16), vm((D, F), bf16), vm((D, F), bf16),
            vm((24, 128), jnp.int32), vm((8, 128), jnp.int32),
            vm((FD_ROWS, 128), u32), vm((9, 128, 128), u32), vm((9, 64, 128), u32), vm((2, 2, DH // 2, 128), u32),
            vm((16 * WP + 16, 128), u32), vm((16 * WP + 16, 128), u32),
            vm((D, S), bf16), vm((D, S), bf16), vm((D, S), bf16),
            pltpu.SemaphoreType.DMA((XC + 5,)),
        ] + [vm((sum(_ROWS[n] for n in group), 128), u32) for group in _GROUPS],
        compiler_params=pltpu.CompilerParams(vmem_limit_bytes=100 * 2**20),
        name="gfnet_glu",
    )(A_x.reshape(S, D).T, A_w_r.T, A_w_i.T, B_w_gate, B_w_up, B_w_down.T, zc)
    return out_t.T.reshape(1, S, D)
```

```python
import numpy as np
import jax
import jax.numpy as jnp
from jax import lax
from jax.experimental import pallas as pl
from jax.experimental.pallas import tpu as pltpu

S, D, F = 2048, 448, 1792
DH, DQ = D // 2, D // 4
NT = S // 128
EPS = 1e-5
bf16, f32, u32 = jnp.bfloat16, jnp.float32, jnp.uint32
NT_DIMS = (((1,), (1,)), ((), ()))
TN_DIMS = (((0,), (0,)), ((), ()))
XC = 4
WP = 136
TPC = 2
CW = TPC * 128
UNROLL = 4
NVOB = 2
FD_ROWS = 56 + 56 + 2 * 112

N_IT = NT // TPC // UNROLL
PA, PB = 1, 0

_GROUPS = (("YE", "YO"), ("V2", "ZE", "ZO"), ("X1E",), ("X1O",), ("X2E",), ("X2O",), ("V1",), ("VOB",), ("HE",))
_ROWS = dict(X1E=4096, X1O=4096, YE=4096, YO=4096, X2E=4096, X2O=4096, V1=4096, V2=4096, ZE=4096, ZO=4096,
             VOB=NVOB * 256, HE=NT * DH)


def _cis(n, period):
    nf = n.astype(f32)
    r = nf - jnp.floor(nf * np.float32(1.0 / period) + 0.5) * np.float32(period)
    ang = r * np.float32(2 * np.pi / period)
    return jnp.cos(ang), -jnp.sin(ang)


def _cmul(a, b):
    return a[0] * b[0] - a[1] * b[1], a[0] * b[1] + a[1] * b[0]


def _geom(base, step, n):
    out = [base]
    for _ in range(n - 1):
        out.append(_cmul(out[-1], step))
    return out


def _pack_rows(vregs):
    return pltpu.bitcast(jnp.concatenate(vregs, axis=0).astype(bf16), u32)


def _bf(w):
    return pltpu.bitcast(w, bf16)


def _lo(w):
    return lax.bitcast_convert_type(lax.shift_left(w, np.uint32(16)), f32)


def _hi(w):
    return lax.bitcast_convert_type(w & np.uint32(0xFFFF0000), f32)


class _V:
    __slots__ = ("a", "n")

    def __init__(self, a, n=False):
        self.a, self.n = a, n

    def __neg__(self):
        return _V(self.a, not self.n)

    def __add__(self, o):
        if o.a is None:
            return self
        if self.a is None:
            return o
        if self.n == o.n:
            return _V(self.a + o.a, self.n)
        return _V(o.a - self.a) if self.n else _V(self.a - o.a)

    def __sub__(self, o):
        return self + (-o)

    def mul(self, c):
        return self if self.a is None else _V(self.a * np.float32(-c if self.n else c))

    def val(self, like):
        if self.a is None:
            return jnp.zeros_like(like)
        return -self.a if self.n else self.a


def _r4(x, sg):
    (x0r, x0i), (x1r, x1i), (x2r, x2i), (x3r, x3i) = x
    t0r, t0i, t1r, t1i = x0r + x2r, x0i + x2i, x0r - x2r, x0i - x2i
    t2r, t2i, t3r, t3i = x1r + x3r, x1i + x3i, x1r - x3r, x1i - x3i
    ur, ui = (-t3i, t3r) if sg > 0 else (t3i, -t3r)
    return [(t0r + t2r, t0i + t2i), (t1r + ur, t1i + ui), (t0r - t2r, t0i - t2i), (t1r - ur, t1i - ui)]


def _tw(x, e, sg):
    xr, xi = x
    if e % 4 == 0:
        q = (sg * (e // 4)) % 4
        return [(xr, xi), (-xi, xr), (-xr, -xi), (xi, -xr)][q]
    c, s = np.cos(2 * np.pi * e / 16), sg * np.sin(2 * np.pi * e / 16)
    if e % 2 == 0:
        sc = (lambda v: v) if c > 0 else (lambda v: -v)
        ss = (lambda v: v) if s > 0 else (lambda v: -v)
        return (sc(xr) - ss(xi)).mul(abs(c)), (sc(xi) + ss(xr)).mul(abs(c))
    return xr.mul(c) - xi.mul(s), xi.mul(c) + xr.mul(s)


def _fft16(re, im, sg):
    x = [(_V(re[a]), _V(im[a])) for a in range(16)]
    t = [_r4([x[4 * a1 + a0] for a1 in range(4)], sg) for a0 in range(4)]
    out_re, out_im = [None] * 16, [None] * 16
    for k0 in range(4):
        y = _r4([_tw(t[a0][k0], a0 * k0, sg) for a0 in range(4)], sg)
        for k1 in range(4):
            out_re[k0 + 4 * k1] = y[k1][0].val(re[0])
            out_im[k0 + 4 * k1] = y[k1][1].val(re[0])
    return out_re, out_im


def _colsum(x):
    parts = [x[i:i + 8] for i in range(0, x.shape[0], 8)]
    while len(parts) > 1:
        nxt = [parts[i] + parts[i + 1] for i in range(0, len(parts) - 1, 2)]
        if len(parts) % 2:
            nxt.append(parts[-1])
        parts = nxt
    return jnp.sum(parts[0], axis=0, keepdims=True)


class _Buf:
    def __init__(self, ref, zs, zl, off=0, n=None, views=None):
        self.ref, self.zs, self.zl, self.off = ref, zs, zl, off
        self.sv, self.lv = views or (ref.at[pl.ds(zs, n)], ref.at[pl.ds(zl, n)])

    def at_rows(self, start, n):
        if isinstance(start, int):
            return _Buf(self.ref, self.zs, self.zl, self.off + start, views=(self.sv, self.lv))
        base = pl.multiple_of(self.off + start, 8)
        return _Buf(self.ref, self.zs + base, self.zl + base, n=n)

    def st(self, row, val, stride=None):
        row += self.off
        idx = pl.ds(row, val.shape[0]) if stride is None else pl.ds(row, val.shape[0], stride=stride)
        self.sv[idx, :] = lax.bitcast_convert_type(val, u32)

    def ld(self, row, n):
        row += self.off
        return lax.bitcast_convert_type(self.lv[row:row + n, :], f32)


def _kernel(x_hbm, wr_hbm, wi_hbm, wg_hbm, wu_hbm, wd_hbm, z_hbm, out_hbm,
            x_v, wr_v, wi_v, wg_v, wu_v, wd_v, z_v, zb_v, fd_v, g_v, gs_v, bd_v,
            wtr_v, wti_v, out_v, hh_v, hb_v, sems, *arenas):
    xw = S // XC
    x_cp = [pltpu.make_async_copy(x_hbm.at[:, pl.ds(c * xw, xw)], x_v.at[:, pl.ds(c * xw, xw)], sems.at[c])
            for c in range(XC)]
    cp_z = pltpu.make_async_copy(z_hbm, z_v, sems.at[0])
    cp_wr = pltpu.make_async_copy(wr_hbm, wr_v, sems.at[XC])
    cp_wi = pltpu.make_async_copy(wi_hbm, wi_v, sems.at[XC + 1])
    cp_gu = [pltpu.make_async_copy(h, v, sems.at[XC + 2]) for h, v in ((wg_hbm, wg_v), (wu_hbm, wu_v))]
    cp_wd = pltpu.make_async_copy(wd_hbm, wd_v, sems.at[XC + 5])
    out_sem = sems.at[XC + 3]
    cp_bar = pltpu.make_async_copy(z_hbm.at[pl.ds(0, 8)], zb_v, sems.at[XC + 4])
    for cp in [cp_z, cp_bar] + x_cp + [cp_wr, cp_wi] + cp_gu + [cp_wd]:
        cp.start()

    i = lax.broadcasted_iota(jnp.int32, (8, 128), 0)
    c = lax.broadcasted_iota(jnp.int32, (8, 128), 1)
    f = _geom(_cis(i * c, 128), _cis(8 * c, 128), 16)
    t1 = _cis(c, S)
    t = t1
    for km in range(9):
        g = f
        if km:
            if km > 1:
                t = _cmul(t, t1)
            g = [_cmul(e, t) for e in f]
        g_v[km, 0:64, :] = _pack_rows([e[0] for e in g])
        g_v[km, 64:128, :] = _pack_rows([e[1] for e in g])
        gs_v[km] = _pack_rows([e[0] + e[1] for e in g])
    b0, st0 = _cis(4 * i * c, D), _cis(32 * c, D)
    e0 = _geom(b0, st0, 7)
    e2 = _geom(_cmul(b0, _cis(2 * c, D)), st0, 7)
    nyq = (1 - 2 * (c & 1)).astype(f32)
    fd_v[0:56, :] = _pack_rows([e[0] for e in e0] + [jnp.where(i == 0, nyq, e0[0][1])] + [e[1] for e in e0[1:]])
    fd_v[56:112, :] = _pack_rows([e[0] for e in e2] + [e[1] for e in e2])
    for kt in range(2):
        dd = c + 128 * kt
        eo = _geom(_cis((2 * i + 1) * dd, D), _cis(16 * dd, D), 14)
        fd_v[112 + 112 * kt:224 + 112 * kt, :] = _pack_rows([e[0] for e in eo] + [e[1] for e in eo])
    sc = np.float32(1.0 / (D * S))
    for p in range(2):
        kd = 2 * c + p
        if p == 0:
            wgt = jnp.where((c == 0) | (c == DQ), sc, jnp.where(c < DQ, 2 * sc, np.float32(0)))
        else:
            wgt = jnp.where(c < DQ, 2 * sc, np.float32(0))
        base, step = _cis(kd * i, D), _cis(8 * kd, D)
        if p == 0:
            base = (base[0], jnp.where(c == DQ, np.float32(0), base[1]))
            step = (step[0], jnp.where(c == DQ, np.float32(0), step[1]))
        e = _geom((base[0] * wgt, base[1] * wgt), step, DH // 8)
        bd_v[p, 0] = _pack_rows([v[0] for v in e])
        bd_v[p, 1] = _pack_rows([v[1] for v in e])

    cp_z.wait()
    x_cp[0].wait()
    zz = z_v[0:16, :]
    z1 = pl.multiple_of(jnp.max(zz[0:8]), 8)
    z2 = pl.multiple_of(jnp.max(zz[8:16]), 8)
    bufs = {}
    for ref, group in zip(arenas, _GROUPS):
        whole = _Buf(ref, z1, z2, n=ref.shape[0])
        off = 0
        for name in group:
            bufs[name] = whole.at_rows(off, _ROWS[name])
            off += _ROWS[name]
    X1, Y = (bufs["X1E"], bufs["X1O"]), (bufs["YE"], bufs["YO"])
    X2, Z, HE = (bufs["X2E"], bufs["X2O"]), (bufs["ZE"], bufs["ZO"]), bufs["HE"]

    def vbuf(p, k1):
        if p == PA:
            return bufs["V1"], k1 * 256
        if k1 >= 16 - NVOB:
            return bufs["VOB"], (k1 - (16 - NVOB)) * 256
        return bufs["V2"], k1 * 256

    rstd, eos = [None] * NT, [None] * NT

    def ln1(a):
        x = x_v[:, a * 128:(a + 1) * 128].astype(f32)
        a0, a2s, dl, dh = [], [], [], []
        acc = [None] * 4

        def add(k, v):
            acc[k] = v if acc[k] is None else acc[k] + v

        for j in range(DQ // 16):
            x0, x1, x2, x3 = (x[q * DQ + 16 * j:q * DQ + 16 * j + 16] for q in range(4))
            s02, s13, d02, d13 = x0 + x2, x1 + x3, x0 - x2, x1 - x3
            a2 = s02 - s13
            a0.append(s02 + s13)
            a2s.append(a2)
            dl.append(d02)
            dh.append(d13)
            add(0, d02 * d02)
            add(1, d13 * d13)
            add(2, a2 * a2)
        m4 = _colsum(jnp.concatenate(a0, axis=0)) * (4.0 / D)
        a0c = [v - m4 for v in a0]
        for v in a0c:
            add(3, v * v)
        var = _colsum((acc[0] + acc[1]) * 2.0 + (acc[2] + acc[3])) * (0.25 / D)
        rstd[a] = lax.rsqrt(var + EPS)
        eos[a] = (a0c, a2s, dl + dh)

    row0 = lax.broadcasted_iota(jnp.int32, (8, 128), 0) == 0

    def dftd_e(a, q):
        rhs = jnp.concatenate(eos[a][q] + [jnp.zeros((16, 128), f32)], axis=0).astype(bf16)
        r = jnp.dot(_bf(fd_v[56 * q:56 * q + 56, :]), rhs, preferred_element_type=f32) * rstd[a]
        for part in range(2):
            for v in range(7):
                blk = r[56 * part + 8 * v:56 * part + 8 * v + 8]
                if q == 0 and part == 1 and v == 0:
                    X1[0].st(a * 256 + 112, jnp.where(row0, blk, 0.0))
                    blk = jnp.where(row0, 0.0, blk)
                X1[0].st(a * 256 + 128 * part + 16 * v + q, blk, stride=2)

    def dftd_o(a):
        lhs = jnp.concatenate([_bf(fd_v[112:224, :]), _bf(fd_v[224:336, :])], axis=1)
        rhs = jnp.concatenate(eos[a][2] + [jnp.zeros((32, 128), f32)], axis=0).astype(bf16)
        r = jnp.dot(lhs, rhs, preferred_element_type=f32) * rstd[a]
        X1[1].st(a * 256, r[:DQ])
        X1[1].st(a * 256 + 128, r[DQ:])

    def fwd_tile(a):
        if a % 2 == 0:
            dftd_e(a, 0)
            dftd_e(a, 1)
            dftd_o(a)
        else:
            dftd_o(a)
            dftd_e(a, 0)
            dftd_e(a, 1)

    def rad_fwd(p, j):
        r = 8 * j
        re = [X1[p].ld(a * 256 + r, 8) for a in range(16)]
        only_nyq = p == 0 and j == 14
        im = [None if only_nyq else X1[p].ld(a * 256 + 128 + r, 8) for a in range(16)]
        ore, oim = _fft16(re, im, -1)
        for k1 in range(16):
            Y[p].st(k1 * 256 + r, ore[k1])
            Y[p].st(k1 * 256 + 128 + r, oim[k1])

    def cmul3(km, conj, a, b, dims):
        gr, gi, gs = _bf(g_v[km, 0:64, :]), _bf(g_v[km, 64:128, :]), _bf(gs_v[km])
        m1 = lax.dot_general(gr, a.astype(bf16), dims, preferred_element_type=f32)
        m2 = lax.dot_general(gi, b.astype(bf16), dims, preferred_element_type=f32)
        if conj:
            m3 = lax.dot_general(gs, (b - a).astype(bf16), dims, preferred_element_type=f32)
            return m1 + m2, m3 + (m1 - m2)
        m3 = lax.dot_general(gs, (a + b).astype(bf16), dims, preferred_element_type=f32)
        return m1 - m2, m3 - (m1 + m2)

    def dft128(p, k1):
        n = 112 if p else 120
        pad = jnp.zeros((128 - n, 128), f32)
        yr = jnp.concatenate([Y[p].ld(k1 * 256, n), pad], axis=0)
        yi = jnp.concatenate([Y[p].ld(k1 * 256 + 128, n), pad], axis=0)
        xr, xi = cmul3(k1 if k1 < 8 else 16 - k1, k1 >= 8, yr, yi, NT_DIMS)
        X2[p].st(k1 * 256, xr)
        X2[p].st(k1 * 256 + 128, xi)

    def wprep(w_v, wt_v, a):
        w32 = pltpu.bitcast(w_v[0:DH, a * 128:(a + 1) * 128], u32)
        ny = jnp.broadcast_to(w_v[DH:DH + 1, a * 128:(a + 1) * 128].astype(f32), (8, 128))
        ny = lax.shift_right_logical(lax.bitcast_convert_type(ny, u32), np.uint32(16))
        tile = jnp.concatenate([w32, jnp.where(row0, ny, np.uint32(0)), jnp.zeros((8, 128), u32)], axis=0).T
        for j in range(8):
            wt_v[pl.ds(a * WP + 17 * j, 8), :] = tile[16 * j:16 * j + 8, :]
            wt_v[pl.ds((15 - a) * WP + 17 * (7 - j) + 8, 8), :] = tile[16 * j + 8:16 * j + 16, :]

    def idft128(p, k1):
        wr32 = jnp.concatenate([wtr_v[pl.ds(a * WP + k1, 8, stride=17), :] for a in range(16)], axis=0)
        wi32 = jnp.concatenate([wti_v[pl.ds(a * WP + k1, 8, stride=17), :] for a in range(16)], axis=0)
        wr, wi = (_hi(wr32), _hi(wi32)) if p else (_lo(wr32), _lo(wi32))
        xr, xi = X2[p].ld(k1 * 256, 128), X2[p].ld(k1 * 256 + 128, 128)
        vr, vi = cmul3(k1 if k1 < 8 else 16 - k1, k1 < 8, xr * wr - xi * wi, xr * wi + xi * wr, TN_DIMS)
        vb, r0 = vbuf(p, k1)
        vb.st(r0, vr)
        vb.st(r0 + 128, vi)

    def rad_inv(p, j):
        r = 8 * j
        src = [vbuf(p, k1) for k1 in range(16)]
        re = [vb.ld(r0 + r, 8) for vb, r0 in src]
        im = [vb.ld(r0 + 128 + r, 8) for vb, r0 in src]
        ore, oim = _fft16(re, im, +1)
        for s1 in range(16):
            Z[p].st(s1 * 256 + r, ore[s1])
            Z[p].st(s1 * 256 + 128 + r, oim[s1])

    def idftd(p, zb, a):
        z = jnp.concatenate([zb.ld(a * 256, 128), zb.ld(a * 256 + 128, 128)], axis=1).astype(bf16)
        lhs = jnp.concatenate([_bf(bd_v[p, 0]), _bf(bd_v[p, 1])], axis=1)
        return lax.dot_general(lhs, z, NT_DIMS, preferred_element_type=f32)

    def cols(ch, t=0, n=CW):
        if isinstance(ch, int):
            return pl.ds(ch * CW + t * 128, n)
        return pl.ds(pl.multiple_of(ch * CW, CW) + t * 128, n)

    def prologue(ch):
        zo, he = Z[PB].at_rows(ch * (TPC * 256), TPC * 256), HE.at_rows(ch * (TPC * DH), TPC * DH)
        e = jnp.concatenate([idftd(PB, zo, t) for t in range(TPC)], axis=1)
        o = jnp.concatenate([he.ld(t * DH, DH) for t in range(TPC)], axis=1)
        acc = [None] * 4
        for j in range(DH // 16):
            ej, oj = e[16 * j:16 * j + 16], o[16 * j:16 * j + 16]
            for k, (r, y) in enumerate(((16 * j, ej + oj), (DH + 16 * j, ej - oj))):
                hs = x_v[r:r + 16, cols(ch)].astype(f32) + y
                hb_v[r:r + 16, cols(ch)] = hs.astype(bf16)
                q = (2 * j + k) % 4
                acc[q] = hs if acc[q] is None else acc[q] + hs
        mean = _colsum((acc[0] + acc[1]) + (acc[2] + acc[3])) * (1.0 / D)
        acc = [None] * 4
        for j in range(D // 16):
            d = hb_v[16 * j:16 * j + 16, cols(ch)].astype(f32) - mean
            acc[j % 4] = d * d if acc[j % 4] is None else acc[j % 4] + d * d
        scale = lax.rsqrt(_colsum((acc[0] + acc[1]) + (acc[2] + acc[3])) * (1.0 / D) + EPS)
        hn = ((hb_v[:, cols(ch)].astype(f32) - mean) * scale).astype(bf16)
        return hn

    def gate_up(hn):
        g = lax.dot_general(hn, wg_v[...], TN_DIMS, preferred_element_type=f32)
        u = lax.dot_general(hn, wu_v[...], TN_DIMS, preferred_element_type=f32)
        return (g * u).astype(bf16)

    def down(ch, hh):
        for t in range(TPC):
            y = lax.dot_general(wd_v[...], hh(t), NT_DIMS, preferred_element_type=f32)
            h = hb_v[:, cols(ch, t, 128)].astype(f32)
            out_v[:, cols(ch, t, 128)] = (h + y.astype(bf16).astype(f32)).astype(bf16)
            pltpu.make_async_copy(out_v.at[:, cols(ch, t, 128)], out_hbm.at[:, cols(ch, t, 128)], out_sem).start()

    last = NT - NT // XC
    ln1(0)
    for a in range(1, last):
        if a % (NT // XC) == 0:
            x_cp[a // (NT // XC)].wait()
        fwd_tile(a - 1)
        ln1(a)
    x_cp[XC - 1].wait()
    for a in range(last, NT):
        ln1(a)
    for a in range(last - 1, NT):
        dftd_o(a)
    for a in range(last - 1, NT):
        dftd_e(a, 0)
        dftd_e(a, 1)
    for j in range(14):
        rad_fwd(1, j)
    cp_wr.wait()
    for q in range(32):
        if q == 24:
            cp_wi.wait()
        dft128((PA, PB)[q // 16], q % 16)
        if 1 <= q < 16:
            rad_fwd(0, q - 1)
        if q >= 16:
            for a in (2 * (q % 8), 2 * (q % 8) + 1):
                wprep(*((wr_v, wtr_v) if q < 24 else (wi_v, wti_v)), a)
    cp_bar.wait()
    for k1 in range(16):
        idft128(PA, k1)
    for k1 in range(16):
        idft128(PB, k1)
        if k1 < 8:
            rad_inv(PA, 2 * k1)
            rad_inv(PA, 2 * k1 + 1)
    for a in range(NT):
        HE.st(a * DH, idftd(PA, Z[PA], a))
        rad_inv(PB, a)
    hn = prologue(0)
    for cp in cp_gu:
        cp.wait()
    for it in range(N_IT):
        nxt = prologue((it + 1) * UNROLL) if it + 1 < N_IT else None
        hh_v[it * CW:(it + 1) * CW, :] = gate_up(hn)
        hn = nxt
    cp_wd.wait()

    def body(it, carry):
        hn = prologue(it * UNROLL + 1)
        down(it * UNROLL, lambda t: hh_v[pl.ds(pl.multiple_of(it * CW, CW) + t * 128, 128), :])
        for k in range(1, UNROLL):
            nxt = prologue(it * UNROLL + k + 1) if k < UNROLL - 1 else None
            hh = gate_up(hn)
            down(it * UNROLL + k, lambda t: hh[t * 128:(t + 1) * 128])
            hn = nxt
        return carry

    lax.fori_loop(0, N_IT, body, 0)
    pltpu.make_async_copy(out_v, out_hbm, out_sem).wait()


@jax.jit
def pallas_sequential_preLN__spectral_gfnet__glu_gated_bilinear__prompt_kernel(
    A_x: jax.Array,
    A_w_r: jax.Array,
    A_w_i: jax.Array,
    B_x: jax.Array,
    B_w_gate: jax.Array,
    B_w_up: jax.Array,
    B_w_down: jax.Array,
):
    del B_x
    zc = np.zeros((24, 128), np.int32)
    zc[16:] = np.arange(128)
    any_spec = pl.BlockSpec(memory_space=pl.ANY)
    vm = pltpu.VMEM
    out_t = pl.pallas_call(
        _kernel,
        out_shape=jax.ShapeDtypeStruct((D, S), bf16),
        in_specs=[any_spec] * 7,
        out_specs=any_spec,
        scratch_shapes=[
            vm((D, S), bf16), vm((DH + 1, S), bf16), vm((DH + 1, S), bf16),
            vm((D, F), bf16), vm((D, F), bf16), vm((D, F), bf16),
            vm((24, 128), jnp.int32), vm((8, 128), jnp.int32),
            vm((FD_ROWS, 128), u32), vm((9, 128, 128), u32), vm((9, 64, 128), u32), vm((2, 2, DH // 2, 128), u32),
            vm((16 * WP + 16, 128), u32), vm((16 * WP + 16, 128), u32),
            vm((D, S), bf16), vm((N_IT * CW, F), bf16), vm((D, S), bf16),
            pltpu.SemaphoreType.DMA((XC + 6,)),
        ] + [vm((sum(_ROWS[n] for n in group), 128), u32) for group in _GROUPS],
        compiler_params=pltpu.CompilerParams(vmem_limit_bytes=100 * 2**20),
        name="gfnet_glu",
    )(A_x.reshape(S, D).T, A_w_r.T, A_w_i.T, B_w_gate, B_w_up, B_w_down.T, zc)
    return out_t.T.reshape(1, S, D)
```
